```python
import jax
import jax.numpy as jnp

def _softmax(x, axis=-1):
    return jax.nn.softmax(x, axis=axis)
def _gelu(x):
    return jax.nn.gelu(x, approximate=True)
def _silu(x):
    return jax.nn.silu(x)
def _sigmoid(x):
    return jax.nn.sigmoid(x)
def _layernorm(x, axis=-1, eps=1e-5):
    m = jnp.mean(x, axis=axis, keepdims=True)
    v = jnp.var(x, axis=axis, keepdims=True)
    return (x - m) / jnp.sqrt(v + eps)
def _scatter_add(tgt, idx, src, axis=0):
    return tgt.at[idx].add(src)
def _segment_sum(src, seg, n):
    return jax.ops.segment_sum(src, seg, n)
class _Rng:
    def __init__(self, key):
        self._k = key
    def _next(self):
        self._k, sub = jax.random.split(self._k)
        return sub
    def normal(self, shape):
        return jax.random.normal(self._next(), shape, dtype=jnp.bfloat16)
    def randint(self, lo, hi, shape):
        return jax.random.randint(self._next(), shape, lo, hi, dtype=jnp.int32)
    def uniform(self, shape, lo=0.0, hi=1.0):
        return jax.random.uniform(self._next(), shape, jnp.bfloat16, lo, hi)
    def permutation(self, n):
        return jax.random.permutation(self._next(), n)


kernel_name = 'recurrent_scan__sliding_local_dilated__geglu_ffn__prompt'

def setup_inputs():
    _rng = _Rng(jax.random.key(int.from_bytes(__import__("os").urandom(4), "little")))
    _w = (lambda a: (lambda t: t.astype(jnp.bfloat16) if jnp.issubdtype(t.dtype, jnp.floating) else t)(jnp.asarray(a)))
    def _A_setup():
        B, S, D = 1, 2048, 1024
        return {
            "x": _w((lambda *s: _rng.normal(s) * 0.05)(B, S, D)),
            "wqkv": _w((lambda *s: _rng.normal(s) * 0.05)(D, 3 * D)),
            "wo": _w((lambda *s: _rng.normal(s) * 0.05)(D, D)),
        }
    _A_in = _A_setup()

    def _B_setup():
        B, S, D, F = 1, 2048, 1024, 3584
        return {
            "x": _w((lambda *s: _rng.normal(s) * 0.05)(B, S, D)),
            "w_gate": _w((lambda *s: _rng.normal(s) * 0.05)(D, F)),
            "w_up": _w((lambda *s: _rng.normal(s) * 0.05)(D, F)),
            "w_down": _w((lambda *s: _rng.normal(s) * 0.05)(F, D)),
        }
    _B_in = _B_setup()

    return {
        "A_x": _A_in["x"],
        "A_wqkv": _A_in["wqkv"],
        "A_wo": _A_in["wo"],
        "B_x": _B_in["x"],
        "B_w_gate": _B_in["w_gate"],
        "B_w_up": _B_in["w_up"],
        "B_w_down": _B_in["w_down"],
    }

def reference(A_x, A_wqkv, A_wo, B_x, B_w_gate, B_w_up, B_w_down):
    def _A_ref(x, wqkv, wo):
        B, S, D = x.shape
        H = 32; Dh = D // H
        W, dil = 8, 2
        qkv = (lambda x, *d: x.transpose(*d))((x @ wqkv).reshape(B, S, 3, H, Dh), 2, 0, 3, 1, 4)
        q, k, v = qkv[0], qkv[1], qkv[2]
        scale = Dh ** -0.5
        pos = jnp.arange(S)
        off = jnp.arange(W) * dil
        idx = pos[:, None] - off[None, :]
        mask = idx >= 0
        idx_c = jnp.where(mask, idx, 0).reshape(-1)
        kg = k[:, :, idx_c, :].reshape(B, H, S, W, Dh)
        vg = v[:, :, idx_c, :].reshape(B, H, S, W, Dh)
        logits = jnp.einsum("bhsd,bhswd->bhsw", q, kg) * scale
        logits = jnp.where(mask[None, None, :, :], logits, -1e9)
        attn = _softmax(logits, axis=-1)
        o = jnp.einsum("bhsw,bhswd->bhsd", attn, vg)
        return (lambda x, *d: x.transpose(*d))(o, 0, 2, 1, 3).reshape(B, S, D) @ wo

    def _B_ref(x, w_gate, w_up, w_down):
        return (_gelu(x @ w_gate) * (x @ w_up)) @ w_down

    x = A_x
    xn = _layernorm(x, axis=-1)
    s = _A_ref(xn, A_wqkv, A_wo)
    g = _silu(_B_ref(xn, B_w_gate, B_w_up, B_w_down))
    return x + s * g
```

```python
import jax
import jax.numpy as jnp
from jax import lax
import jax.experimental.pallas as pl
import jax.experimental.pallas.tpu as pltpu

F32 = jnp.float32
BF16 = jnp.bfloat16

N_HEADS = 32
WINDOW = 8
DILATION = 2
LN_EPS = 1e-5
MASKED_LOGIT = -1e9

LANES = 128
HALO = 16
TILE = 256
FCHUNK = 512
ATT_ROWS = 32


def _dot(a, b):
    return jnp.dot(a, b, preferred_element_type=F32)


def _lhs_operands(a11, a12, a21, a22):
    ops = (a11 + a22, a21 + a22, a11, a22, a11 + a12, a21 - a11, a12 - a22)
    return [t.astype(BF16) for t in ops]


def _strassen(lhs, rhs, fill=None):
    def add(p, q, sign=1):
        p, q = rhs(*p).astype(F32), rhs(*q).astype(F32)
        return (p + q if sign > 0 else p - q).astype(BF16)

    def prod(i, b):
        m = _dot(lhs(i), b)
        if fill is not None:
            fill()
        return m

    b11, b12, b21, b22 = (0, 0), (0, 1), (1, 0), (1, 1)
    m2 = prod(1, rhs(*b11))
    m4 = prod(3, add(b21, b11, -1))
    c21 = m2 + m4
    m5 = prod(4, rhs(*b22))
    m3 = prod(2, add(b12, b22, -1))
    c12 = m3 + m5
    m1 = prod(0, add(b11, b22))
    c22 = (m1 + (m3 - m2)) + prod(5, add(b11, b12))
    c11 = (m1 + (m4 - m5)) + prod(6, add(b21, b22))
    return c11, c12, c21, c22


def _layernorm(x):
    x = x.astype(F32)
    inv_n = 1.0 / x.shape[-1]
    c = x - jnp.sum(x, axis=-1, keepdims=True) * inv_n
    var = jnp.sum(c * c, axis=-1, keepdims=True) * inv_n
    return c * lax.rsqrt(var + LN_EPS)


def _geglu(g, u):
    k0 = 0.7978845608028654
    t = jnp.tanh(g * (k0 + (k0 * 0.044715) * (g * g)))
    return ((0.5 * g) * u) * (1.0 + t)


def _silu(d):
    h = 0.5 * d
    return h * (1.0 + jnp.tanh(h))


def _lane_bit(shape, bit):
    return (lax.broadcasted_iota(jnp.int32, shape, 1) & bit) != 0


def _swap_group_and_lane_bits(cols):
    cols = list(cols)
    for gbit, lbit in ((1, 4), (2, 8), (4, 16)):
        hi = _lane_bit(cols[0].shape, lbit)
        for i in range(len(cols)):
            if not i & gbit:
                a, b = cols[i], cols[i | gbit]
                cols[i] = jnp.where(hi, pltpu.roll(b, lbit, 1), a)
                cols[i | gbit] = jnp.where(hi, b, pltpu.roll(a, LANES - lbit, 1))
    return cols


def _kernel(x_hbm, wqkv_hbm, wo_hbm, wg_hbm, wu_hbm, wd_hbm, out_hbm,
            xbuf, wgu, wqkv, wd, wo, xa, ha, qkv, oa, gbuf, obuf,
            x_sem, wgu_sem, wqkv_sem, w_sem, out_sem):
    _, half, d = x_hbm.shape
    n_tiles = half // TILE
    n_chunks = wgu.shape[0]
    hd, hc = d // 2, FCHUNK // 2
    groups = d // LANES

    def x_copy(t):
        rows = pl.ds(t * TILE, TILE)
        return pltpu.make_async_copy(x_hbm.at[:, rows], xbuf.at[:, rows], x_sem.at[t])

    def wgu_copies(c):
        cols = pl.ds(c * FCHUNK, FCHUNK)
        return [
            pltpu.make_async_copy(w.at[:, cols], wgu.at[c, i], wgu_sem.at[2 * c + i])
            for i, w in enumerate((wg_hbm, wu_hbm))
        ]

    def wgu_wait(c):
        for i in range(2):
            buf = wgu.at[c, i]
            pltpu.make_async_copy(buf, buf, wgu_sem.at[2 * c + i]).wait()

    def wqkv_copy(p):
        src = wqkv_hbm.at[pl.ds((p % 2) * hd, hd), pl.ds((p // 2) * d, d)]
        return pltpu.make_async_copy(src, wqkv.at[p], wqkv_sem.at[p])

    wd_copy = pltpu.make_async_copy(wd_hbm, wd, w_sem.at[0])
    wo_copy = pltpu.make_async_copy(wo_hbm, wo, w_sem.at[1])

    def out_copy(t, slot):
        rows = pl.ds(pl.multiple_of(t * TILE, TILE), TILE)
        return pltpu.make_async_copy(obuf.at[slot], out_hbm.at[:, rows], out_sem.at[slot])

    def norm_rows(lo, n):
        rows = pl.ds(lo, n)
        top, bot = _layernorm(xbuf[0, rows, :]), _layernorm(xbuf[1, rows, :])
        ops = _lhs_operands(top[:, :hd], top[:, hd:], bot[:, :hd], bot[:, hd:])
        for i, op in enumerate(ops):
            xa[i, rows, :] = op

    def ffn_up(c, rows, width, fill=None):
        for lo in range(0, hc, width):
            g, u = [
                _strassen(
                    lambda i: xa[i, rows, :],
                    lambda r, s: wgu[c, mat, pl.ds(r * hd, hd), pl.ds(s * hc + lo, width)],
                    fill,
                )
                for mat in range(2)
            ]
            ops = _lhs_operands(*[_geglu(gi, ui) for gi, ui in zip(g, u)])
            for i, op in enumerate(ops):
                ha[c, i, rows, pl.ds(lo, width)] = op

    def filler(jobs):
        jobs = list(jobs)

        def fill():
            if jobs:
                jobs.pop(0)()

        return fill, jobs

    x_copy(0).start()
    for cp in wgu_copies(0):
        cp.start()
    x_copy(1).start()
    x_copy(0).wait()
    norm_rows(0, TILE)
    wgu_wait(0)
    for t in range(n_tiles):
        more = t + 1 < n_tiles
        if more:
            x_copy(t + 1).wait()
        if t == 0:
            for tt in range(2, n_tiles):
                x_copy(tt).start()
        if t == 1:
            for c in range(1, n_chunks):
                for cp in wgu_copies(c):
                    cp.start()
                wqkv_copy(c - 1).start()
            wd_copy.start()
            wo_copy.start()
        step = 32
        fill, left = filler(
            [lambda lo=lo: norm_rows(lo, step)
             for lo in range((t + 1) * TILE, (t + 2) * TILE, step)] if more else [])
        ffn_up(0, pl.ds(t * TILE, TILE), hc, fill)
        assert not left

    assert n_chunks - 1 == wqkv.shape[0]

    def shuffle_rows(p, lo, n):
        rows = pl.ds(lo, n)
        w = pltpu.bitcast(wqkv[p, rows, :], jnp.uint32)
        cols = _swap_group_and_lane_bits(
            [w[:, j * LANES:(j + 1) * LANES] for j in range(groups)])
        wqkv[p, rows, :] = pltpu.bitcast(jnp.concatenate(cols, axis=1), BF16)

    @pl.loop(1, n_chunks)
    def _(c):
        wgu_wait(c)
        buf = wqkv.at[c - 1]
        pltpu.make_async_copy(buf, buf, wqkv_sem.at[c - 1]).wait()
        step = 32
        fill, left = filler(
            [lambda lo=lo: shuffle_rows(c - 1, lo, step) for lo in range(0, hd, step)])
        ffn_up(c, pl.ds(0, half), LANES, fill)
        assert not left

    @pl.loop(0, 3)
    def _(p):
        for j in range(groups // 2):
            c11, c12, c21, c22 = _strassen(
                lambda i: xa[i],
                lambda r, s: wqkv[2 * p + r, :, pl.ds(s * hd + j * LANES, LANES)],
            )
            for g, top, bot in ((j, c11, c21), (j + groups // 2, c12, c22)):
                qkv[p, g, pl.ds(0, HALO), :] = jnp.broadcast_to(top[:1], (HALO, LANES))
                qkv[p, g, pl.ds(HALO, half), :] = top
                qkv[p, g, pl.ds(HALO + half, half), :] = bot

    scale = float(d // N_HEADS) ** -0.5

    def attend(pos, off, n, masked):
        def load(p, g, w):
            return qkv[p, g, pl.ds(pos + (HALO + off - DILATION * w), n), :]

        q = [load(0, g, 0) for g in range(groups)]
        odd1, odd2 = _lane_bit((n, LANES), 1), _lane_bit((n, LANES), 2)
        logits = []
        for w in range(WINDOW):
            s = q[0] * load(1, 0, w)
            for g in range(1, groups):
                s = s + q[g] * load(1, g, w)
            for bit, odd in ((1, odd1), (2, odd2)):
                s = s + jnp.where(odd, pltpu.roll(s, bit, 1), pltpu.roll(s, LANES - bit, 1))
            s = s * scale
            if masked and w:
                row = pos + off + lax.broadcasted_iota(jnp.int32, (n, LANES), 0)
                s = jnp.where(row >= DILATION * w, s, MASKED_LOGIT)
            logits.append(s)
        top = logits[0]
        for s in logits[1:]:
            top = jnp.maximum(top, s)
        e = [jnp.exp(s - top) for s in logits]
        total = e[0]
        for t in e[1:]:
            total = total + t
        inv = 1.0 / total
        prob = [t * inv for t in e]
        out = []
        for g in range(groups):
            o = prob[0] * load(2, g, 0)
            for w in range(1, WINDOW):
                o = o + prob[w] * load(2, g, w)
            out.append(o)
        return jnp.concatenate(_swap_group_and_lane_bits(out), axis=1)

    wd_copy.wait()
    wo_copy.wait()

    @pl.loop(0, n_tiles)
    def _(t):
        slot = t % 2
        pos = pl.multiple_of(t * TILE, TILE)
        rows = pl.ds(pos, TILE)

        @pl.when(t >= 2)
        def _():
            out_copy(t - 2, slot).wait()

        def attend_rows(lo):
            top = attend(pos, lo, ATT_ROWS, lo < HALO)
            bot = attend(pos, half + lo, ATT_ROWS, False)
            ops = _lhs_operands(top[:, :hd], top[:, hd:], bot[:, :hd], bot[:, hd:])
            for i, op in enumerate(ops):
                oa[i, pl.ds(lo, ATT_ROWS), :] = op

        fill, left = filler(
            [lambda lo=lo: attend_rows(lo) for lo in range(0, TILE, ATT_ROWS)])
        width = 2 * LANES
        for lo in range(0, hd, width):
            down = _strassen(
                lambda i: jnp.concatenate(
                    [ha[c, i, rows, :] for c in range(n_chunks)], axis=1),
                lambda r, s: jnp.concatenate(
                    [wd[pl.ds(c * FCHUNK + r * hc, hc), pl.ds(s * hd + lo, width)]
                     for c in range(n_chunks)], axis=0),
                fill,
            )
            for i, blk in enumerate(down):
                gbuf[i // 2, :, pl.ds((i % 2) * hd + lo, width)] = _silu(blk)
        assert not left
        for lo in range(0, hd, width):
            proj = _strassen(
                lambda i: oa[i],
                lambda r, s: wo[pl.ds(r * hd, hd), pl.ds(s * hd + lo, width)],
            )
            for i, blk in enumerate(proj):
                cols = pl.ds((i % 2) * hd + lo, width)
                res = xbuf[i // 2, rows, cols].astype(F32) + blk * gbuf[i // 2, :, cols]
                obuf[slot, i // 2, :, cols] = res.astype(obuf.dtype)
        out_copy(t, slot).start()

    for t in range(max(n_tiles - 2, 0), n_tiles):
        out_copy(t, t % 2).wait()


@jax.jit
def pallas_recurrent_scan__sliding_local_dilated__geglu_ffn__prompt_kernel(
    A_x: jax.Array,
    A_wqkv: jax.Array,
    A_wo: jax.Array,
    B_x: jax.Array,
    B_w_gate: jax.Array,
    B_w_up: jax.Array,
    B_w_down: jax.Array,
):
    del B_x
    b, s, d = A_x.shape
    f = B_w_gate.shape[1]
    assert b == 1 and d == N_HEADS * 32 and s % (2 * TILE) == 0 and f % FCHUNK == 0
    half, n_chunks = s // 2, f // FCHUNK

    hbm = pl.BlockSpec(memory_space=pl.ANY)
    out = pl.pallas_call(
        _kernel,
        out_shape=jax.ShapeDtypeStruct((2, half, d), A_x.dtype),
        in_specs=[hbm] * 6,
        out_specs=hbm,
        scratch_shapes=[
            pltpu.VMEM((2, half, d), BF16),
            pltpu.VMEM((n_chunks, 2, d, FCHUNK), BF16),
            pltpu.VMEM((6, d // 2, d), BF16),
            pltpu.VMEM((f, d), BF16),
            pltpu.VMEM((d, d), BF16),
            pltpu.VMEM((7, half, d // 2), BF16),
            pltpu.VMEM((n_chunks, 7, half, FCHUNK // 2), BF16),
            pltpu.VMEM((3, d // LANES, HALO + s, LANES), F32),
            pltpu.VMEM((7, TILE, d // 2), BF16),
            pltpu.VMEM((2, TILE, d), F32),
            pltpu.VMEM((2, 2, TILE, d), A_x.dtype),
            pltpu.SemaphoreType.DMA((half // TILE,)),
            pltpu.SemaphoreType.DMA((2 * n_chunks,)),
            pltpu.SemaphoreType.DMA((6,)),
            pltpu.SemaphoreType.DMA((2,)),
            pltpu.SemaphoreType.DMA((2,)),
        ],
        compiler_params=pltpu.CompilerParams(vmem_limit_bytes=120 * 1024 * 1024),
        name="fused_local_attn_geglu",
    )(A_x.reshape(2, half, d), A_wqkv, A_wo, B_w_gate, B_w_up, B_w_down)
    return out.reshape(b, s, d)
```

```python
import contextlib
import jax
import jax.numpy as jnp
from jax import lax
import jax.experimental.pallas as pl
import jax.experimental.pallas.tpu as pltpu


PH = "1234"
FLAGS = {}
SCOPES = 0


def scope(name):
    return jax.named_scope(name) if SCOPES else contextlib.nullcontext()


F32 = jnp.float32
BF16 = jnp.bfloat16
U32 = jnp.uint32

N_HEADS = 32
WINDOW = 8
DILATION = 2
LN_EPS = 1e-5
MASKED_LOGIT = -1e9

LANES = 128
SUB = 8
PACK = 16
HALO = 16
FCHUNK = 512
NORM_TILE = 128
OUT_TILE = 256
ATT3 = 96
UP_ROWS = [128,128,128,128]
WO_ROWS = [256]
WO_WIDTH = 256
SLOT3 = [0,1,2,4]
OUTER3 = [0,1,2,3,4,5,6]
SLOT4 = [2,3,4,5,6]
END1 = 2
END2 = 27
END3 = 37
AHEAD = 4
MARGIN = 2
ATT3_LO = 49
ATT3_HI = 147
ASLOT3 = [0,1]
ORDER = (1, 3, 4, 2, 0, 5, 6)
END4 = 47


def _add(a, b):
    return [[x.astype(F32) + y.astype(F32) for x, y in zip(r, s)] for r, s in zip(a, b)]


def _sub(a, b):
    return [[x.astype(F32) - y.astype(F32) for x, y in zip(r, s)] for r, s in zip(a, b)]


_LHS = ((_add, 0, 3), (_add, 2, 3), (None, 0), (None, 3), (_add, 0, 1), (_sub, 2, 0), (_sub, 1, 3))
_RHS = ((_add, 0, 3), (None, 0), (_sub, 1, 3), (_sub, 2, 0), (None, 3), (_add, 0, 1), (_add, 2, 3))


def _operands(side, size, block):
    if size == 1:
        op = block(0, 0, 0).astype(BF16)
        return lambda i: op
    h, n = size // 2, 7 ** (size.bit_length() - 2)
    parts = {}

    def get(i):
        use = i // n
        if use not in parts:
            op, *quads = side[use]
            terms = [[[block(q // 2 * h + r, q % 2 * h + c, use) for c in range(h)]
                      for r in range(h)] for q in quads]
            part = op(*terms) if op else terms[0]
            parts[use] = _operands(side, h, lambda r, c, _: part[r][c])
        return parts[use](i % n)

    return get


def _strassen(levels, product, base=0):
    if levels == 0:
        return [[product(base)]]

    def m(i):
        return _strassen(levels - 1, product, base + (i - 1) * 7 ** (levels - 1))

    m2, m4 = m(2), m(4)
    c21 = _add(m2, m4)
    m5, m3 = m(5), m(3)
    c12 = _add(m3, m5)
    m1 = m(1)
    c22 = _add(_add(m1, _sub(m3, m2)), m(6))
    c11 = _add(_add(m1, _sub(m4, m5)), m(7))
    return [r + s for r, s in zip(c11, c12)] + [r + s for r, s in zip(c21, c22)]


def _merge(*lists):
    keyed = [((i + 0.5) / len(l), n, x) for n, l in enumerate(lists) for i, x in enumerate(l)]
    return [x for _, _, x in sorted(keyed, key=lambda t: t[:2])]


class _Matmuls:
    def __init__(self, *plan):
        self.calls, self.jobs = 0, {}
        for jobs, slots in plan:
            for i, job in enumerate(jobs):
                self.jobs.setdefault(slots[i * len(slots) // len(jobs)], []).append(job)

    def __call__(self, lhs, rhs):
        value = jnp.dot(lhs, rhs, preferred_element_type=F32)
        jobs = self.jobs.pop(self.calls, [])
        for i, job in enumerate(jobs):
            row = i * (value.shape[0] // SUB) // len(jobs) * SUB
            job(value[row:row + SUB, :LANES])
        self.calls += 1
        return value


def _layernorm(x):
    inv_n = 1.0 / x.shape[-1]
    c = x - jnp.sum(x, axis=-1, keepdims=True) * inv_n
    var = jnp.sum(c * c, axis=-1, keepdims=True) * inv_n
    return c * lax.rsqrt(var + LN_EPS)


def _geglu(g, u):
    k0 = 0.7978845608028654
    t = jnp.tanh(g * (k0 + (k0 * 0.044715) * (g * g)))
    return ((0.5 * g) * u) * (1.0 + t)


def _silu(d):
    h = 0.5 * d
    return h * (1.0 + jnp.tanh(h))


def _lane_bit(bit):
    return (lax.broadcasted_iota(jnp.int32, (SUB, LANES), 1) & bit) != 0


def _lane_groups(x):
    return [x[:, j:j + LANES] for j in range(0, x.shape[1], LANES)]


def _swap_group_and_lane_bits(cols):
    cols = list(cols)
    for gbit, lbit in ((1, 4), (2, 8), (4, 16)):
        hi = _lane_bit(lbit)
        for i in range(len(cols)):
            if not i & gbit:
                a, b = cols[i], cols[i | gbit]
                cols[i] = jnp.where(hi, pltpu.roll(b, lbit, 1), a)
                cols[i | gbit] = jnp.where(hi, b, pltpu.roll(a, LANES - lbit, 1))
    return cols


def _load_rows(ref, index, starts, n):
    words = ref.bitcast(U32)
    starts = [lo // 2 if isinstance(lo, int) else pl.multiple_of(lo // 2, SUB) for lo in starts]
    return jnp.concatenate([
        jnp.concatenate([pltpu.bitcast(words[(*index, g, pl.ds(lo, n // 2))], BF16) for lo in starts], axis=0)
        for g in range(ref.shape[-3])], axis=1)


def _kernel(x_hbm, wqkv_hbm, wo_hbm, wg_hbm, wu_hbm, wd_hbm, out_hbm,
            xbuf, wbig, wo, xa1, xa2, wgu, wa, ha, qk, vbuf, gbuf, obuf,
            x_sem, wbig_sem, wgu_sem, wo_sem, out_sem):
    _, quarter, d = x_hbm.shape
    half = 2 * quarter
    n_chunks = ha.shape[1]
    hd, qd = d // 2, d // 4
    groups = d // LANES
    n_norm, n_out = quarter // NORM_TILE, 2 * quarter // OUT_TILE

    class Copies:
        def __init__(self, src, dst, sem):
            self.cps = [pltpu.make_async_copy(src(j), dst(j), sem) for j in range(2)]

        def start(self):
            for cp in self.cps:
                cp.start()

        def wait(self):
            for cp in self.cps:
                cp.wait()

    def x_copy(t):
        rows = pl.ds(t * NORM_TILE, NORM_TILE)
        return Copies(lambda j: x_hbm.at[:, rows, pl.ds(j * hd, hd)],
                      lambda j: xbuf.at[j, :, rows], x_sem.at[t])

    def wqk_copy(p):
        return Copies(lambda j: wqkv_hbm.at[p % 2, :, pl.ds(p // 2 * d + j * hd, hd)],
                      lambda j: wbig.at[j, p], wbig_sem.at[p])

    def wv_copy(a):
        return Copies(lambda j: wqkv_hbm.at[:, :, pl.ds(2 * d + j * hd + a * qd, qd)],
                      lambda j: wbig.at[j, pl.ds(4, 2), :, pl.ds(a * qd, qd)], wbig_sem.at[4 + a])

    def wd_copy(c):
        rows = pl.ds(pl.multiple_of(c * FCHUNK, FCHUNK), FCHUNK)
        return Copies(lambda j: wd_hbm.at[rows, pl.ds(j * hd, hd)],
                      lambda j: wbig.at[j, c], wbig_sem.at[c])

    def wgu_copy(c):
        cols = pl.ds(pl.multiple_of(c * FCHUNK, FCHUNK), FCHUNK)
        return Copies(lambda j: (wg_hbm, wu_hbm)[j].at[:, cols],
                      lambda j: wgu.at[c % 3, j], wgu_sem.at[c % 3])

    wo_copy = Copies(lambda j: wo_hbm.at[:, pl.ds(j * hd, hd)], lambda j: wo.at[j], wo_sem)

    def out_copy(step):
        rows = pl.ds(pl.multiple_of(step // 2 * OUT_TILE, OUT_TILE), OUT_TILE)
        cols = pl.ds(pl.multiple_of(step % 2 * hd, hd), hd)
        return pltpu.make_async_copy(obuf.at[step], out_hbm.at[:, rows, cols], out_sem.at[step])

    def after(token, x):
        if token is None:
            return x
        return jnp.concatenate(
            [jnp.where(never, pltpu.bitcast(token, x.dtype), x[r:r + SUB])
             for r in range(0, x.shape[0], SUB)], axis=0)

    def xn_ref(q, g, part):
        return ha.bitcast(F32).at[groups + q * groups + g, part]

    def norm_jobs(t):
        def norm(q, lo, token):
            cols = [g for j in range(2)
                    for g in _lane_groups(xbuf[j, q, pl.ds(lo, SUB), :].astype(F32))]
            cols[0] = after(token, cols[0])
            for g, v in enumerate(_lane_groups(_layernorm(jnp.concatenate(cols, axis=1)))):
                xn_ref(q, g, lo // (quarter // 2))[pl.ds(lo % (quarter // 2), SUB), :] = v

        def split(u, lo):
            for g in range(groups // 2):
                ops = _operands(_LHS, 2, lambda r, c, _: xn_ref(
                    2 * r + u, c * groups // 2 + g, lo // (quarter // 2))[pl.ds(lo % (quarter // 2), PACK), :])
                for i in range(7):
                    xa1[i, g, pl.ds(u * quarter + lo, PACK), :] = ops(i)

        def last(q, lo, token):
            norm(q, lo + SUB, token)
            split(q - 2, lo)

        jobs = []
        for lo in range(t * NORM_TILE, (t + 1) * NORM_TILE, PACK):
            for u in range(2):
                jobs += [lambda tok, a=a: norm(*a, tok) for a in ((u, lo), (u, lo + SUB), (u + 2, lo))]
                jobs += [lambda tok, a=(u + 2, lo): last(*a, tok)]
        return jobs

    def shuffle_weight_jobs(p):
        def shuffle(lo, token):
            rows = pl.ds(lo, PACK)
            cols = _swap_group_and_lane_bits(
                [after(token, g) for j in range(2)
                 for g in _lane_groups(pltpu.bitcast(wbig[j, p, rows, :], U32))])
            for j in range(2):
                wbig[j, p, rows, :] = pltpu.bitcast(jnp.concatenate(cols[4 * j:4 * j + 4], axis=1), BF16)

        return [lambda tok, lo=lo: shuffle(lo, tok) for lo in range(0, hd, PACK)]

    def split_jobs(side, block, store, positions, uses=range(7)):
        def split(pos, use, token):
            first = side[use][1]
            ops = _operands(side, 4, lambda r, c, _: after(
                token if r // 2 * 2 + c // 2 == first else None, block(pos, r, c, use).astype(F32)))
            for i in range(7 * use, 7 * use + 7):
                store(pos, i, ops(i))

        return [lambda tok, a=(pos, use): split(*a, tok) for pos in positions for use in uses]

    def split_weight_jobs(c, positions, uses):
        def block(pos, r, s, use):
            mat, lo = pos
            return wgu[(c + 3 * use) % 3, mat, pl.ds(lo + r * qd, PACK), pl.ds(s * LANES, LANES)]

        def store(pos, i, op):
            mat, lo = pos
            wa[i, mat, pl.ds(lo, PACK), :] = op

        return split_jobs(_RHS, block, store, positions, uses)

    for cp in (x_copy(0), wv_copy(0), wv_copy(1), x_copy(1), x_copy(2), wqk_copy(0)):
        cp.start()
    with scope("S_x0wait"):
        x_copy(0).wait()
    never = jnp.abs(xbuf[0, 0, :SUB, :LANES].astype(F32)) < 0
    with scope("S_ln0"):
        for job in norm_jobs(0):
            job(None)
    wv = [_operands(_RHS, 2, lambda r, s, _, a=a: wbig[s, 4 + r, :, pl.ds(a * qd, qd)]) for a in range(2)]

    def project_v(t, parts, jobs):
        if not ("1" in PH and (t == 1 or "x" in PH or PH == "1234")):
            return
        matmul = _Matmuls((jobs, range(7 * len(parts) - END1)))
        with scope("S_p1"):
            for a in parts:
                out = _strassen(1, lambda i: matmul(_load_rows(
                    xa1, (i,), [u * quarter + t * NORM_TILE for u in range(2)], NORM_TILE), wv[a](i)))
                for r in range(2):
                    for s in range(2):
                        for g, v in enumerate(_lane_groups(out[r][s])):
                            for u in range(2):
                                ha[(s * hd + a * qd) // LANES + g, 2 * r + u,
                                   pl.ds(t * NORM_TILE, NORM_TILE), :] = (
                                       v[u * NORM_TILE:(u + 1) * NORM_TILE].astype(BF16))

    with scope("S_w0wait"):
        wv_copy(0).wait()
    project_v(0, [0], [])
    starts = ([x_copy(3), wqk_copy(1), wqk_copy(2), wqk_copy(3)], [wgu_copy(0)], [wgu_copy(1)], [wo_copy])
    shuffles = [[], [0], [1], [2, 3]]
    for t in range(n_norm):
        for cp in starts[t]:
            cp.start()
        if t == 0:
            wv_copy(1).wait()
        jobs = []
        if t + 1 < n_norm:
            x_copy(t + 1).wait()
            jobs.append(norm_jobs(t + 1))
        else:
            wgu_copy(0).wait()
        for p in shuffles[t]:
            wqk_copy(p).wait()
            jobs.append(shuffle_weight_jobs(p))
        project_v(t, [0, 1] if t else [1], _merge(*jobs))

    def project_qk(step):
        p, u = step // 2, step % 2
        row0 = u * quarter if isinstance(step, int) else pl.multiple_of(u * quarter, quarter)

        def aligned(x):
            return x if isinstance(x, int) else pl.multiple_of(x, PACK)

        def shuffle_v(lo, token):
            words = ha.bitcast(U32)
            cols = _swap_group_and_lane_bits(
                [after(token, words[g, step, pl.ds(lo // 2, SUB), :]) for g in range(groups)])
            rows = pl.ds(aligned(step * quarter) + (HALO + lo), PACK)
            for g in range(groups):
                vbuf[g, rows, :] = pltpu.bitcast(cols[g], BF16).astype(F32)

        def load_x(pos, r, c, use):
            g, lo = pos
            return xn_ref(r, 2 * c + g, (p + 2 * use) % 2)[pl.ds(aligned(u * (quarter // 4)) + lo, PACK), :]

        def store_x(pos, i, op):
            g, lo = pos
            xa2[i, g, pl.ds(aligned(step * (quarter // 4)) + lo, PACK), :] = op

        jobs = _merge(
            [lambda tok, lo=lo: shuffle_v(lo, tok) for lo in range(0, quarter, PACK)],
            split_jobs(_LHS, load_x, store_x, [(g, lo) for lo in range(0, quarter // 4, PACK) for g in range(2)]),
            split_weight_jobs(3 * step, [(p, aligned(u * (qd // 2)) + lo) for lo in range(0, qd // 2, PACK)],
                              ORDER[:AHEAD]))
        matmul = _Matmuls((jobs, range(END2)))
        with scope("S_p2"):
            for j in range(groups // 2 if "2" in PH else 0):
                rhs = _operands(_RHS, 2, lambda r, s, _: wbig[s, 2 * p + r, :, pl.ds(j * LANES, LANES)])
                out = _strassen(1, lambda i: matmul(_load_rows(xa1, (i,), [row0], quarter), rhs(i)))
                for r in range(2):
                    for s in range(2):
                        qk[p, j + s * groups // 2, pl.ds(row0 + (HALO + r * half), quarter), :] = out[r][s]

    project_qk(0)
    pl.loop(1, 4)(project_qk)

    for g in range(groups):
        for ref in (qk.at[1, g], vbuf.at[g]):
            ref[pl.ds(0, HALO), :] = jnp.broadcast_to(ref[pl.ds(HALO, 1), :], (HALO, LANES))

    scale = float(d // N_HEADS) ** -0.5

    def attend(pos, off, masked, token):
        def rows(w):
            return pl.ds(pos + (HALO + off - DILATION * w), SUB)

        q = [qk[0, g, rows(0), :] for g in range(groups)]
        q[0] = after(token, q[0])
        logits = []
        for w in range(WINDOW):
            s = q[0] * qk[1, 0, rows(w), :]
            for g in range(1, groups):
                s = s + q[g] * qk[1, g, rows(w), :]
            for bit in (1, 2):
                s = s + jnp.where(_lane_bit(bit), pltpu.roll(s, bit, 1), pltpu.roll(s, LANES - bit, 1))
            if masked and w:
                row = pos + off + lax.broadcasted_iota(jnp.int32, (SUB, LANES), 0)
                s = jnp.where(row >= DILATION * w, s, MASKED_LOGIT / scale)
            logits.append(s)
        top = logits[0]
        for s in logits[1:]:
            top = jnp.maximum(top, s)
        e = [jnp.exp2((s - top) * (scale * 1.4426950408889634)) for s in logits]
        total = e[0]
        for t in e[1:]:
            total = total + t
        inv = 1.0 / total
        out = []
        for g in range(groups):
            o = e[0] * vbuf[g, rows(0), :]
            for w in range(1, WINDOW):
                o = o + e[w] * vbuf[g, rows(w), :]
            out.append(o * inv)
        return _swap_group_and_lane_bits(out)

    def attend_jobs(pos, count, may_be_first):
        parts = []

        def job(lo, off, token):
            parts.append(attend(pos, off + lo, may_be_first and off + lo < HALO, token))
            if len(parts) == 4:
                for g in range(groups // 2):
                    ops = _operands(_LHS, 2, lambda r, c, _: jnp.concatenate(
                        [parts[2 * r + u][c * groups // 2 + g] for u in range(2)], axis=0))
                    for i in range(7):
                        xa1[i, g, pl.ds(pos + lo, PACK), :] = ops(i)
                parts.clear()

        return [lambda tok, a=(lo, off): job(*a, tok)
                for lo in range(0, count, PACK) for off in (0, SUB, half, half + SUB)]

    att4 = -(-(half - n_chunks * ATT3) // (3 * PACK)) * PACK

    @pl.loop(0, n_chunks)
    def _(c):
        @pl.when(c + 2 < n_chunks)
        def _():
            wgu_copy(c + 2).start()

        wd_copy(c).start()

        @pl.when(c + 1 < n_chunks)
        def _():
            wgu_copy(c + 1).wait()

        with scope("S_p3"):
            last = 49 * (len(UP_ROWS) - 1)
            ok = lambda r: [i for i in r if i % 7 in SLOT3]
            plan = []
            everywhere = [(mat, lo) for mat in range(2) for lo in range(0, qd, PACK)]
            n_now = 7 - AHEAD
            for k, use in enumerate(ORDER[AHEAD:]):
                end = 7 * (AHEAD + k) - MARGIN
                plan.append((split_weight_jobs(c, everywhere, [use]), ok(range(k * 40 // n_now, min(end, (k + 1) * 40 // n_now)))))
            for k, use in enumerate(ORDER[:AHEAD]):
                span = num = (END3 - 7) // AHEAD
                plan.append((split_weight_jobs(c + 1, everywhere, [use]), ok(range(last + max(7 * k + 7, 7 + k * span), last + 7 + (k + 1) * span))))
            plan.append((attend_jobs(pl.multiple_of(c * ATT3, PACK), ATT3, True),
                         [i for i in range(ATT3_LO, ATT3_HI) if i % 7 in ASLOT3]))
            matmul = _Matmuls(*plan)
            lo = 0
            for n in UP_ROWS if "3" in PH else []:
                out = _strassen(2, lambda i: matmul(
                    _load_rows(xa2, (i,), [lo], n), _load_rows(wa, (i,), [0], qd)))
                hid = [[_geglu(*_lane_groups(t)) for t in row[::-1]] for row in out]
                ops = _operands(_LHS, 4, lambda r, s, _: hid[r][s])
                for i in range(49):
                    ha[i, c, pl.ds(lo, n), :] = ops(i)
                lo += n

    for c in range(n_chunks):
        wd_copy(c).wait()
    wo_copy.wait()

    @pl.loop(0, n_out)
    def _(t):
        pos = pl.multiple_of(jnp.minimum(n_chunks * ATT3 + t * att4, half - att4), PACK)
        row0 = pl.multiple_of(t // 2 * OUT_TILE, OUT_TILE)
        matmul = _Matmuls((attend_jobs(pos, att4, False), [i for i in range(END4) if i % 7 in SLOT4]))
        with scope("S_p4"):
          if "4" in PH:
            rhs = _operands(_RHS, 4, lambda r, s, use: jnp.concatenate(
                [wbig[(t + 2 * use) % 2, c, pl.ds((3 - r) * LANES, LANES), pl.ds(s * LANES, LANES)]
                 for c in range(n_chunks)], axis=0))
            down = _strassen(2, lambda i: matmul(_load_rows(ha, (i,), [row0], OUT_TILE), rhs(i)))
            for r in range(4):
                for s in range(4):
                    gbuf[r, :, pl.ds(s * LANES, LANES)] = _silu(down[r][s])
            width = WO_WIDTH
            for col in range(0, qd, width):
                rhs = _operands(_RHS, 2, lambda r, s, _: wo[t % 2, pl.ds(r * hd, hd), pl.ds(s * qd + col, width)])
                lo = 0
                for n in WO_ROWS:
                    out = _strassen(1, lambda i: matmul(
                        _load_rows(xa1, (i,), [row0 + (u * quarter + lo) for u in range(2)], n), rhs(i)))
                    for r in range(2):
                        for s in range(2):
                            for u in range(2):
                                cols = pl.ds(s * qd + col, width)
                                res = (xbuf[t % 2, 2 * r + u, pl.ds(row0 + lo, n), cols].astype(F32)
                                       + out[r][s][u * n:(u + 1) * n] * gbuf[2 * r + u, pl.ds(lo, n), cols])
                                obuf[t, 2 * r + u, pl.ds(lo, n), cols] = res.astype(obuf.dtype)
                    lo += n
        if PH != "1234":
            t = t % 2
            z = (xa1[t, t, pl.ds(row0, 16), :] + xa2[t, t, pl.ds(row0, 16), :] + ha[t, t, pl.ds(row0, 16), :]
                 + (qk[t, t, pl.ds(row0, 16), :] + vbuf[t, pl.ds(row0, 16), :]).astype(BF16)
                 + wbig[t, t, pl.ds(row0, 16), :128] + wa[t, t, :16, :])
            obuf[0, 0, :16, :128] = z
        out_copy(t).start()

    for t in range(n_out):
        with scope("S_outwait"):
            out_copy(t).wait()


@jax.jit
def pallas_recurrent_scan__sliding_local_dilated__geglu_ffn__prompt_kernel(
    A_x: jax.Array,
    A_wqkv: jax.Array,
    A_wo: jax.Array,
    B_x: jax.Array,
    B_w_gate: jax.Array,
    B_w_up: jax.Array,
    B_w_down: jax.Array,
):
    del B_x
    b, s, d = A_x.shape
    f = B_w_gate.shape[1]
    quarter, n_chunks = s // 4, f // FCHUNK

    hbm = pl.BlockSpec(memory_space=pl.ANY)
    out = pl.pallas_call(
        _kernel,
        out_shape=jax.ShapeDtypeStruct((4, quarter, d), A_x.dtype),
        in_specs=[hbm] * 6,
        out_specs=hbm,
        scratch_shapes=[
            pltpu.VMEM((2, 4, quarter, d // 2), BF16),
            pltpu.VMEM((2, n_chunks, FCHUNK, d // 2), BF16),
            pltpu.VMEM((2, d, d // 2), BF16),
            pltpu.VMEM((7, d // 2 // LANES, s // 2, LANES), BF16),
            pltpu.VMEM((49, d // 4 // LANES, quarter, LANES), BF16),
            pltpu.VMEM((3, 2, d, FCHUNK), BF16),
            pltpu.VMEM((49, 2, d // 4, LANES), BF16),
            pltpu.VMEM((49, n_chunks, quarter, LANES), BF16),
            pltpu.VMEM((2, d // LANES, HALO + s, LANES), F32),
            pltpu.VMEM((d // LANES, HALO + s, LANES), F32),
            pltpu.VMEM((4, OUT_TILE, d // 2), F32),
            pltpu.VMEM((2 * quarter // OUT_TILE, 4, OUT_TILE, d // 2), BF16),
            pltpu.SemaphoreType.DMA((quarter // NORM_TILE,)),
            pltpu.SemaphoreType.DMA((n_chunks,)),
            pltpu.SemaphoreType.DMA((3,)),
            pltpu.SemaphoreType.DMA(()),
            pltpu.SemaphoreType.DMA((2 * quarter // OUT_TILE,)),
        ],
        compiler_params=pltpu.CompilerParams(vmem_limit_bytes=127 * 1024 * 1024, flags=FLAGS),
        name="fused_local_attn_geglu",
    )(A_x.reshape(4, quarter, d), A_wqkv.reshape(2, d // 2, 3 * d), A_wo, B_w_gate, B_w_up, B_w_down)
    return out.reshape(b, s, d)
```

```python
import functools

import jax
import jax.numpy as jnp
import numpy as np
from jax import lax
import jax.experimental.pallas as pl
import jax.experimental.pallas.tpu as pltpu

F32 = jnp.float32
BF16 = jnp.bfloat16
U32 = jnp.uint32

N_HEADS = 32
WINDOW = 8
DILATION = 2
LN_EPS = 1e-5
MASKED_LOGIT = -1e9

LANES = 128
SUB = 8
PACK = 16
HALO = 16
FCHUNK = 512
TILE = 128
PLAIN = 2


STRASSEN_LEFT = ("c+d", "d", "a+b", "a", "t", "c-a", "b-d")
STRASSEN_RIGHT = ("a", "c-a", "d", "b-d", "t", "a+b", "c+d")


def _strassen(m):
    m0, m1 = m(0), m(1)
    c = lax.add(m0, m1)
    m2, m3 = m(2), m(3)
    b = lax.add(m2, m3)
    m4 = m(4)
    d = lax.add(lax.add(m4, lax.sub(m3, m0)), m(5))
    a = lax.add(lax.add(m4, lax.sub(m1, m2)), m(6))
    return a, b, c, d


BALANCED_LEFT = ("a-b", "a+b", "t+t", "d-b", "d+b", "t-s", "t+s")
BALANCED_RIGHT = ("d-b", "d+b", "t", "t+s", "t-s", "a+b", "a-b")
LEFT_FAMILIES = ((0, 1), (2, 5, 6), (3, 4))
LEFT_ORDER = sum(LEFT_FAMILIES, ())
RIGHT_FAMILIES = ((0, 1), (2, 3, 4), (5, 6))
DELTA = (1.0, 3.0 ** 0.5, 3.0 ** 0.5, 3.0)


def _balanced(m):
    m0, m1 = m(0), m(1)
    b = lax.sub(m1, m0)
    diag = lax.sub(m(2), lax.add(m0, m1))
    m3, m4 = m(3), m(4)
    a = lax.sub(diag, lax.add(m3, m4))
    low = lax.add(b, lax.sub(m3, m4))
    m5, m6 = m(5), m(6)
    return a, b, lax.add(low, lax.sub(m6, m5)), lax.sub(diag, lax.add(m5, m6))


def _unscale(r, c):
    return DELTA[c] / DELTA[r] / 4


def _position(outer, inner):
    return outer // 2 * 2 + inner // 2, outer % 2 * 2 + inner % 2


def _combinations(quadrant):
    @functools.cache
    def term(name):
        if len(name) == 3:
            return (lax.add if name[1] == "+" else lax.sub)(term(name[0]), term(name[2]))
        if name in "ts":
            return term("a+d" if name == "t" else "b+c")
        return quadrant("abcd".index(name))

    return term


def _operands(side, family, block):
    outer = _combinations(lambda i: _stack([block(*_position(i, j)) for j in range(4)]))
    parts = _stack([outer(side[i]) for i in family])
    inner = _combinations(lambda j: lax.index_in_dim(parts, j, 1, keepdims=False))
    return lambda j: inner(side[j])


class _Matmuls:
    def __init__(self, *plan):
        self.calls = 0
        self.jobs = sorted(
            ((first + (last - first) * (i + 0.618 * n % 1) / len(jobs), n, job)
             for n, (jobs, first, last) in enumerate(plan) for i, job in enumerate(jobs)),
            key=lambda t: t[:2], reverse=True)

    def __call__(self, lhs, rhs):
        value = lax.dot_general(lhs, rhs, (((1,), (0,)), ((), ())), preferred_element_type=F32)
        while self.jobs and self.jobs[-1][0] < self.calls + 1:
            when, _, job = self.jobs.pop()
            row = int((when - self.calls) * (value.shape[0] // SUB)) * SUB
            job(lax.slice(value, (row, 0), (row + SUB, LANES)))
        self.calls += 1
        return value


def _jobs(fn, args):
    return [functools.partial(fn, *a) for a in args]


def _times(x, c):
    return x if c == 1.0 else lax.mul(x, np.float32(c))


def _plus(x, c):
    return lax.add(x, np.float32(c))


def _stack(xs):
    return lax.reshape(lax.concatenate(xs, 0), (len(xs), *xs[0].shape))


def _unstack(x):
    return [lax.index_in_dim(x, i, 0, keepdims=False) for i in range(x.shape[0])]


def _rows(x, lo, n):
    return lax.slice_in_dim(x, lo, lo + n, axis=0)


def _lane_groups(x):
    return [lax.slice_in_dim(x, j, j + LANES, axis=1) for j in range(0, x.shape[1], LANES)]


def _bf16(x):
    return lax.convert_element_type(x, BF16)


def _unpack(words):
    return lax.convert_element_type(pltpu.bitcast(words, BF16), F32)


def _geglu(g, u, scale):
    k0 = (2 / np.pi) ** 0.5
    t = lax.tanh(lax.mul(g, _plus(_times(lax.mul(g, g), k0 * 0.044715 * scale ** 3), k0 * scale)))
    return lax.mul(lax.mul(_times(g, 0.5 * scale ** 2), u), _plus(t, 1.0))


def _silu(x, scale):
    h = _times(x, 0.5)
    return lax.mul(_times(h, scale), _plus(lax.tanh(h), 1.0))


def _load(ref, index, lo, n):
    lo = lo // 2 if isinstance(lo, int) else pl.multiple_of(lo // 2, SUB)
    words = ref.bitcast(U32)[(*index, pl.ds(lo, n // 2), slice(None))]
    return lax.concatenate(_unstack(pltpu.bitcast(words, BF16)), 1)


class _ColumnCopy:
    def __init__(self, src, col, dst, sem):
        self.src, self.col, self.dst, self.sem = src, col, dst, sem

    def start(self):
        for g in range(self.dst.shape[0]):
            cols = pl.ds(self.col + g * LANES, LANES)
            pltpu.make_async_copy(self.src.at[:, cols], self.dst.at[g], self.sem).start()

    def wait(self):
        pltpu.make_async_copy(self.dst, self.dst, self.sem).wait()


def _start(*copies):
    for cp in copies:
        cp.start()


def _wait(*copies):
    for cp in copies:
        cp.wait()


def _kernel(x_hbm, wqkv_hbm, wo_hbm, wg_hbm, wu_hbm, wd_hbm, out_hbm,
            xbuf,
            wd,
            ring,
            xa,
            wa,
            wb,
            ha,
            mbuf,
            qkv,
            gbuf,
            x_sem, wd_sem, ring_sem, out_sem):
    _, quarter, d = x_hbm.shape
    n_chunks, n_tiles = ha.shape[2], quarter // TILE
    hd, qd, groups = d // 2, d // 4, d // LANES
    q_slot, k_slot, v_slot, o_slot = n_chunks % 3, None, 1, (n_chunks + 1) % 3

    def weight_words(slot):
        return (wd.bitcast(U32), ()) if slot is None else (ring.bitcast(U32), (slot,))

    def x_copies(t):
        at = [(slice(None), pl.ds(t * TILE, TILE), pl.ds(col, hd)) for col in (0, hd)]
        return [pltpu.make_async_copy(x_hbm.at[i], xbuf.at[i], x_sem.at[t]) for i in at]

    def ring_copy(slot, h, src=None, col=None):
        dst = ring.at[slot, pl.ds(h * (groups // 2), groups // 2)]
        return _ColumnCopy(src, col, dst, ring_sem.at[2 * slot + h])

    def wd_copy(h, src, col, row=0):
        dst = wd.at[pl.ds(h * (groups // 2), groups // 2), pl.ds(row, src.shape[0])]
        return _ColumnCopy(src, col, dst, wd_sem.at[h])

    def chunk_copies(c):
        col = c * FCHUNK if isinstance(c, int) else pl.multiple_of(c * FCHUNK, FCHUNK)
        return [ring_copy(c % 3, h, w, col) for h, w in enumerate((wg_hbm, wu_hbm))]

    def out_copies(t, h):
        return [pltpu.make_async_copy(
            ring.at[i, g, pl.ds(h * quarter + t * TILE, TILE)],
            out_hbm.at[2 * h + i, pl.ds(t * TILE, TILE), pl.ds(g * LANES, LANES)],
            out_sem.at[2 * t + h]) for i in range(2) for g in range(groups)]

    xs = [x_copies(t) for t in range(n_tiles)]
    wq = [wd_copy(h, wqkv_hbm, h * hd, d) for h in range(2)]
    wk = [wd_copy(h, wqkv_hbm, d + h * hd) for h in range(2)]
    wv = [ring_copy(v_slot, h, wqkv_hbm, 2 * d + h * hd) for h in range(2)]

    _start(*xs[0], wk[0])
    xs[0][0].wait()
    _start(*xs[1], wk[1])
    xs[0][1].wait()
    _start(*wv)

    never = jnp.abs(xbuf[0, :SUB, :LANES].astype(F32)) < 0
    zero = jnp.sum(jnp.where(never, 1, 0))
    lane = lax.broadcasted_iota(jnp.int32, (SUB, LANES), 1)
    lane_bit = {bit: (lane & bit) != 0 for bit in (1, 2, 4, 8, 16)}

    def after(token, x):
        if token is None:
            return x
        if x.dtype != token.dtype:
            token = pltpu.bitcast(token, x.dtype)
        n = x.shape[0] // SUB
        return lax.select(lax.concatenate([never] * n, 0), lax.concatenate([token] * n, 0), x)

    def swap_group_and_lane_bits(cols, bits=3):
        cols = list(cols)
        for gbit, lbit in ((1, 4), (2, 8), (4, 16))[:bits]:
            for i in range(len(cols)):
                if not i & gbit:
                    a, b = cols[i], cols[i | gbit]
                    cols[i] = lax.select(lane_bit[lbit], pltpu.roll(b, lbit, 1), a)
                    cols[i | gbit] = lax.select(lane_bit[lbit], b, pltpu.roll(a, LANES - lbit, 1))
        return cols

    def operand_jobs(side, family, load, dst, first, row0, positions):
        def job(g, lo, token):
            operand = _operands(side, family, lambda r, c: load(r, c, g, lo, token))
            for j in range(7):
                dst[pl.ds(first, len(family)), j, g, pl.ds(row0 + lo, PACK), :] = _bf16(operand(j))

        return _jobs(job, positions)

    def left_jobs(load, row0, rows):
        return [job for family in LEFT_FAMILIES for job in operand_jobs(
            BALANCED_LEFT, family, lambda r, c, g, lo, token: after(token, load(r, 2 * c + g, lo)),
            xa, LEFT_ORDER.index(family[0]), row0, [(g, lo) for lo in rows for g in range(2)])]

    def right_jobs(slot, family, dst=wa, heads=False):
        words, index = weight_words(slot)
        family = RIGHT_FAMILIES[family]

        def load(r, c, g, lo, token):
            def rows(at):
                return _unpack(after(token, words[(*index, 4 * g + c, pl.ds(at // 2, SUB))]))

            if heads:
                at = lo // PACK % 2 * hd + lo // (2 * PACK) * (2 * PACK) + r // 2 * PACK
                x = lax.concatenate([_rows(rows(at + i * qd), r % 2 * SUB, SUB) for i in range(2)], 0)
            else:
                x = rows(r * qd + lo)
            return _times(x, DELTA[r] / DELTA[c])

        return operand_jobs(BALANCED_RIGHT, family, load, dst, family[0] if dst is wa else 0, 0,
                            [(g, lo) for lo in range(0, qd, PACK) for g in range(2)])

    def move(i, j, g, lo, token):
        rows = pl.ds(lo, 4 * SUB)
        wa.bitcast(U32)[2 + i, j, g, rows, :] = after(token, wb.bitcast(U32)[i, j, g, rows, :])

    moves = _jobs(move, [(i, j, g, lo) for i in range(3) for j in range(7) for g in range(2)
                         for lo in range(0, qd // 2, 4 * SUB)])

    def refill_early(slot, last, **kw):
        return [(right_jobs(slot, 1, wb, **kw), max(last - 90, 23), last - 3),
                (right_jobs(slot, 0, **kw), last + 14.5, last + 47),
                (moves[:len(moves) // 2], last + 22, last + 47)]

    def refill_late(slot, **kw):
        return [(moves[len(moves) // 2:], 0, 22), (right_jobs(slot, 2, **kw), 0, 33.5)]

    def partial(slot, i, j, g, lo, n):
        if slot < 2:
            return mbuf, (slot, i, j, pl.ds(*g), pl.ds(lo, n))
        return gbuf, (1, j, pl.ds(i // 4 * 2 + g[0], g[1]), pl.ds(i % 4 * TILE + lo, n))

    def project(matmul, t, slot):
        for i in range(7):
            blocks = _balanced(lambda j: matmul(
                _load(xa, (LEFT_ORDER.index(i), j, slice(None)), t * TILE, TILE),
                _load(wa, (i, j, slice(None)), 0, qd)))
            for j, block in enumerate(blocks):
                ref, index = partial(slot, i, j, (0, 2), 0, TILE)
                ref[index] = _stack(_lane_groups(block))

    def finish_jobs(slot, n, use, quadrants=range(4)):
        def job(lo, j, g, token):
            def product(i):
                ref, index = partial(slot, i, j, g, lo, n)
                return after(None if i else token, lax.reshape(ref[index], (PACK, LANES)))

            out = _balanced(product)
            for i in quadrants:
                use(*_position(i, j), g[0], lo, out[i])

        return _jobs(job, [(lo, j, g) for lo in range(0, TILE, n) for j in range(4)
                           for g in (((0, 1), (1, 1)) if n == PACK else ((0, 2),))])

    def during(step):
        return 49 * step, 49 * step + 47

    def norm(q, lo, scaled, plain, token):
        def rows(lo):
            first, *rest = _lane_groups(lax.convert_element_type(xbuf[q, pl.ds(lo, SUB), :], F32))
            x = lax.concatenate([after(token, first)] + rest, 1)
            x = x - jnp.sum(x, axis=-1, keepdims=True) * (1.0 / d)
            inv = lax.rsqrt(jnp.sum(x * x, axis=-1, keepdims=True) * (1.0 / d) + LN_EPS)
            inv = lax.broadcast_in_dim(inv, (SUB, LANES), (0, 1))
            return [lax.mul(v, _times(inv, DELTA[q] / DELTA[g // 2] if scaled else 1.0))
                    for g, v in enumerate(_lane_groups(x))]

        if scaled:
            gbuf[:, :, q, pl.ds(lo, SUB), :] = lax.reshape(_stack(rows(lo)), (2, 4, SUB, LANES))
        if plain and lo % PACK:
            lo -= SUB
            cols = ([_times(gbuf[g // 4, g % 4, q, pl.ds(lo, PACK), :], DELTA[g // 2] / DELTA[q])
                     for g in range(groups)] if scaled else
                    [lax.concatenate(v, 0) for v in zip(rows(lo), rows(lo + SUB))])
            for g, v in enumerate(cols):
                ha[lo // TILE, g // 4, g % 4, pl.ds(q * TILE + lo % TILE, PACK), :] = _bf16(v)

    def norm_jobs(t, scaled=True, plain=False):
        return _jobs(norm, [(q, t * TILE + lo, scaled, plain)
                            for q in range(4) for lo in range(0, TILE, SUB)])

    def split_x_jobs(t):
        return left_jobs(lambda q, g, lo: gbuf[g // 4, g % 4, q, pl.ds(lo, PACK), :],
                         0, range(t * TILE, (t + 1) * TILE, PACK))

    def shuffle_weight_jobs(slot, row0=0):
        words, index = weight_words(slot)

        def job(lo, token):
            at = (*index, slice(None), pl.ds(lo // 2, SUB))
            words[at] = _stack(swap_group_and_lane_bits([after(token, v) for v in _unstack(words[at])]))

        return _jobs(job, [(row0 + lo + r * qd,) for lo in range(0, qd, PACK) for r in range(4)])

    def plain_k(t, gs, *plan):
        matmul = _Matmuls(*plan)
        for g in gs:
            k = lax.add(*[matmul(_load(ha, (t, h, pl.ds(0, 4)), 0, 4 * TILE),
                                 _load(wd, (pl.ds(g, 1),), h * hd, hd)) for h in range(2)])
            k = pltpu.bitcast(_bf16(k), F32)
            for lo in range(0, 4 * TILE, PACK):
                row = HALO + lo // TILE * quarter + t * TILE + lo % TILE
                qkv[1, g, pl.ds(row, SUB), :] = _rows(k, lo // 2, SUB)

    def shuffle_k(row, token):
        cols = [after(token, v) for v in _unstack(pltpu.bitcast(qkv[1, :, pl.ds(row, SUB), :], U32))]
        qkv[1, :, pl.ds(row, PACK), :] = _unpack(_stack(swap_group_and_lane_bits(cols)))

    def finish_qkv(p, t, slot):
        def use(r, c, _, lo, x):
            x = _times(x, _unscale(r, c))
            for g in range(2):
                qkv[p, 4 * g + c, pl.ds(HALO + r * quarter + t * TILE + lo, SUB), :] = _rows(x, g * SUB, SUB)

        return finish_jobs(slot, SUB, use)

    for job in norm_jobs(0, plain=True):
        job(None)
    wk[0].wait()
    _start(*xs[2], *xs[3])
    plain_k(0, range(4), (split_x_jobs(0), 0, 7))
    _wait(*xs[1], wk[1])
    _start(*wq, *chunk_copies(0))
    plain_k(0, range(4, 8), (norm_jobs(1, plain=True), 0, 6.5))
    _wait(*wv)
    plain_k(1, range(8), (shuffle_weight_jobs(v_slot), 0, 12.5),
            *[(right_jobs(v_slot, f), 2, 15.5) for f in range(3)])
    _start(*chunk_copies(1))
    _wait(*xs[2], *xs[3])
    matmul = _Matmuls((norm_jobs(2) + norm_jobs(3), 0, 44), (split_x_jobs(1)[:32], 0, 47))
    project(matmul, 0, 0)
    _wait(*wq)
    matmul = _Matmuls(
        (split_x_jobs(1)[32:], 0, 19), (split_x_jobs(2), *during(0)), (split_x_jobs(3), *during(1)),
        *[(finish_qkv(2, t, t % 2), *during(t)) for t in range(3)],
        (shuffle_weight_jobs(k_slot), 0, 96),
        (right_jobs(k_slot, 1, wb), 98, 119), (right_jobs(k_slot, 0), 119, 146),
        (moves[:len(moves) // 2], 121, 146))
    project(matmul, 1, 1)
    project(matmul, 2, 0)

    @pl.loop(0, 2)
    def _(h):
        ring_copy(0, h).wait()

    project(matmul, 3, 1)
    matmul = _Matmuls(
        *refill_late(k_slot), *refill_early(0, 49),
        (shuffle_weight_jobs(k_slot, d), 0, 92),
        (finish_qkv(2, 3, 1), *during(0)), (finish_qkv(1, 2, 0), *during(1)))
    project(matmul, 2, 0)
    project(matmul, 3, 2)

    def geglu_jobs(t):
        def use(r, c, _, lo, x):
            gbuf[0, c, r, pl.ds(t * TILE + lo, SUB), :] = _geglu(
                _rows(x, 0, SUB), _rows(x, SUB, SUB), _unscale(r, c))

        return finish_jobs(t % 2, SUB, use)

    def split_hidden_jobs(chunk, t):
        return [job for lo in range(t * TILE, (t + 1) * TILE, PACK)
                for family in ((0, 1), (2, 3), (4,), (5,), (6,)) for job in operand_jobs(
                    STRASSEN_LEFT, family,
                    lambda r, c, g, lo, token: after(token, gbuf[0, c, r, pl.ds(lo, PACK), :]),
                    ha, family[0], 0, [(chunk, lo)])]

    @pl.loop(0, n_chunks)
    def _(c):
        _wait(*[ring_copy((c + 1) % 3, h) for h in range(2)])
        pl.when(c + 2 < n_chunks)(lambda: _start(*chunk_copies(c + 2)))
        pl.when(c + 2 == n_chunks)(lambda: _start(*[pltpu.make_async_copy(
            wq[h].dst, ring_copy(q_slot, h).dst, ring_copy(q_slot, h).sem) for h in range(2)]))
        pl.when(c + 1 == n_chunks)(
            lambda: _start(*[ring_copy(o_slot, h, wo_hbm, h * hd) for h in range(2)]))
        previous = jnp.maximum(c - 1, 0)
        matmul = _Matmuls(
            *refill_late(c % 3), *refill_early((c + 1) % 3, 147),
            *[(geglu_jobs((t - 1) % n_tiles), *during(t)) for t in range(n_tiles)],
            (split_hidden_jobs(previous, 2), 30, 60), (split_hidden_jobs(previous, 3), 60, 98),
            (split_hidden_jobs(c, 0), 98, 145), (split_hidden_jobs(c, 1), 145, 163))
        for t in range(n_tiles):
            project(matmul, t, t % 2)

    @pl.loop(0, 2)
    def _(h):
        ring_copy(o_slot, h).wait()
        wd_copy(h, wd_hbm, pl.multiple_of(h * hd, hd)).start()

    matmul = _Matmuls(
        *refill_late(q_slot), *refill_early(o_slot, 147, heads=True),
        (split_hidden_jobs(n_chunks - 1, 2), 30, 60), (split_hidden_jobs(n_chunks - 1, 3), 60, 98),
        (finish_qkv(1, 3, 2), 49, 147),
        (_jobs(shuffle_k, [(HALO + q * quarter + lo,) for lo in range(0, PLAIN * TILE, PACK)
                           for q in range(4)]), 35, 180),
        (geglu_jobs(n_tiles - 1), *during(0)),
        *[(finish_qkv(0, t, t % 2), *during(t + 1)) for t in range(n_tiles - 1)])
    for t in range(n_tiles):
        project(matmul, t, t % 2)
    for job in finish_qkv(0, n_tiles - 1, 1):
        job(None)

    for p in (1, 2):
        for g in range(groups):
            qkv[p, g, pl.ds(0, HALO), :] = jnp.broadcast_to(qkv[p, g, pl.ds(HALO, 1), :], (HALO, LANES))

    scale = float(d // N_HEADS) ** -0.5

    def attend(row0, q, lo, token):
        off = q * quarter + lo

        def load(p, w):
            return qkv[p, :, pl.ds(row0 + (HALO + off - DILATION * w), SUB), :]

        first, *rest = _unstack(load(0, 0))
        query = _stack([after(token, first)] + rest)
        logits = []
        for w in range(WINDOW):
            s = lax.reduce_sum(lax.mul(query, load(1, w)), (0,))
            for bit in (1, 2):
                other = lax.select(lane_bit[bit], pltpu.roll(s, bit, 1), pltpu.roll(s, LANES - bit, 1))
                s = lax.add(s, other)
            if off < DILATION * w:
                row = row0 + off + lax.broadcasted_iota(jnp.int32, (SUB, LANES), 0)
                s = jnp.where(row >= DILATION * w, s, MASKED_LOGIT / scale)
            logits.append(s)
        top = functools.reduce(lax.max, logits)
        weights = [lax.exp2(_times(lax.sub(s, top), scale * np.log2(np.e))) for s in logits]
        inv = lax.div(np.float32(1), functools.reduce(lax.add, weights))
        out = functools.reduce(lax.add, [
            lax.mul(lax.broadcast(weights[w], (groups,)), load(2, w)) for w in range(WINDOW)])
        out = [lax.mul(v, _times(inv, DELTA[q] / DELTA[g // 2])) for g, v in enumerate(_unstack(out))]
        mbuf[1, q, :, :, pl.ds(lo, SUB), :] = lax.reshape(
            _stack(swap_group_and_lane_bits(out, 1)), (4, 2, SUB, LANES))

    _wait(*[wd_copy(h, wd_hbm, h * hd) for h in range(2)])

    @pl.loop(0, n_tiles)
    def _(step):
        row0 = pl.multiple_of(step * TILE, TILE)
        plan = []
        for lo in range(0, TILE, PACK):
            first, last = 43 * lo / TILE, 43 * (lo + PACK) / TILE
            plan += [
                (_jobs(attend, [(row0, q, lo + i) for q in range(4) for i in (0, SUB)]), first, last),
                (left_jobs(lambda q, g, lo: mbuf[1, q, g // 2, g % 2, pl.ds(lo, PACK), :],
                           row0, [lo]), last + 1, last + 5)]
        matmul = _Matmuls(*plan)
        row0 = pl.multiple_of(step // 2 * (2 * TILE), 2 * TILE)
        for i in range(7):
            half = (step + 2 * i) % 2
            right = _operands(STRASSEN_RIGHT, [i], lambda r, c: lax.concatenate(
                [_unpack(wd.bitcast(U32)[4 * half + c, pl.ds((n * FCHUNK + r * LANES) // 2, LANES // 2), :])
                 for n in range(n_chunks)], 0))
            blocks = _strassen(lambda j: matmul(
                _load(ha, (i, j, slice(None)), row0, 2 * TILE), _bf16(_unstack(right(j))[0])))
            for j, block in enumerate(blocks):
                mbuf[0, i, j] = lax.reshape(block, (2, TILE, LANES))
        for j in range(4):
            blocks = _strassen(lambda i: lax.reshape(mbuf[0, i, j], (2 * TILE, LANES)))
            for i, block in enumerate(blocks):
                r, c = _position(i, j)
                gbuf[step % 2, c, r, pl.ds(row0, 2 * TILE), :] = _silu(block, _unscale(r, c))

    def output_jobs(t, quadrants=range(4)):
        def use(r, c, g, lo, attn):
            rows = pl.ds(t * TILE + lo, PACK)
            x = lax.convert_element_type(xbuf[r, rows, pl.ds(g * hd + c * LANES, LANES)], F32)
            slot = r % 2 + (zero if lo == g == r % 2 == c % 2 == 0 else 0)
            ring[slot, 4 * g + c, pl.ds(r // 2 * quarter + t * TILE + lo, PACK), :] = (
                _bf16(lax.add(x, lax.mul(attn, gbuf[g, c, r, rows, :]))))

        def send(token):
            _start(*[cp for h in range(2) if 3 * h in quadrants for cp in out_copies(t, h)])

        return finish_jobs(1 - t % 2, PACK, use, quadrants) + [send]

    matmul = _Matmuls(
        *refill_late(o_slot, heads=True),
        (output_jobs(0), *during(1)), (output_jobs(1), *during(2)),
        (output_jobs(2), 147, 176), (output_jobs(3, [1]), 176, 182), (output_jobs(3, [0]), 182, 188))
    for t in range(n_tiles):
        project(matmul, t, 1 - t % 2)
    for job in output_jobs(3, [2, 3]):
        job(None)
    _wait(*[cp for t in range(n_tiles) for h in range(2) for cp in out_copies(t, h)])


@jax.jit
def pallas_recurrent_scan__sliding_local_dilated__geglu_ffn__prompt_kernel(
    A_x: jax.Array,
    A_wqkv: jax.Array,
    A_wo: jax.Array,
    B_x: jax.Array,
    B_w_gate: jax.Array,
    B_w_up: jax.Array,
    B_w_down: jax.Array,
):
    del B_x
    b, s, d = A_x.shape
    f = B_w_gate.shape[1]
    assert (b, s, d, f) == (1, 16 * TILE, 8 * LANES, 7 * FCHUNK) and A_x.dtype == BF16
    quarter, groups = s // 4, d // LANES

    hbm = pl.BlockSpec(memory_space=pl.ANY)
    out = pl.pallas_call(
        _kernel,
        out_shape=jax.ShapeDtypeStruct((4, quarter, d), BF16),
        in_specs=[hbm] * 6,
        out_specs=hbm,
        scratch_shapes=[
            pltpu.VMEM((4, quarter, d), BF16),
            pltpu.VMEM((groups, f, LANES), BF16),
            pltpu.VMEM((3, groups, d, LANES), BF16),
            pltpu.VMEM((7, 7, 2, quarter, LANES), BF16),
            pltpu.VMEM((7, 7, 2, d // 4, LANES), BF16),
            pltpu.VMEM((3, 7, 2, d // 4, LANES), BF16),
            pltpu.VMEM((7, 7, f // FCHUNK, quarter, LANES), BF16),
            pltpu.VMEM((2, 7, 4, 2, TILE, LANES), F32),
            pltpu.VMEM((3, groups, HALO + s, LANES), F32),
            pltpu.VMEM((2, 4, 4, quarter, LANES), F32),
            pltpu.SemaphoreType.DMA((4,)),
            pltpu.SemaphoreType.DMA((2,)),
            pltpu.SemaphoreType.DMA((6,)),
            pltpu.SemaphoreType.DMA((8,)),
        ],
        compiler_params=pltpu.CompilerParams(
            vmem_limit_bytes=127 * 1024 * 1024, disable_bounds_checks=True),
        name="fused_local_attn_geglu",
    )(A_x.reshape(4, quarter, d), A_wqkv, A_wo, B_w_gate, B_w_up, B_w_down)
    return out.reshape(b, s, d)
```

```python
import functools

import jax
import jax.numpy as jnp
import numpy as np
from jax import lax
import jax.experimental.pallas as pl
import jax.experimental.pallas.tpu as pltpu

F32 = jnp.float32
BF16 = jnp.bfloat16
U32 = jnp.uint32

N_HEADS = 32
WINDOW = 8
DILATION = 2
LN_EPS = 1e-5
MASKED_LOGIT = -1e9

LANES = 128
SUB = 8
PACK = 16
HALO = 16
FCHUNK = 512
TILE = 128
ROOM = [a * b for a in (1, 1, 1, 1, 1, 1, 1) for b in (.5, 1, 1, 1, 1, 1, 1)]
PLAIN = 2


STRASSEN_LEFT = ("c+d", "d", "a+b", "a", "t", "c-a", "b-d")
STRASSEN_RIGHT = ("a", "c-a", "d", "b-d", "t", "a+b", "c+d")


def _strassen(m):
    m0, m1 = m(0), m(1)
    c = lax.add(m0, m1)
    m2, m3 = m(2), m(3)
    b = lax.add(m2, m3)
    m4 = m(4)
    d = lax.add(lax.add(m4, lax.sub(m3, m0)), m(5))
    a = lax.add(lax.add(m4, lax.sub(m1, m2)), m(6))
    return a, b, c, d


BALANCED_LEFT = ("a-b", "a+b", "t+t", "d-b", "d+b", "t-s", "t+s")
BALANCED_RIGHT = ("d-b", "d+b", "t", "t+s", "t-s", "a+b", "a-b")
LEFT_FAMILIES = ((0, 1), (2, 5, 6), (3, 4))
LEFT_ORDER = sum(LEFT_FAMILIES, ())
RIGHT_FAMILIES = ((0, 1), (2, 3, 4), (5, 6))
DELTA = (1.0, 3.0 ** 0.5, 3.0 ** 0.5, 3.0)


def _balanced(m):
    m0, m1 = m(0), m(1)
    b = lax.sub(m1, m0)
    diag = lax.sub(m(2), lax.add(m0, m1))
    m3, m4 = m(3), m(4)
    a = lax.sub(diag, lax.add(m3, m4))
    low = lax.add(b, lax.sub(m3, m4))
    m5, m6 = m(5), m(6)
    return a, b, lax.add(low, lax.sub(m6, m5)), lax.sub(diag, lax.add(m5, m6))


def _unscale(r, c):
    return DELTA[c] / DELTA[r] / 4


def _position(outer, inner):
    return outer // 2 * 2 + inner // 2, outer % 2 * 2 + inner % 2


def _combinations(quadrant):
    @functools.cache
    def term(name):
        if len(name) == 3:
            return (lax.add if name[1] == "+" else lax.sub)(term(name[0]), term(name[2]))
        if name in "ts":
            return term("a+d" if name == "t" else "b+c")
        return quadrant("abcd".index(name))

    return term


def _operands(side, family, block):
    outer = _combinations(lambda i: _stack([block(*_position(i, j)) for j in range(4)]))
    parts = _stack([outer(side[i]) for i in family])
    inner = _combinations(lambda j: lax.index_in_dim(parts, j, 1, keepdims=False))
    return lambda j: inner(side[j])


class _Matmuls:
    def __init__(self, *plan, warp=None):
        self.calls = 0
        warp = warp or (lambda t: t)
        self.jobs = sorted(
            ((warp(first + (last - first) * (i + 0.618 * n % 1) / len(jobs)), n, job)
             for n, (jobs, first, last) in enumerate(plan) for i, job in enumerate(jobs)),
            key=lambda t: t[:2], reverse=True)

    def __call__(self, lhs, rhs):
        value = lax.dot_general(lhs, rhs, (((1,), (0,)), ((), ())), preferred_element_type=F32)
        while self.jobs and self.jobs[-1][0] < self.calls + 1:
            when, _, job = self.jobs.pop()
            row = int((when - self.calls) * (value.shape[0] // SUB)) * SUB
            job(lax.slice(value, (row, 0), (row + SUB, LANES)))
        self.calls += 1
        return value


def _jobs(fn, args):
    return [functools.partial(fn, *a) for a in args]


def _times(x, c):
    return x if c == 1.0 else lax.mul(x, np.float32(c))


def _plus(x, c):
    return lax.add(x, np.float32(c))


def _aligned(i, n):
    return i if isinstance(i, int) else pl.multiple_of(i, n)


def _stack(xs):
    return lax.reshape(lax.concatenate(xs, 0), (len(xs), *xs[0].shape))


def _unstack(x):
    return [lax.index_in_dim(x, i, 0, keepdims=False) for i in range(x.shape[0])]


def _rows(x, lo, n):
    return lax.slice_in_dim(x, lo, lo + n, axis=0)


def _lane_groups(x):
    return [lax.slice_in_dim(x, j, j + LANES, axis=1) for j in range(0, x.shape[1], LANES)]


def _bf16(x):
    return lax.convert_element_type(x, BF16)


def _unpack(words):
    return lax.convert_element_type(pltpu.bitcast(words, BF16), F32)


def _geglu(g, u, scale):
    k0 = (2 / np.pi) ** 0.5
    t = lax.tanh(lax.mul(g, _plus(_times(lax.mul(g, g), k0 * 0.044715 * scale ** 3), k0 * scale)))
    return lax.mul(lax.mul(_times(g, 0.5 * scale ** 2), u), _plus(t, 1.0))


def _silu(x, scale):
    h = _times(x, 0.5)
    return lax.mul(_times(h, scale), _plus(lax.tanh(h), 1.0))


def _load(ref, index, lo, n):
    words = ref.bitcast(U32)[(*index, pl.ds(_aligned(lo // 2, SUB), n // 2))]
    return lax.concatenate(_unstack(pltpu.bitcast(words, BF16)), 1)


class _ColumnCopy:
    def __init__(self, src, col, dst, sem):
        self.src, self.col, self.dst, self.sem = src, col, dst, sem

    def start(self):
        for g in range(self.dst.shape[0]):
            cols = pl.ds(self.col + g * LANES, LANES)
            pltpu.make_async_copy(self.src.at[:, cols], self.dst.at[g], self.sem).start()

    def wait(self):
        pltpu.make_async_copy(self.dst, self.dst, self.sem).wait()


def _start(*copies):
    for cp in copies:
        cp.start()


def _wait(*copies):
    for cp in copies:
        cp.wait()


def _kernel(x_hbm, wqkv_hbm, wo_hbm, wg_hbm, wu_hbm, wd_hbm, out_hbm,
            xbuf,
            wbuf,
            xa,
            wa,
            wb,
            ha,
            mbuf,
            qkv,
            gbuf,
            x_sem, w_sem, out_sem):
    _, quarter, d = x_hbm.shape
    n_chunks, n_tiles = ha.shape[2], quarter // TILE
    hd, qd, groups = d // 2, d // 4, d // LANES

    def chunk_slot(c):
        return 1 + (c + 2) % 3

    q_slot, k_slot, v_slot, o_slot, down_slot = 0, 4, chunk_slot(1), chunk_slot(n_chunks), 2

    def x_copies(t):
        at = [(slice(None), pl.ds(t * TILE, TILE), pl.ds(col, hd)) for col in (0, hd)]
        return [pltpu.make_async_copy(x_hbm.at[i], xbuf.at[i], x_sem.at[t]) for i in at]

    def w_copy(slot, h, src=None, col=None):
        rows = pl.ds(_aligned(slot * d, d), d if src is None else src.shape[0])
        dst = wbuf.at[pl.ds(h * (groups // 2), groups // 2), rows]
        return _ColumnCopy(src, col, dst, w_sem.at[2 * slot + h])

    def chunk_copies(c):
        return [w_copy(chunk_slot(c), h, w, _aligned(c * FCHUNK, FCHUNK)) for h, w in enumerate((wg_hbm, wu_hbm))]

    def out_copies(t, h):
        return [pltpu.make_async_copy(
            wbuf.at[g, pl.ds((down_slot + i) * d + h * quarter + t * TILE, TILE)],
            out_hbm.at[2 * h + i, pl.ds(t * TILE, TILE), pl.ds(g * LANES, LANES)],
            out_sem.at[2 * t + h]) for i in range(2) for g in range(groups)]

    xs = [x_copies(t) for t in range(n_tiles)]
    wq = [w_copy(q_slot, h, wqkv_hbm, h * hd) for h in range(2)]
    wk = [w_copy(k_slot, h, wqkv_hbm, d + h * hd) for h in range(2)]
    wv = [w_copy(v_slot, h, wqkv_hbm, 2 * d + h * hd) for h in range(2)]

    _start(*xs[0], wk[0])
    xs[0][0].wait()
    _start(*xs[1], wk[1])
    xs[0][1].wait()
    _start(*wv)

    never = jnp.abs(xbuf[0, :SUB, :LANES].astype(F32)) < 0
    zero = jnp.sum(jnp.where(never, 1, 0))
    lane = lax.broadcasted_iota(jnp.int32, (SUB, LANES), 1)
    lane_bit = {bit: (lane & bit) != 0 for bit in (1, 2, 4, 8, 16)}

    def after(token, x):
        if token is None:
            return x
        if x.dtype != token.dtype:
            token = pltpu.bitcast(token, x.dtype)
        n = x.shape[0] // SUB
        return lax.select(lax.concatenate([never] * n, 0), lax.concatenate([token] * n, 0), x)

    def swap_group_and_lane_bits(cols, bits=3):
        cols = list(cols)
        for gbit, lbit in ((1, 4), (2, 8), (4, 16))[:bits]:
            for i in range(len(cols)):
                if not i & gbit:
                    a, b = cols[i], cols[i | gbit]
                    cols[i] = lax.select(lane_bit[lbit], pltpu.roll(b, lbit, 1), a)
                    cols[i | gbit] = lax.select(lane_bit[lbit], b, pltpu.roll(a, LANES - lbit, 1))
        return cols

    def operand_jobs(side, family, load, dst, first, row0, positions):
        def job(g, lo, token):
            operand = _operands(side, family, lambda r, c: load(r, c, g, lo, token))
            for j in range(7):
                dst[pl.ds(first, len(family)), j, g, pl.ds(row0 + lo, PACK), :] = _bf16(operand(j))

        return _jobs(job, positions)

    def left_jobs(load, row0, rows):
        return [job for family in LEFT_FAMILIES for job in operand_jobs(
            BALANCED_LEFT, family, lambda r, c, g, lo, token: after(token, load(r, 2 * c + g, lo)),
            xa, LEFT_ORDER.index(family[0]), row0, [(g, lo) for lo in rows for g in range(2)])]

    def right_jobs(slot, family, dst=wa, heads=False):
        word0 = _aligned(slot * hd, hd)
        family = RIGHT_FAMILIES[family]

        def load(r, c, g, lo, token):
            def rows(at):
                return _unpack(after(token, wbuf.bitcast(U32)[4 * g + c, pl.ds(word0 + at // 2, SUB)]))

            if heads:
                at = lo // PACK % 2 * hd + lo // (2 * PACK) * (2 * PACK) + r // 2 * PACK
                x = lax.concatenate([_rows(rows(at + i * qd), r % 2 * SUB, SUB) for i in range(2)], 0)
            else:
                x = rows(r * qd + lo)
            return _times(x, DELTA[r] / DELTA[c])

        return operand_jobs(BALANCED_RIGHT, family, load, dst, family[0] if dst is wa else 0, 0,
                            [(g, lo) for lo in range(0, qd, PACK) for g in range(2)])

    def move(i, j, g, lo, token):
        rows = pl.ds(lo, 4 * SUB)
        wa.bitcast(U32)[2 + i, j, g, rows, :] = after(token, wb.bitcast(U32)[i, j, g, rows, :])

    moves = _jobs(move, [(i, j, g, lo) for i in range(3) for j in range(7) for g in range(2)
                         for lo in range(0, qd // 2, 4 * SUB)])

    def refill_early(slot, last, **kw):
        return [(right_jobs(slot, 1, wb, **kw), max(last - 90, 23), max(last - 3, 62)),
                (right_jobs(slot, 0, **kw), last + 14.5, last + 47),
                (moves[:len(moves) // 2], last + 22, last + 47)]

    def refill_late(slot, **kw):
        return [(moves[len(moves) // 2:], 0, 22), (right_jobs(slot, 2, **kw), 0, 33.5)]

    def partial(slot, i, j, g, lo, n):
        if slot < 2:
            return mbuf, (slot, i, j, pl.ds(*g), pl.ds(lo, n))
        return gbuf, (1, j, pl.ds(i // 4 * 2 + g[0], g[1]), pl.ds(i % 4 * TILE + lo, n))

    def project(matmul, t, slot):
        for i in range(7):
            blocks = _balanced(lambda j: matmul(
                _load(xa, (LEFT_ORDER.index(i), j, slice(None)), t * TILE, TILE),
                _load(wa, (i, j, slice(None)), 0, qd)))
            for j, block in enumerate(blocks):
                ref, index = partial(slot, i, j, (0, 2), 0, TILE)
                ref[index] = _stack(_lane_groups(block))

    def finish_jobs(slot, n, use, quadrants=range(4)):
        def job(lo, j, g, token):
            def product(i):
                ref, index = partial(slot, i, j, g, lo, n)
                return after(None if i else token, lax.reshape(ref[index], (PACK, LANES)))

            out = _balanced(product)
            for i in quadrants:
                use(*_position(i, j), g[0], lo, out[i])

        return _jobs(job, [(lo, j, g) for lo in range(0, TILE, n) for j in range(4)
                           for g in (((0, 1), (1, 1)) if n == PACK else ((0, 2),))])

    def during(step):
        return 49 * step, 49 * step + 47

    def norm(q, lo, scaled, plain, token):
        def rows(lo):
            first, *rest = _lane_groups(lax.convert_element_type(xbuf[q, pl.ds(lo, SUB), :], F32))
            x = lax.concatenate([after(token, first)] + rest, 1)
            x = x - jnp.sum(x, axis=-1, keepdims=True) * (1.0 / d)
            inv = lax.rsqrt(jnp.sum(x * x, axis=-1, keepdims=True) * (1.0 / d) + LN_EPS)
            inv = lax.broadcast_in_dim(inv, (SUB, LANES), (0, 1))
            return [lax.mul(v, _times(inv, DELTA[q] / DELTA[g // 2] if scaled else 1.0))
                    for g, v in enumerate(_lane_groups(x))]

        if scaled:
            gbuf[:, :, q, pl.ds(lo, SUB), :] = lax.reshape(_stack(rows(lo)), (2, 4, SUB, LANES))
        if plain and lo % PACK:
            lo -= SUB
            cols = ([_times(gbuf[g // 4, g % 4, q, pl.ds(lo, PACK), :], DELTA[g // 2] / DELTA[q])
                     for g in range(groups)] if scaled else
                    [lax.concatenate(v, 0) for v in zip(rows(lo), rows(lo + SUB))])
            for g, v in enumerate(cols):
                ha[lo // TILE, g // 4, g % 4, pl.ds(q * TILE + lo % TILE, PACK), :] = _bf16(v)

    def norm_jobs(t, scaled=True, plain=False):
        return _jobs(norm, [(q, t * TILE + lo, scaled, plain)
                            for q in range(4) for lo in range(0, TILE, SUB)])

    def split_x_jobs(t):
        return left_jobs(lambda q, g, lo: gbuf[g // 4, g % 4, q, pl.ds(lo, PACK), :],
                         0, range(t * TILE, (t + 1) * TILE, PACK))

    def shuffle_weight_jobs(slot):
        words = wbuf.bitcast(U32)

        def job(lo, token):
            at = (slice(None), pl.ds(lo // 2, SUB))
            words[at] = _stack(swap_group_and_lane_bits([after(token, v) for v in _unstack(words[at])]))

        return _jobs(job, [(slot * d + lo + r * qd,) for lo in range(0, qd, PACK) for r in range(4)])

    def plain_k(t, gs, *plan):
        matmul = _Matmuls(*plan)
        for g in gs:
            k = lax.add(*[matmul(_load(ha, (t, h, pl.ds(0, 4)), 0, 4 * TILE),
                                 _load(wbuf, (pl.ds(g, 1),), k_slot * d + h * hd, hd)) for h in range(2)])
            k = pltpu.bitcast(_bf16(k), F32)
            for lo in range(0, 4 * TILE, PACK):
                row = HALO + lo // TILE * quarter + t * TILE + lo % TILE
                qkv[1, g, pl.ds(row, SUB), :] = _rows(k, lo // 2, SUB)

    def shuffle_k(row, token):
        cols = [after(token, v) for v in _unstack(pltpu.bitcast(qkv[1, :, pl.ds(row, SUB), :], U32))]
        qkv[1, :, pl.ds(row, PACK), :] = _unpack(_stack(swap_group_and_lane_bits(cols)))

    def finish_qkv(p, t, slot):
        def use(r, c, _, lo, x):
            x = _times(x, _unscale(r, c))
            for g in range(2):
                qkv[p, 4 * g + c, pl.ds(HALO + r * quarter + t * TILE + lo, SUB), :] = _rows(x, g * SUB, SUB)

        return finish_jobs(slot, SUB, use)

    for job in norm_jobs(0, plain=True):
        job(None)
    wk[0].wait()
    _start(*xs[2], *xs[3])
    plain_k(0, range(4), (split_x_jobs(0), 0, 7))
    _wait(*xs[1], wk[1])
    _start(*wq, *chunk_copies(0))
    plain_k(0, range(4, 8), (norm_jobs(1, plain=True), 0, 6.5))
    _wait(*wv)
    plain_k(1, range(8), (shuffle_weight_jobs(v_slot), 0, 13.5),
            *[(right_jobs(v_slot, f), 1.5, 15.5) for f in range(3)])
    _start(*chunk_copies(1))
    _wait(*xs[2], *xs[3])
    matmul = _Matmuls((norm_jobs(2) + norm_jobs(3), 0, 44), (split_x_jobs(1)[:32], 0, 47))
    project(matmul, 0, 0)
    _wait(*wq)
    matmul = _Matmuls(
        (split_x_jobs(1)[32:], 0, 19), (split_x_jobs(2), *during(0)), (split_x_jobs(3), *during(1)),
        *[(finish_qkv(2, t, t % 2), *during(t)) for t in range(3)],
        (shuffle_weight_jobs(k_slot), 0, 96),
        (right_jobs(k_slot, 1, wb), 98, 119), (right_jobs(k_slot, 0), 119, 146),
        (moves[:len(moves) // 2], 121, 146))
    project(matmul, 1, 1)
    project(matmul, 2, 0)

    @pl.loop(0, 2)
    def _(h):
        w_copy(chunk_slot(0), h).wait()

    project(matmul, 3, 1)
    matmul = _Matmuls(
        *refill_late(k_slot), *refill_early(chunk_slot(0), 49),
        (shuffle_weight_jobs(q_slot), 0, 92),
        (finish_qkv(2, 3, 1), *during(0)), (finish_qkv(1, 2, 0), *during(1)))
    project(matmul, 2, 0)
    project(matmul, 3, 2)

    def geglu_jobs(t):
        def use(r, c, _, lo, x):
            gbuf[0, c, r, pl.ds(t * TILE + lo, SUB), :] = _geglu(
                _rows(x, 0, SUB), _rows(x, SUB, SUB), _unscale(r, c))

        return finish_jobs(t % 2, SUB, use)

    def split_hidden_jobs(chunk, t):
        return [job for lo in range(t * TILE, (t + 1) * TILE, PACK)
                for family in ((0, 1), (2, 3), (4,), (5,), (6,)) for job in operand_jobs(
                    STRASSEN_LEFT, family,
                    lambda r, c, g, lo, token: after(token, gbuf[0, c, r, pl.ds(lo, PACK), :]),
                    ha, family[0], 0, [(chunk, lo)])]

    @pl.loop(0, n_chunks)
    def _(c):
        pl.when(c + 1 < n_chunks)(lambda: _wait(*chunk_copies(c + 1)))
        pl.when(c + 2 < n_chunks)(lambda: _start(*chunk_copies(c + 2)))
        pl.when(c + 2 == n_chunks)(
            lambda: _start(*[w_copy(o_slot, h, wo_hbm, h * hd) for h in range(2)]))
        previous = jnp.maximum(c - 1, 0)
        following = jnp.where(c + 1 < n_chunks, chunk_slot(c + 1), q_slot)
        matmul = _Matmuls(
            *refill_late(chunk_slot(c)), *refill_early(following, 147),
            *[(geglu_jobs((t - 1) % n_tiles), *during(t)) for t in range(n_tiles)],
            (split_hidden_jobs(previous, 2), 30, 60), (split_hidden_jobs(previous, 3), 60, 98),
            (split_hidden_jobs(c, 0), 98, 145), (split_hidden_jobs(c, 1), 145, 163))
        for t in range(n_tiles):
            project(matmul, t, t % 2)

    @pl.loop(0, 2)
    def _(h):
        w_copy(o_slot, h).wait()
        w_copy(down_slot, h, wd_hbm, pl.multiple_of(h * hd, hd)).start()

    matmul = _Matmuls(
        *refill_late(q_slot), *refill_early(o_slot, 147, heads=True),
        (split_hidden_jobs(n_chunks - 1, 2), 30, 60), (split_hidden_jobs(n_chunks - 1, 3), 60, 98),
        (finish_qkv(1, 3, 2), 49, 147),
        (_jobs(shuffle_k, [(HALO + q * quarter + lo,) for lo in range(0, PLAIN * TILE, PACK)
                           for q in range(4)]), 35, 165),
        (geglu_jobs(n_tiles - 1), *during(0)),
        *[(finish_qkv(0, t, t % 2), *during(t + 1)) for t in range(n_tiles - 1)])
    for t in range(n_tiles):
        project(matmul, t, t % 2)
    for job in finish_qkv(0, n_tiles - 1, 1):
        job(None)

    for p in (1, 2):
        for g in range(groups):
            qkv[p, g, pl.ds(0, HALO), :] = jnp.broadcast_to(qkv[p, g, pl.ds(HALO, 1), :], (HALO, LANES))

    scale = float(d // N_HEADS) ** -0.5

    def attend(row0, q, lo, token):
        off = q * quarter + lo

        def load(p, w):
            return qkv[p, :, pl.ds(row0 + (HALO + off - DILATION * w), SUB), :]

        first, *rest = _unstack(load(0, 0))
        query = _stack([after(token, first)] + rest)
        logits = []
        for w in range(WINDOW):
            s = lax.reduce_sum(lax.mul(query, load(1, w)), (0,))
            for bit in (1, 2):
                other = lax.select(lane_bit[bit], pltpu.roll(s, bit, 1), pltpu.roll(s, LANES - bit, 1))
                s = lax.add(s, other)
            if off < DILATION * w:
                row = row0 + off + lax.broadcasted_iota(jnp.int32, (SUB, LANES), 0)
                s = jnp.where(row >= DILATION * w, s, MASKED_LOGIT / scale)
            logits.append(s)
        top = functools.reduce(lax.max, logits)
        weights = [lax.exp2(_times(lax.sub(s, top), scale * np.log2(np.e))) for s in logits]
        inv = lax.div(np.float32(1), functools.reduce(lax.add, weights))
        out = functools.reduce(lax.add, [
            lax.mul(lax.broadcast(weights[w], (groups,)), load(2, w)) for w in range(WINDOW)])
        out = [lax.mul(v, _times(inv, DELTA[q] / DELTA[g // 2])) for g, v in enumerate(_unstack(out))]
        mbuf[1, q, :, :, pl.ds(lo % (2 * PACK), SUB), :] = lax.reshape(
            _stack(swap_group_and_lane_bits(out, 1)), (4, 2, SUB, LANES))

    _wait(*[w_copy(down_slot, h, wd_hbm, h * hd) for h in range(2)])

    @pl.loop(0, n_tiles)
    def _(step):
        row0 = pl.multiple_of(step * TILE, TILE)
        plan = []
        for lo in range(0, TILE, PACK):
            first, last = 43 * lo / TILE, 43 * (lo + PACK) / TILE
            plan += [
                (_jobs(attend, [(row0, q, lo + i) for q in range(4) for i in (0, SUB)]), first, last),
                (left_jobs(lambda q, g, lo: mbuf[1, q, g // 2, g % 2, pl.ds(lo % (2 * PACK), PACK), :],
                           row0, [lo]), last + 1, last + 5)]
        matmul = _Matmuls(*plan, warp=lambda t: np.interp(t, np.cumsum([0] + ROOM) * 49 / sum(ROOM), range(50)))
        row0 = pl.multiple_of(step // 2 * (2 * TILE), 2 * TILE)
        for i in range(7):
            half = (step + 2 * i) % 2
            right = _operands(STRASSEN_RIGHT, [i], lambda r, c: lax.concatenate(
                [_unpack(wbuf.bitcast(U32)[4 * half + c, pl.ds((down_slot * d + n * FCHUNK + r * LANES) // 2, LANES // 2), :])
                 for n in range(n_chunks)], 0))
            blocks = _strassen(lambda j: matmul(
                _load(ha, (i, j, slice(None)), row0, 2 * TILE), _bf16(_unstack(right(j))[0])))
            for j, block in enumerate(blocks):
                mbuf[0, i, j] = lax.reshape(block, (2, TILE, LANES))
        for j in range(4):
            blocks = _strassen(lambda i: lax.reshape(mbuf[0, i, j], (2 * TILE, LANES)))
            for i, block in enumerate(blocks):
                r, c = _position(i, j)
                gbuf[step % 2, c, r, pl.ds(row0, 2 * TILE), :] = _silu(block, _unscale(r, c))

    def output_jobs(t, quadrants=range(4)):
        def use(r, c, g, lo, attn):
            rows = pl.ds(t * TILE + lo, PACK)
            x = lax.convert_element_type(xbuf[r, rows, pl.ds(g * hd + c * LANES, LANES)], F32)
            group = 4 * g + c + (zero if lo == g == r % 2 == c % 2 == 0 else 0)
            wbuf[group, pl.ds((down_slot + r % 2) * d + r // 2 * quarter + t * TILE + lo, PACK), :] = (
                _bf16(lax.add(x, lax.mul(attn, gbuf[g, c, r, rows, :]))))

        def send(token):
            _start(*[cp for h in range(2) if 3 * h in quadrants for cp in out_copies(t, h)])
            if quadrants == [0]:
                wbuf.bitcast(U32)[zero, pl.ds((down_slot * d + quarter + t * TILE) // 2, SUB), :] = pltpu.bitcast(token, U32)

        return finish_jobs(1 - t % 2, PACK, use, quadrants) + [send]

    matmul = _Matmuls(
        *refill_late(o_slot, heads=True),
        (output_jobs(0), *during(1)), (output_jobs(1), *during(2)),
        (output_jobs(2), 147, 176), (output_jobs(3, [1]), 176, 182), (output_jobs(3, [0]), 182, 188))
    for t in range(n_tiles):
        project(matmul, t, 1 - t % 2)
    for job in output_jobs(3, [2, 3]):
        job(None)
    _wait(*[cp for t in range(n_tiles) for h in range(2) for cp in out_copies(t, h)])


@jax.jit
def pallas_recurrent_scan__sliding_local_dilated__geglu_ffn__prompt_kernel(
    A_x: jax.Array,
    A_wqkv: jax.Array,
    A_wo: jax.Array,
    B_x: jax.Array,
    B_w_gate: jax.Array,
    B_w_up: jax.Array,
    B_w_down: jax.Array,
):
    del B_x
    b, s, d = A_x.shape
    f = B_w_gate.shape[1]
    assert (b, s, d, f) == (1, 16 * TILE, 8 * LANES, 7 * FCHUNK) and A_x.dtype == BF16
    quarter, groups = s // 4, d // LANES

    hbm = pl.BlockSpec(memory_space=pl.ANY)
    out = pl.pallas_call(
        _kernel,
        out_shape=jax.ShapeDtypeStruct((4, quarter, d), BF16),
        in_specs=[hbm] * 6,
        out_specs=hbm,
        scratch_shapes=[
            pltpu.VMEM((4, quarter, d), BF16),
            pltpu.VMEM((groups, 2 * d + f, LANES), BF16),
            pltpu.VMEM((7, 7, 2, quarter, LANES), BF16),
            pltpu.VMEM((7, 7, 2, d // 4, LANES), BF16),
            pltpu.VMEM((3, 7, 2, d // 4, LANES), BF16),
            pltpu.VMEM((7, 7, f // FCHUNK, quarter, LANES), BF16),
            pltpu.VMEM((2, 7, 4, 2, TILE, LANES), F32),
            pltpu.VMEM((3, groups, HALO + s, LANES), F32),
            pltpu.VMEM((2, 4, 4, quarter, LANES), F32),
            pltpu.SemaphoreType.DMA((4,)),
            pltpu.SemaphoreType.DMA((10,)),
            pltpu.SemaphoreType.DMA((8,)),
        ],
        compiler_params=pltpu.CompilerParams(
            vmem_limit_bytes=127 * 1024 * 1024, disable_bounds_checks=True),
        name="fused_local_attn_geglu",
    )(A_x.reshape(4, quarter, d), A_wqkv, A_wo, B_w_gate, B_w_up, B_w_down)
    return out.reshape(b, s, d)
```

```python
import functools

import jax
import jax.numpy as jnp
import numpy as np
from jax import lax
import jax.experimental.pallas as pl
import jax.experimental.pallas.tpu as pltpu

F32 = jnp.float32
BF16 = jnp.bfloat16
U32 = jnp.uint32

N_HEADS = 32
WINDOW = 8
DILATION = 2
LN_EPS = 1e-5
MASKED_LOGIT = -1e9

LANES = 128
SUB = 8
PACK = 16
HALO = 16
FCHUNK = 512
TILE = 128
ROOM = [a * b for a in (1, 1, 1, 1, 1, 1, 1) for b in (.5, 1, 1, 1, 1, 1, 1)]
PLAIN = 2


STRASSEN_LEFT = ("c+d", "d", "a+b", "a", "t", "c-a", "b-d")
STRASSEN_RIGHT = ("a", "c-a", "d", "b-d", "t", "a+b", "c+d")


def _strassen(m):
    m0, m1 = m(0), m(1)
    c = lax.add(m0, m1)
    m2, m3 = m(2), m(3)
    b = lax.add(m2, m3)
    m4 = m(4)
    d = lax.add(lax.add(m4, lax.sub(m3, m0)), m(5))
    a = lax.add(lax.add(m4, lax.sub(m1, m2)), m(6))
    return a, b, c, d


BALANCED_LEFT = ("a-b", "a+b", "t+t", "d-b", "d+b", "t-s", "t+s")
BALANCED_RIGHT = ("d-b", "d+b", "t", "t+s", "t-s", "a+b", "a-b")
LEFT_FAMILIES = ((0, 1), (2, 5, 6), (3, 4))
LEFT_ORDER = sum(LEFT_FAMILIES, ())
RIGHT_FAMILIES = ((0, 1), (2, 3, 4), (5, 6))
DELTA = (1.0, 3.0 ** 0.5, 3.0 ** 0.5, 3.0)


def _balanced(m):
    m0, m1 = m(0), m(1)
    b = lax.sub(m1, m0)
    diag = lax.sub(m(2), lax.add(m0, m1))
    m3, m4 = m(3), m(4)
    a = lax.sub(diag, lax.add(m3, m4))
    low = lax.add(b, lax.sub(m3, m4))
    m5, m6 = m(5), m(6)
    return a, b, lax.add(low, lax.sub(m6, m5)), lax.sub(diag, lax.add(m5, m6))


def _unscale(r, c):
    return DELTA[c] / DELTA[r] / 4


def _position(outer, inner):
    return outer // 2 * 2 + inner // 2, outer % 2 * 2 + inner % 2


def _combinations(quadrant):
    @functools.cache
    def term(name):
        if len(name) == 3:
            return (lax.add if name[1] == "+" else lax.sub)(term(name[0]), term(name[2]))
        if name in "ts":
            return term("a+d" if name == "t" else "b+c")
        return quadrant("abcd".index(name))

    return term


def _operands(side, family, block):
    outer = _combinations(lambda i: _stack([block(*_position(i, j)) for j in range(4)]))
    parts = _stack([outer(side[i]) for i in family])
    inner = _combinations(lambda j: lax.index_in_dim(parts, j, 1, keepdims=False))
    return lambda j: inner(side[j])


class _Matmuls:
    def __init__(self, *plan, warp=None):
        self.calls = 0
        warp = warp or (lambda t: t)
        self.jobs = sorted(
            ((warp(first + (last - first) * (i + 0.618 * n % 1) / len(jobs)), n, job)
             for n, (jobs, first, last) in enumerate(plan) for i, job in enumerate(jobs)),
            key=lambda t: t[:2], reverse=True)

    def __call__(self, lhs, rhs):
        value = lax.dot_general(lhs, rhs, (((1,), (0,)), ((), ())), preferred_element_type=F32)
        while self.jobs and self.jobs[-1][0] < self.calls + 1:
            when, _, job = self.jobs.pop()
            row = int((when - self.calls) * (value.shape[0] // SUB)) * SUB
            job(lax.slice(value, (row, 0), (row + SUB, LANES)))
        self.calls += 1
        return value


def _jobs(fn, args):
    return [functools.partial(fn, *a) for a in args]


def _times(x, c):
    return x if c == 1.0 else lax.mul(x, np.float32(c))


def _plus(x, c):
    return lax.add(x, np.float32(c))


def _aligned(i, n):
    return i if isinstance(i, int) else pl.multiple_of(i, n)


def _stack(xs):
    return lax.reshape(lax.concatenate(xs, 0), (len(xs), *xs[0].shape))


def _unstack(x):
    return [lax.index_in_dim(x, i, 0, keepdims=False) for i in range(x.shape[0])]


def _rows(x, lo, n):
    return lax.slice_in_dim(x, lo, lo + n, axis=0)


def _lane_groups(x):
    return [lax.slice_in_dim(x, j, j + LANES, axis=1) for j in range(0, x.shape[1], LANES)]


def _bf16(x):
    return lax.convert_element_type(x, BF16)


def _unpack(words):
    return lax.convert_element_type(pltpu.bitcast(words, BF16), F32)


def _geglu(g, u, scale):
    k0 = (2 / np.pi) ** 0.5
    t = lax.tanh(lax.mul(g, _plus(_times(lax.mul(g, g), k0 * 0.044715 * scale ** 3), k0 * scale)))
    return lax.mul(lax.mul(_times(g, 0.5 * scale ** 2), u), _plus(t, 1.0))


def _silu(x, scale):
    h = _times(x, 0.5)
    return lax.mul(_times(h, scale), _plus(lax.tanh(h), 1.0))


def _load(ref, index, lo, n):
    words = ref.bitcast(U32)[(*index, pl.ds(_aligned(lo // 2, SUB), n // 2))]
    return lax.concatenate(_unstack(pltpu.bitcast(words, BF16)), 1)


class _ColumnCopy:
    def __init__(self, src, col, dst, sem):
        self.src, self.col, self.dst, self.sem = src, col, dst, sem

    def start(self):
        for g in range(self.dst.shape[0]):
            cols = pl.ds(self.col + g * LANES, LANES)
            pltpu.make_async_copy(self.src.at[:, cols], self.dst.at[g], self.sem).start()

    def wait(self):
        pltpu.make_async_copy(self.dst, self.dst, self.sem).wait()


def _start(*copies):
    for cp in copies:
        cp.start()


def _wait(*copies):
    for cp in copies:
        cp.wait()


def _kernel(x_hbm, wqkv_hbm, wo_hbm, wg_hbm, wu_hbm, wd_hbm, out_hbm,
            xbuf,
            wbuf,
            xa,
            wa,
            wb,
            ha,
            mbuf,
            qkv,
            gbuf,
            x_sem, w_sem, out_sem):
    _, quarter, d = x_hbm.shape
    n_chunks, n_tiles = ha.shape[2], quarter // TILE
    hd, qd, groups = d // 2, d // 4, d // LANES

    def chunk_slot(c):
        return 1 + (c + 2) % 3

    q_slot, k_slot, v_slot, o_slot, down_slot = 0, 4, chunk_slot(1), chunk_slot(n_chunks), 2

    def x_copies(t):
        at = [(slice(None), pl.ds(t * TILE, TILE), pl.ds(col, hd)) for col in (0, hd)]
        return [pltpu.make_async_copy(x_hbm.at[i], xbuf.at[i], x_sem.at[t]) for i in at]

    def w_copy(slot, h, src=None, col=None):
        rows = pl.ds(0, d if src is None else src.shape[0])
        dst = wbuf.at[slot, pl.ds(h * (groups // 2), groups // 2), rows]
        return _ColumnCopy(src, col, dst, w_sem.at[2 * slot + h])

    def chunk_copies(c):
        return [w_copy(chunk_slot(c), h, w, _aligned(c * FCHUNK, FCHUNK)) for h, w in enumerate((wg_hbm, wu_hbm))]

    def down_copies(h):
        f = wd_hbm.shape[0]
        return [w_copy(down_slot + lo // d, h, wd_hbm.at[pl.ds(lo, min(d, f - lo))], _aligned(h * hd, hd))
                for lo in range(0, f, d)]

    def out_copies(t, h):
        return [pltpu.make_async_copy(
            wbuf.at[down_slot + i, g, pl.ds(h * quarter + t * TILE, TILE)],
            out_hbm.at[2 * h + i, pl.ds(t * TILE, TILE), pl.ds(g * LANES, LANES)],
            out_sem.at[2 * t + h]) for i in range(2) for g in range(groups)]

    xs = [x_copies(t) for t in range(n_tiles)]
    wq = [w_copy(q_slot, h, wqkv_hbm, h * hd) for h in range(2)]
    wk = [w_copy(k_slot, h, wqkv_hbm, d + h * hd) for h in range(2)]
    wv = [w_copy(v_slot, h, wqkv_hbm, 2 * d + h * hd) for h in range(2)]

    _start(*xs[0], wk[0])
    xs[0][0].wait()
    _start(*xs[1], wk[1])
    xs[0][1].wait()
    _start(*wv)

    never = jnp.abs(xbuf[0, :SUB, :LANES].astype(F32)) < 0
    zero = jnp.sum(jnp.where(never, 1, 0))
    lane = lax.broadcasted_iota(jnp.int32, (SUB, LANES), 1)
    lane_bit = {bit: (lane & bit) != 0 for bit in (1, 2, 4, 8, 16)}

    def after(token, x):
        if token is None:
            return x
        if x.dtype != token.dtype:
            token = pltpu.bitcast(token, x.dtype)
        n = x.shape[0] // SUB
        return lax.select(lax.concatenate([never] * n, 0), lax.concatenate([token] * n, 0), x)

    def swap_group_and_lane_bits(cols, bits=3):
        cols = list(cols)
        for gbit, lbit in ((1, 4), (2, 8), (4, 16))[:bits]:
            for i in range(len(cols)):
                if not i & gbit:
                    a, b = cols[i], cols[i | gbit]
                    cols[i] = lax.select(lane_bit[lbit], pltpu.roll(b, lbit, 1), a)
                    cols[i | gbit] = lax.select(lane_bit[lbit], b, pltpu.roll(a, LANES - lbit, 1))
        return cols

    def operand_jobs(side, family, load, dst, first, row0, positions):
        def job(g, lo, token):
            operand = _operands(side, family, lambda r, c: load(r, c, g, lo, token))
            for j in range(7):
                dst[pl.ds(first, len(family)), j, g, pl.ds(row0 + lo, PACK), :] = _bf16(operand(j))

        return _jobs(job, positions)

    def left_jobs(load, row0, rows):
        return [job for family in LEFT_FAMILIES for job in operand_jobs(
            BALANCED_LEFT, family, lambda r, c, g, lo, token: after(token, load(r, 2 * c + g, lo)),
            xa, LEFT_ORDER.index(family[0]), row0, [(g, lo) for lo in rows for g in range(2)])]

    def right_jobs(slot, family, dst=wa, heads=False):
        family = RIGHT_FAMILIES[family]

        def load(r, c, g, lo, token):
            def rows(at):
                return _unpack(after(token, wbuf.bitcast(U32)[slot, 4 * g + c, pl.ds(at // 2, SUB)]))

            if heads:
                at = lo // PACK % 2 * hd + lo // (2 * PACK) * (2 * PACK) + r // 2 * PACK
                x = lax.concatenate([_rows(rows(at + i * qd), r % 2 * SUB, SUB) for i in range(2)], 0)
            else:
                x = rows(r * qd + lo)
            return _times(x, DELTA[r] / DELTA[c])

        return operand_jobs(BALANCED_RIGHT, family, load, dst, family[0] if dst is wa else 0, 0,
                            [(g, lo) for lo in range(0, qd, PACK) for g in range(2)])

    def move(i, j, g, lo, token):
        rows = pl.ds(lo, 4 * SUB)
        wa.bitcast(U32)[2 + i, j, g, rows, :] = after(token, wb.bitcast(U32)[i, j, g, rows, :])

    moves = _jobs(move, [(i, j, g, lo) for i in range(3) for j in range(7) for g in range(2)
                         for lo in range(0, qd // 2, 4 * SUB)])

    def refill_early(slot, last, **kw):
        return [(right_jobs(slot, 1, wb, **kw), max(last - 90, 23), max(last - 3, 62)),
                (right_jobs(slot, 0, **kw), last + 14.5, last + 47),
                (moves[:len(moves) // 2], last + 22, last + 47)]

    def refill_late(slot, **kw):
        return [(moves[len(moves) // 2:], 0, 22), (right_jobs(slot, 2, **kw), 0, 33.5)]

    def partial(slot, i, j, g, lo, n):
        if slot < 2:
            return mbuf, (slot, i, j, pl.ds(*g), pl.ds(lo, n))
        return gbuf, (1, j, pl.ds(i // 4 * 2 + g[0], g[1]), pl.ds(i % 4 * TILE + lo, n))

    def project(matmul, t, slot):
        for i in range(7):
            blocks = _balanced(lambda j: matmul(
                _load(xa, (LEFT_ORDER.index(i), j, slice(None)), t * TILE, TILE),
                _load(wa, (i, j, slice(None)), 0, qd)))
            for j, block in enumerate(blocks):
                ref, index = partial(slot, i, j, (0, 2), 0, TILE)
                ref[index] = _stack(_lane_groups(block))

    def finish_jobs(slot, n, use, quadrants=range(4)):
        def job(lo, j, g, token):
            def product(i):
                ref, index = partial(slot, i, j, g, lo, n)
                return after(None if i else token, lax.reshape(ref[index], (PACK, LANES)))

            out = _balanced(product)
            for i in quadrants:
                use(*_position(i, j), g[0], lo, out[i])

        return _jobs(job, [(lo, j, g) for lo in range(0, TILE, n) for j in range(4)
                           for g in (((0, 1), (1, 1)) if n == PACK else ((0, 2),))])

    def during(step):
        return 49 * step, 49 * step + 47

    def norm(q, lo, scaled, plain, token):
        def rows(lo):
            first, *rest = _lane_groups(lax.convert_element_type(xbuf[q, pl.ds(lo, SUB), :], F32))
            x = lax.concatenate([after(token, first)] + rest, 1)
            x = x - jnp.sum(x, axis=-1, keepdims=True) * (1.0 / d)
            inv = lax.rsqrt(jnp.sum(x * x, axis=-1, keepdims=True) * (1.0 / d) + LN_EPS)
            inv = lax.broadcast_in_dim(inv, (SUB, LANES), (0, 1))
            return [lax.mul(v, _times(inv, DELTA[q] / DELTA[g // 2] if scaled else 1.0))
                    for g, v in enumerate(_lane_groups(x))]

        if scaled:
            gbuf[:, :, q, pl.ds(lo, SUB), :] = lax.reshape(_stack(rows(lo)), (2, 4, SUB, LANES))
        if plain and lo % PACK:
            lo -= SUB
            cols = ([_times(gbuf[g // 4, g % 4, q, pl.ds(lo, PACK), :], DELTA[g // 2] / DELTA[q])
                     for g in range(groups)] if scaled else
                    [lax.concatenate(v, 0) for v in zip(rows(lo), rows(lo + SUB))])
            for g, v in enumerate(cols):
                ha[lo // TILE, g // 4, g % 4, pl.ds(q * TILE + lo % TILE, PACK), :] = _bf16(v)

    def norm_jobs(t, scaled=True, plain=False):
        return _jobs(norm, [(q, t * TILE + lo, scaled, plain)
                            for q in range(4) for lo in range(0, TILE, SUB)])

    def split_x_jobs(t):
        return left_jobs(lambda q, g, lo: gbuf[g // 4, g % 4, q, pl.ds(lo, PACK), :],
                         0, range(t * TILE, (t + 1) * TILE, PACK))

    def shuffle_weight_jobs(slot):
        words = wbuf.bitcast(U32)

        def job(lo, token):
            at = (slot, slice(None), pl.ds(lo // 2, SUB))
            words[at] = _stack(swap_group_and_lane_bits([after(token, v) for v in _unstack(words[at])]))

        return _jobs(job, [(lo + r * qd,) for lo in range(0, qd, PACK) for r in range(4)])

    def plain_k(t, gs, *plan):
        matmul = _Matmuls(*plan)
        for g in gs:
            k = lax.add(*[matmul(_load(ha, (t, h, pl.ds(0, 4)), 0, 4 * TILE),
                                 _load(wbuf, (k_slot, pl.ds(g, 1)), h * hd, hd)) for h in range(2)])
            k = pltpu.bitcast(_bf16(k), F32)
            for lo in range(0, 4 * TILE, PACK):
                row = HALO + lo // TILE * quarter + t * TILE + lo % TILE
                qkv[1, g, pl.ds(row, SUB), :] = _rows(k, lo // 2, SUB)

    def shuffle_k(row, token):
        cols = [after(token, v) for v in _unstack(pltpu.bitcast(qkv[1, :, pl.ds(row, SUB), :], U32))]
        qkv[1, :, pl.ds(row, PACK), :] = _unpack(_stack(swap_group_and_lane_bits(cols)))

    def finish_qkv(p, t, slot):
        def use(r, c, _, lo, x):
            x = _times(x, _unscale(r, c))
            for g in range(2):
                qkv[p, 4 * g + c, pl.ds(HALO + r * quarter + t * TILE + lo, SUB), :] = _rows(x, g * SUB, SUB)

        return finish_jobs(slot, SUB, use)

    for job in norm_jobs(0, plain=True):
        job(None)
    wk[0].wait()
    _start(*xs[2], *xs[3])
    plain_k(0, range(4), (split_x_jobs(0), 0, 7))
    _wait(*xs[1], wk[1])
    _start(*wq, *chunk_copies(0))
    plain_k(0, range(4, 8), (norm_jobs(1, plain=True), 0, 6.5))
    _wait(*wv)
    plain_k(1, range(8), (shuffle_weight_jobs(v_slot), 0, 13.5),
            *[(right_jobs(v_slot, f), 1.5, 15.5) for f in range(3)])
    _start(*chunk_copies(1))
    _wait(*xs[2], *xs[3])
    matmul = _Matmuls((norm_jobs(2) + norm_jobs(3), 0, 44), (split_x_jobs(1)[:32], 0, 47))
    project(matmul, 0, 0)
    _wait(*wq)
    matmul = _Matmuls(
        (split_x_jobs(1)[32:], 0, 19), (split_x_jobs(2), *during(0)), (split_x_jobs(3), *during(1)),
        *[(finish_qkv(2, t, t % 2), *during(t)) for t in range(3)],
        (shuffle_weight_jobs(k_slot), 0, 96),
        (right_jobs(k_slot, 1, wb), 98, 119), (right_jobs(k_slot, 0), 119, 146),
        (moves[:len(moves) // 2], 121, 146))
    project(matmul, 1, 1)
    project(matmul, 2, 0)

    @pl.loop(0, 2)
    def _(h):
        w_copy(chunk_slot(0), h).wait()

    project(matmul, 3, 1)
    matmul = _Matmuls(
        *refill_late(k_slot), *refill_early(chunk_slot(0), 49),
        (shuffle_weight_jobs(q_slot), 0, 92),
        (finish_qkv(2, 3, 1), *during(0)), (finish_qkv(1, 2, 0), *during(1)))
    project(matmul, 2, 0)
    project(matmul, 3, 2)

    def geglu_jobs(t):
        def use(r, c, _, lo, x):
            gbuf[0, c, r, pl.ds(t * TILE + lo, SUB), :] = _geglu(
                _rows(x, 0, SUB), _rows(x, SUB, SUB), _unscale(r, c))

        return finish_jobs(t % 2, SUB, use)

    def split_hidden_jobs(chunk, t):
        return [job for lo in range(t * TILE, (t + 1) * TILE, PACK)
                for family in ((0, 1), (2, 3), (4,), (5,), (6,)) for job in operand_jobs(
                    STRASSEN_LEFT, family,
                    lambda r, c, g, lo, token: after(token, gbuf[0, c, r, pl.ds(lo, PACK), :]),
                    ha, family[0], 0, [(chunk, lo)])]

    @pl.loop(0, n_chunks)
    def _(c):
        pl.when(c + 1 < n_chunks)(lambda: _wait(*chunk_copies(c + 1)))
        pl.when(c + 2 < n_chunks)(lambda: _start(*chunk_copies(c + 2)))
        pl.when(c + 2 == n_chunks)(
            lambda: _start(*[w_copy(o_slot, h, wo_hbm, h * hd) for h in range(2)]))
        previous = jnp.maximum(c - 1, 0)
        following = jnp.where(c + 1 < n_chunks, chunk_slot(c + 1), q_slot)
        matmul = _Matmuls(
            *refill_late(chunk_slot(c)), *refill_early(following, 147),
            *[(geglu_jobs((t - 1) % n_tiles), *during(t)) for t in range(n_tiles)],
            (split_hidden_jobs(previous, 2), 30, 60), (split_hidden_jobs(previous, 3), 60, 98),
            (split_hidden_jobs(c, 0), 98, 145), (split_hidden_jobs(c, 1), 145, 163))
        for t in range(n_tiles):
            project(matmul, t, t % 2)

    @pl.loop(0, 2)
    def _(h):
        w_copy(o_slot, h).wait()
        _start(*down_copies(h))

    matmul = _Matmuls(
        *refill_late(q_slot), *refill_early(o_slot, 147, heads=True),
        (split_hidden_jobs(n_chunks - 1, 2), 30, 60), (split_hidden_jobs(n_chunks - 1, 3), 60, 98),
        (finish_qkv(1, 3, 2), 49, 147),
        (_jobs(shuffle_k, [(HALO + q * quarter + lo,) for lo in range(0, PLAIN * TILE, PACK)
                           for q in range(4)]), 35, 165),
        (geglu_jobs(n_tiles - 1), *during(0)),
        *[(finish_qkv(0, t, t % 2), *during(t + 1)) for t in range(n_tiles - 1)])
    for t in range(n_tiles):
        project(matmul, t, t % 2)
    for job in finish_qkv(0, n_tiles - 1, 1):
        job(None)

    for p in (1, 2):
        for g in range(groups):
            qkv[p, g, pl.ds(0, HALO), :] = jnp.broadcast_to(qkv[p, g, pl.ds(HALO, 1), :], (HALO, LANES))

    scale = float(d // N_HEADS) ** -0.5

    def attend(row0, q, lo, token):
        off = q * quarter + lo

        def load(p, w):
            return qkv[p, :, pl.ds(row0 + (HALO + off - DILATION * w), SUB), :]

        first, *rest = _unstack(load(0, 0))
        query = _stack([after(token, first)] + rest)
        logits = []
        for w in range(WINDOW):
            s = lax.reduce_sum(lax.mul(query, load(1, w)), (0,))
            for bit in (1, 2):
                other = lax.select(lane_bit[bit], pltpu.roll(s, bit, 1), pltpu.roll(s, LANES - bit, 1))
                s = lax.add(s, other)
            if off < DILATION * w:
                row = row0 + off + lax.broadcasted_iota(jnp.int32, (SUB, LANES), 0)
                s = jnp.where(row >= DILATION * w, s, MASKED_LOGIT / scale)
            logits.append(s)
        top = functools.reduce(lax.max, logits)
        weights = [lax.exp2(_times(lax.sub(s, top), scale * np.log2(np.e))) for s in logits]
        inv = lax.div(np.float32(1), functools.reduce(lax.add, weights))
        out = functools.reduce(lax.add, [
            lax.mul(lax.broadcast(weights[w], (groups,)), load(2, w)) for w in range(WINDOW)])
        out = [lax.mul(v, _times(inv, DELTA[q] / DELTA[g // 2])) for g, v in enumerate(_unstack(out))]
        mbuf[1, q, :, :, pl.ds(lo % (2 * PACK), SUB), :] = lax.reshape(
            _stack(swap_group_and_lane_bits(out, 1)), (4, 2, SUB, LANES))

    _wait(*down_copies(0), *down_copies(1))

    @pl.loop(0, n_tiles)
    def _(step):
        row0 = pl.multiple_of(step * TILE, TILE)
        plan = []
        for lo in range(0, TILE, PACK):
            first, last = 43 * lo / TILE, 43 * (lo + PACK) / TILE
            plan += [
                (_jobs(attend, [(row0, q, lo + i) for q in range(4) for i in (0, SUB)]), first, last),
                (left_jobs(lambda q, g, lo: mbuf[1, q, g // 2, g % 2, pl.ds(lo % (2 * PACK), PACK), :],
                           row0, [lo]), last + 1, last + 5)]
        matmul = _Matmuls(*plan, warp=lambda t: np.interp(t, np.cumsum([0] + ROOM) * 49 / sum(ROOM), range(50)))
        row0 = pl.multiple_of(step // 2 * (2 * TILE), 2 * TILE)
        for i in range(7):
            half = (step + 2 * i) % 2
            right = _operands(STRASSEN_RIGHT, [i], lambda r, c: lax.concatenate(
                [_unpack(wbuf.bitcast(U32)[down_slot + n // 2, 4 * half + c,
                                           pl.ds((n % 2 * FCHUNK + r * LANES) // 2, LANES // 2), :])
                 for n in range(n_chunks)], 0))
            blocks = _strassen(lambda j: matmul(
                _load(ha, (i, j, slice(None)), row0, 2 * TILE), _bf16(_unstack(right(j))[0])))
            for j, block in enumerate(blocks):
                mbuf[0, i, j] = lax.reshape(block, (2, TILE, LANES))
        for j in range(4):
            blocks = _strassen(lambda i: lax.reshape(mbuf[0, i, j], (2 * TILE, LANES)))
            for i, block in enumerate(blocks):
                r, c = _position(i, j)
                gbuf[step % 2, c, r, pl.ds(row0, 2 * TILE), :] = _silu(block, _unscale(r, c))

    def output_jobs(t, quadrants=range(4)):
        def use(r, c, g, lo, attn):
            rows = pl.ds(t * TILE + lo, PACK)
            x = lax.convert_element_type(xbuf[r, rows, pl.ds(g * hd + c * LANES, LANES)], F32)
            group = 4 * g + c + (zero if lo == g == r % 2 == c % 2 == 0 else 0)
            wbuf[down_slot + r % 2, group, pl.ds(r // 2 * quarter + t * TILE + lo, PACK), :] = (
                _bf16(lax.add(x, lax.mul(attn, gbuf[g, c, r, rows, :]))))

        def send(token):
            _start(*[cp for h in range(2) if 3 * h in quadrants for cp in out_copies(t, h)])
            if quadrants == [0]:
                wbuf.bitcast(U32)[down_slot, zero, pl.ds((quarter + t * TILE) // 2, SUB), :] = pltpu.bitcast(token, U32)

        return finish_jobs(1 - t % 2, PACK, use, quadrants) + [send]

    matmul = _Matmuls(
        *refill_late(o_slot, heads=True),
        (output_jobs(0), *during(1)), (output_jobs(1), *during(2)),
        (output_jobs(2), 147, 176), (output_jobs(3, [1]), 176, 182), (output_jobs(3, [0]), 182, 188))
    for t in range(n_tiles):
        project(matmul, t, 1 - t % 2)
    for job in output_jobs(3, [2, 3]):
        job(None)
    _wait(*[cp for t in range(n_tiles) for h in range(2) for cp in out_copies(t, h)])


@jax.jit
def pallas_recurrent_scan__sliding_local_dilated__geglu_ffn__prompt_kernel(
    A_x: jax.Array,
    A_wqkv: jax.Array,
    A_wo: jax.Array,
    B_x: jax.Array,
    B_w_gate: jax.Array,
    B_w_up: jax.Array,
    B_w_down: jax.Array,
):
    del B_x
    b, s, d = A_x.shape
    f = B_w_gate.shape[1]
    assert (b, s, d, f) == (1, 16 * TILE, 8 * LANES, 7 * FCHUNK) and A_x.dtype == BF16
    quarter, groups = s // 4, d // LANES

    hbm = pl.BlockSpec(memory_space=pl.ANY)
    out = pl.pallas_call(
        _kernel,
        out_shape=jax.ShapeDtypeStruct((4, quarter, d), BF16),
        in_specs=[hbm] * 6,
        out_specs=hbm,
        scratch_shapes=[
            pltpu.VMEM((4, quarter, d), BF16),
            pltpu.VMEM((6, groups, d, LANES), BF16),
            pltpu.VMEM((7, 7, 2, quarter, LANES), BF16),
            pltpu.VMEM((7, 7, 2, d // 4, LANES), BF16),
            pltpu.VMEM((3, 7, 2, d // 4, LANES), BF16),
            pltpu.VMEM((7, 7, f // FCHUNK, quarter, LANES), BF16),
            pltpu.VMEM((2, 7, 4, 2, TILE, LANES), F32),
            pltpu.VMEM((3, groups, HALO + s, LANES), F32),
            pltpu.VMEM((2, 4, 4, quarter, LANES), F32),
            pltpu.SemaphoreType.DMA((4,)),
            pltpu.SemaphoreType.DMA((12,)),
            pltpu.SemaphoreType.DMA((8,)),
        ],
        compiler_params=pltpu.CompilerParams(
            vmem_limit_bytes=127 * 1024 * 1024, disable_bounds_checks=True),
        name="fused_local_attn_geglu",
    )(A_x.reshape(4, quarter, d), A_wqkv, A_wo, B_w_gate, B_w_up, B_w_down)
    return out.reshape(b, s, d)
```

```python
import functools

import jax
import jax.numpy as jnp
import numpy as np
from jax import lax
import jax.experimental.pallas as pl
import jax.experimental.pallas.tpu as pltpu

F32 = jnp.float32
BF16 = jnp.bfloat16
U32 = jnp.uint32

N_HEADS = 32
WINDOW = 8
DILATION = 2
LN_EPS = 1e-5
MASKED_LOGIT = -1e9

LANES = 128
SUB = 8
PACK = 16
HALO = 16
FCHUNK = 512
TILE = 128
PLAIN = 2


STRASSEN_LEFT = ("c+d", "d", "a+b", "a", "t", "c-a", "b-d")
STRASSEN_RIGHT = ("a", "c-a", "d", "b-d", "t", "a+b", "c+d")


def _strassen(m):
    m0, m1 = m(0), m(1)
    c = lax.add(m0, m1)
    m2, m3 = m(2), m(3)
    b = lax.add(m2, m3)
    m4 = m(4)
    d = lax.add(lax.add(m4, lax.sub(m3, m0)), m(5))
    a = lax.add(lax.add(m4, lax.sub(m1, m2)), m(6))
    return a, b, c, d


BALANCED_LEFT = ("a-b", "a+b", "t+t", "d-b", "d+b", "t-s", "t+s")
BALANCED_RIGHT = ("d-b", "d+b", "t", "t+s", "t-s", "a+b", "a-b")
LEFT_FAMILIES = ((0, 1), (2, 5, 6), (3, 4))
LEFT_ORDER = sum(LEFT_FAMILIES, ())
RIGHT_FAMILIES = ((0, 1), (2, 3, 4), (5, 6))
DELTA = (1.0, 3.0 ** 0.5, 3.0 ** 0.5, 3.0)


def _balanced(m):
    m0, m1 = m(0), m(1)
    b = lax.sub(m1, m0)
    diag = lax.sub(m(2), lax.add(m0, m1))
    m3, m4 = m(3), m(4)
    a = lax.sub(diag, lax.add(m3, m4))
    low = lax.add(b, lax.sub(m3, m4))
    m5, m6 = m(5), m(6)
    return a, b, lax.add(low, lax.sub(m6, m5)), lax.sub(diag, lax.add(m5, m6))


def _unscale(r, c):
    return DELTA[c] / DELTA[r] / 4


def _position(outer, inner):
    return outer // 2 * 2 + inner // 2, outer % 2 * 2 + inner % 2


def _combinations(quadrant):
    @functools.cache
    def term(name):
        if len(name) == 3:
            return (lax.add if name[1] == "+" else lax.sub)(term(name[0]), term(name[2]))
        if name in "ts":
            return term("a+d" if name == "t" else "b+c")
        return quadrant("abcd".index(name))

    return term


def _operands(side, family, block):
    outer = _combinations(lambda i: _stack([block(*_position(i, j)) for j in range(4)]))
    parts = _stack([outer(side[i]) for i in family])
    inner = _combinations(lambda j: lax.index_in_dim(parts, j, 1, keepdims=False))
    return lambda j: inner(side[j])


def _token(value, row, n, dtype):
    x = lax.slice(value, (row, 0), (row + SUB, LANES))
    return lax.concatenate([x if dtype == x.dtype else pltpu.bitcast(x, dtype)] * (n // SUB), 0)


class _Matmuls:
    def __init__(self, *plan):
        self.calls = 0
        self.jobs = sorted(
            ((first + (last - first) * (i + 0.618 * n % 1) / len(jobs), n, job)
             for n, (jobs, first, last) in enumerate(plan) for i, job in enumerate(jobs)),
            key=lambda t: t[:2], reverse=True)

    def __call__(self, lhs, rhs):
        value = lax.dot_general(lhs, rhs, (((1,), (0,)), ((), ())), preferred_element_type=F32)
        while self.jobs and self.jobs[-1][0] < self.calls + 1:
            when, _, job = self.jobs.pop()
            row = int((when - self.calls) * (value.shape[0] // SUB)) * SUB
            job(functools.cache(functools.partial(_token, value, row)))
        self.calls += 1
        return value


def _jobs(fn, args):
    return [functools.partial(fn, *a) for a in args]


def _times(x, c):
    return x if c == 1.0 else lax.mul(x, np.float32(c))


def _plus(x, c):
    return lax.add(x, np.float32(c))


def _aligned(i, n):
    return i if isinstance(i, int) else pl.multiple_of(i, n)


def _stack(xs):
    return lax.reshape(lax.concatenate(xs, 0), (len(xs), *xs[0].shape))


def _unstack(x):
    return [lax.index_in_dim(x, i, 0, keepdims=False) for i in range(x.shape[0])]


def _rows(x, lo, n):
    return lax.slice_in_dim(x, lo, lo + n, axis=0)


def _lane_groups(x):
    return [lax.slice_in_dim(x, j, j + LANES, axis=1) for j in range(0, x.shape[1], LANES)]


def _bf16(x):
    return lax.convert_element_type(x, BF16)


def _unpack(words):
    return lax.convert_element_type(pltpu.bitcast(words, BF16), F32)


def _geglu(g, u, scale):
    k0 = (2 / np.pi) ** 0.5
    t = lax.tanh(lax.mul(g, _plus(_times(lax.mul(g, g), k0 * 0.044715 * scale ** 3), k0 * scale)))
    return lax.mul(lax.mul(_times(g, 0.5 * scale ** 2), u), _plus(t, 1.0))


def _silu(x, scale):
    h = _times(x, 0.5)
    return lax.mul(_times(h, scale), _plus(lax.tanh(h), 1.0))


def _load(ref, index, lo, n):
    words = ref.bitcast(U32)[(*index, pl.ds(_aligned(lo // 2, SUB), n // 2))]
    return lax.concatenate(_unstack(pltpu.bitcast(words, BF16)), 1)


class _ColumnCopy:
    def __init__(self, src, col, dst, sem):
        self.src, self.col, self.dst, self.sem = src, col, dst, sem

    def start(self):
        for g in range(self.dst.shape[0]):
            cols = pl.ds(self.col + g * LANES, LANES)
            pltpu.make_async_copy(self.src.at[:, cols], self.dst.at[g], self.sem).start()

    def wait(self):
        pltpu.make_async_copy(self.dst, self.dst, self.sem).wait()


def _start(*copies):
    for cp in copies:
        cp.start()


def _wait(*copies):
    for cp in copies:
        cp.wait()


def _kernel(x_hbm, wqkv_hbm, wo_hbm, wg_hbm, wu_hbm, wd_hbm, out_hbm,
            xbuf,
            wbuf,
            xa,
            wa,
            wb,
            ha,
            mbuf,
            qkv,
            gbuf,
            x_sem, w_sem, out_sem):
    _, quarter, d = x_hbm.shape
    n_chunks, n_tiles = ha.shape[2], quarter // TILE
    hd, qd, groups = d // 2, d // 4, d // LANES

    def chunk_slot(c):
        return 1 + (c + 2) % 3

    q_slot, k_slot, v_slot, o_slot, down_slot = 0, 4, chunk_slot(1), chunk_slot(n_chunks), 2

    def x_copies(t):
        at = [(slice(None), pl.ds(t * TILE, TILE), pl.ds(col, hd)) for col in (0, hd)]
        return [pltpu.make_async_copy(x_hbm.at[i], xbuf.at[i], x_sem.at[t]) for i in at]

    def w_copy(slot, h, src=None, col=None):
        rows = pl.ds(0, d if src is None else src.shape[0])
        dst = wbuf.at[slot, pl.ds(h * (groups // 2), groups // 2), rows]
        return _ColumnCopy(src, col, dst, w_sem.at[2 * slot + h])

    def chunk_copies(c):
        return [w_copy(chunk_slot(c), h, w, _aligned(c * FCHUNK, FCHUNK)) for h, w in enumerate((wg_hbm, wu_hbm))]

    def down_copies(h):
        f = wd_hbm.shape[0]
        return [w_copy(down_slot + lo // d, h, wd_hbm.at[pl.ds(lo, min(d, f - lo))], _aligned(h * hd, hd))
                for lo in range(0, f, d)]

    def out_copies(t, h):
        return [pltpu.make_async_copy(
            wbuf.at[down_slot + i, g, pl.ds(h * quarter + t * TILE, TILE)],
            out_hbm.at[2 * h + i, pl.ds(t * TILE, TILE), pl.ds(g * LANES, LANES)],
            out_sem.at[2 * t + h]) for i in range(2) for g in range(groups)]

    xs = [x_copies(t) for t in range(n_tiles)]
    wq = [w_copy(q_slot, h, wqkv_hbm, h * hd) for h in range(2)]
    wk = [w_copy(k_slot, h, wqkv_hbm, d + h * hd) for h in range(2)]
    wv = [w_copy(v_slot, h, wqkv_hbm, 2 * d + h * hd) for h in range(2)]

    _start(*xs[0], wk[0])
    zero = lax.fori_loop(0, 2, lambda i, z: lax.min(i, z), 0)
    _start(*xs[1], wk[1])
    _wait(*xs[0])
    _start(*wv)

    never = {n: lax.broadcasted_iota(jnp.int32, (n, LANES), 0) < zero for n in (SUB, PACK, 2 * PACK)}
    lane = lax.broadcasted_iota(jnp.int32, (SUB, LANES), 1)
    lane_bit = {bit: (lane & bit) != 0 for bit in (1, 2, 4, 8, 16)}

    def after(token, x):
        if token is None:
            return x
        return lax.select(never[x.shape[0]], token(x.shape[0], x.dtype), x)

    def swap_group_and_lane_bits(cols, bits=3):
        cols = list(cols)
        for gbit, lbit in ((1, 4), (2, 8), (4, 16))[:bits]:
            for i in range(len(cols)):
                if not i & gbit:
                    a, b = cols[i], cols[i | gbit]
                    cols[i] = lax.select(lane_bit[lbit], pltpu.roll(b, lbit, 1), a)
                    cols[i | gbit] = lax.select(lane_bit[lbit], b, pltpu.roll(a, LANES - lbit, 1))
        return cols

    def operand_jobs(side, family, load, dst, first, row0, positions):
        def job(g, lo, token):
            operand = _operands(side, family, lambda r, c: load(r, c, g, lo, token))
            for j in range(7):
                dst[pl.ds(first, len(family)), j, g, pl.ds(row0 + lo, PACK), :] = _bf16(operand(j))

        return _jobs(job, positions)

    def left_jobs(load, row0, rows):
        return [job for family in LEFT_FAMILIES for job in operand_jobs(
            BALANCED_LEFT, family, lambda r, c, g, lo, token: after(token, load(r, 2 * c + g, lo)),
            xa, LEFT_ORDER.index(family[0]), row0, [(g, lo) for lo in rows for g in range(2)])]

    def right_jobs(slot, family, dst=wa, heads=False):
        family = RIGHT_FAMILIES[family]

        def load(r, c, g, lo, token):
            def rows(at):
                return _unpack(after(token, wbuf.bitcast(U32)[slot, 4 * g + c, pl.ds(at // 2, SUB)]))

            if heads:
                at = lo // PACK % 2 * hd + lo // (2 * PACK) * (2 * PACK) + r // 2 * PACK
                x = lax.concatenate([_rows(rows(at + i * qd), r % 2 * SUB, SUB) for i in range(2)], 0)
            else:
                x = rows(r * qd + lo)
            return _times(x, DELTA[r] / DELTA[c])

        return operand_jobs(BALANCED_RIGHT, family, load, dst, family[0] if dst is wa else 0, 0,
                            [(g, lo) for lo in range(0, qd, PACK) for g in range(2)])

    def move(i, j, g, lo, token):
        rows = pl.ds(lo, 4 * SUB)
        wa.bitcast(U32)[2 + i, j, g, rows, :] = after(token, wb.bitcast(U32)[i, j, g, rows, :])

    moves = _jobs(move, [(i, j, g, lo) for i in range(3) for j in range(7) for g in range(2)
                         for lo in range(0, qd // 2, 4 * SUB)])

    def refill_early(slot, last, **kw):
        return [(right_jobs(slot, 1, wb, **kw), max(last - 90, 23), max(last - 3, 62)),
                (right_jobs(slot, 0, **kw), last + 15.5, last + 46),
                (moves[:len(moves) // 2], last + 24, last + 47)]

    def refill_late(slot, **kw):
        return [(moves[len(moves) // 2:], 0, 22), (right_jobs(slot, 2, **kw), 0, 32)]

    def partial(slot, i, j, g, lo, n):
        if slot < 2:
            return mbuf, (slot, i, j, pl.ds(*g), pl.ds(lo, n))
        return gbuf, (1, j, pl.ds(i // 4 * 2 + g[0], g[1]), pl.ds(i % 4 * TILE + lo, n))

    def project(matmul, t, slot):
        for i in range(7):
            blocks = _balanced(lambda j: matmul(
                _load(xa, (LEFT_ORDER.index(i), j, slice(None)), t * TILE, TILE),
                _load(wa, (i, j, slice(None)), 0, qd)))
            for j, block in enumerate(blocks):
                ref, index = partial(slot, i, j, (0, 2), 0, TILE)
                ref[index] = _stack(_lane_groups(block))

    def finish_jobs(slot, n, use, quadrants=range(4)):
        def job(lo, j, g, token):
            def product(i):
                ref, index = partial(slot, i, j, g, lo, n)
                return after(None if i else token, lax.reshape(ref[index], (PACK, LANES)))

            out = _balanced(product)
            for i in quadrants:
                use(*_position(i, j), g[0], lo, out[i])

        return _jobs(job, [(lo, j, g) for lo in range(0, TILE, n) for j in range(4)
                           for g in (((0, 1), (1, 1)) if n == PACK else ((0, 2),))])

    def during(step):
        return 49 * step, 49 * step + 48

    def norm(q, lo, scaled, plain, token):
        def rows(lo):
            first, *rest = _lane_groups(lax.convert_element_type(xbuf[q, pl.ds(lo, SUB), :], F32))
            x = lax.concatenate([after(token, first)] + rest, 1)
            x = x - jnp.sum(x, axis=-1, keepdims=True) * (1.0 / d)
            inv = lax.rsqrt(jnp.sum(x * x, axis=-1, keepdims=True) * (1.0 / d) + LN_EPS)
            inv = lax.broadcast_in_dim(inv, (SUB, LANES), (0, 1))
            return [lax.mul(v, _times(inv, DELTA[q] / DELTA[g // 2] if scaled else 1.0))
                    for g, v in enumerate(_lane_groups(x))]

        if scaled:
            gbuf[:, :, q, pl.ds(lo, SUB), :] = lax.reshape(_stack(rows(lo)), (2, 4, SUB, LANES))
        if plain and lo % PACK:
            lo -= SUB
            cols = ([_times(gbuf[g // 4, g % 4, q, pl.ds(lo, PACK), :], DELTA[g // 2] / DELTA[q])
                     for g in range(groups)] if scaled else
                    [lax.concatenate(v, 0) for v in zip(rows(lo), rows(lo + SUB))])
            for g, v in enumerate(cols):
                ha[lo // TILE, g // 4, g % 4, pl.ds(q * TILE + lo % TILE, PACK), :] = _bf16(v)

    def norm_jobs(t, scaled=True, plain=False):
        return _jobs(norm, [(q, t * TILE + lo, scaled, plain)
                            for q in range(4) for lo in range(0, TILE, SUB)])

    def split_x_jobs(t):
        return left_jobs(lambda q, g, lo: gbuf[g // 4, g % 4, q, pl.ds(lo, PACK), :],
                         0, range(t * TILE, (t + 1) * TILE, PACK))

    def shuffle_weight_jobs(slot):
        words = wbuf.bitcast(U32)

        def job(lo, token):
            at = (slot, slice(None), pl.ds(lo // 2, SUB))
            words[at] = _stack(swap_group_and_lane_bits([after(token, v) for v in _unstack(words[at])]))

        return _jobs(job, [(lo + r * qd,) for lo in range(0, qd, PACK) for r in range(4)])

    def plain_k(t, gs, *plan):
        matmul = _Matmuls(*plan)
        for g in gs:
            k = lax.add(*[matmul(_load(ha, (t, h, pl.ds(0, 4)), 0, 4 * TILE),
                                 _load(wbuf, (k_slot, pl.ds(g, 1)), h * hd, hd)) for h in range(2)])
            k = pltpu.bitcast(_bf16(k), F32)
            for lo in range(0, 4 * TILE, PACK):
                row = HALO + lo // TILE * quarter + t * TILE + lo % TILE
                qkv[1, g, pl.ds(row, SUB), :] = _rows(k, lo // 2, SUB)

    def shuffle_k(row, token):
        cols = [after(token, v) for v in _unstack(pltpu.bitcast(qkv[1, :, pl.ds(row, SUB), :], U32))]
        qkv[1, :, pl.ds(row, PACK), :] = _unpack(_stack(swap_group_and_lane_bits(cols)))

    def finish_qkv(p, t, slot):
        def use(r, c, _, lo, x):
            x = _times(x, _unscale(r, c))
            for g in range(2):
                qkv[p, 4 * g + c, pl.ds(HALO + r * quarter + t * TILE + lo, SUB), :] = _rows(x, g * SUB, SUB)

        return finish_jobs(slot, SUB, use)

    for job in norm_jobs(0, plain=True):
        job(None)
    wk[0].wait()
    _start(*xs[2], *xs[3])
    plain_k(0, range(4), (split_x_jobs(0), 0, 7))
    _wait(*xs[1], wk[1])
    _start(*wq, *chunk_copies(0))
    plain_k(0, range(4, 8), (norm_jobs(1, plain=True), 0, 6.5))
    _wait(*wv)
    plain_k(1, range(8), (shuffle_weight_jobs(v_slot), 0, 13.5),
            *[(right_jobs(v_slot, f), 1.5, 15.5) for f in range(3)])
    _start(*chunk_copies(1))
    _wait(*xs[2], *xs[3])
    matmul = _Matmuls((norm_jobs(2) + norm_jobs(3), 0, 44), (split_x_jobs(1)[:32], 0, 47))
    project(matmul, 0, 0)
    _wait(*wq)
    matmul = _Matmuls(
        (split_x_jobs(1)[32:], 0, 19), (split_x_jobs(2), *during(0)), (split_x_jobs(3), *during(1)),
        *[(finish_qkv(2, t, t % 2), *during(t)) for t in range(3)],
        (shuffle_weight_jobs(k_slot), 0, 96),
        (right_jobs(k_slot, 1, wb), 98, 119), (right_jobs(k_slot, 0), 119, 146),
        (moves[:len(moves) // 2], 121, 146))
    project(matmul, 1, 1)
    project(matmul, 2, 0)

    @pl.loop(0, 2)
    def _(h):
        w_copy(chunk_slot(0), h).wait()

    project(matmul, 3, 1)
    matmul = _Matmuls(
        *refill_late(k_slot), *refill_early(chunk_slot(0), 49),
        (shuffle_weight_jobs(q_slot), 0, 92),
        (finish_qkv(2, 3, 1), *during(0)), (finish_qkv(1, 2, 0), *during(1)))
    project(matmul, 2, 0)
    project(matmul, 3, 2)

    def geglu_jobs(t):
        def use(r, c, _, lo, x):
            gbuf[0, c, r, pl.ds(t * TILE + lo, SUB), :] = _geglu(
                _rows(x, 0, SUB), _rows(x, SUB, SUB), _unscale(r, c))

        return finish_jobs(t % 2, SUB, use)

    def split_hidden_jobs(chunk, t):
        return [job for lo in range(t * TILE, (t + 1) * TILE, PACK)
                for family in ((0, 1), (2, 3), (4,), (5,), (6,)) for job in operand_jobs(
                    STRASSEN_LEFT, family,
                    lambda r, c, g, lo, token: after(token, gbuf[0, c, r, pl.ds(lo, PACK), :]),
                    ha, family[0], 0, [(chunk, lo)])]

    @pl.loop(0, n_chunks)
    def _(c):
        pl.when(c + 1 < n_chunks)(lambda: _wait(*chunk_copies(c + 1)))
        pl.when(c + 2 < n_chunks)(lambda: _start(*chunk_copies(c + 2)))
        pl.when(c + 2 == n_chunks)(
            lambda: _start(*[w_copy(o_slot, h, wo_hbm, h * hd) for h in range(2)]))
        previous = jnp.maximum(c - 1, 0)
        following = jnp.where(c + 1 < n_chunks, chunk_slot(c + 1), q_slot)
        matmul = _Matmuls(
            *refill_late(chunk_slot(c)), *refill_early(following, 147),
            *[(geglu_jobs((t - 1) % n_tiles), *during(t)) for t in range(n_tiles)],
            (split_hidden_jobs(previous, 2), 30, 60), (split_hidden_jobs(previous, 3), 60, 98),
            (split_hidden_jobs(c, 0), 98, 145), (split_hidden_jobs(c, 1), 145, 160))
        for t in range(n_tiles):
            project(matmul, t, t % 2)

    @pl.loop(0, 2)
    def _(h):
        w_copy(o_slot, h).wait()
        _start(*down_copies(h))

    matmul = _Matmuls(
        *refill_late(q_slot), *refill_early(o_slot, 147, heads=True),
        (split_hidden_jobs(n_chunks - 1, 2), 30, 60), (split_hidden_jobs(n_chunks - 1, 3), 60, 98),
        (finish_qkv(1, 3, 2), 49, 147),
        (_jobs(shuffle_k, [(HALO + q * quarter + lo,) for lo in range(0, PLAIN * TILE, PACK)
                           for q in range(4)]), 35, 165),
        (geglu_jobs(n_tiles - 1), *during(0)),
        *[(finish_qkv(0, t, t % 2), *during(t + 1)) for t in range(n_tiles - 1)])
    for t in range(n_tiles):
        project(matmul, t, t % 2)
    for job in finish_qkv(0, n_tiles - 1, 1):
        job(None)

    for p in (1, 2):
        for g in range(groups):
            qkv[p, g, pl.ds(0, HALO), :] = jnp.broadcast_to(qkv[p, g, pl.ds(HALO, 1), :], (HALO, LANES))

    scale = float(d // N_HEADS) ** -0.5

    def attend(row0, q, lo, token):
        off = q * quarter + lo

        def load(p, w):
            return qkv[p, :, pl.ds(row0 + (HALO + off - DILATION * w), SUB), :]

        first, *rest = _unstack(load(0, 0))
        query = _stack([after(token, first)] + rest)
        logits = []
        for w in range(WINDOW):
            s = lax.reduce_sum(lax.mul(query, load(1, w)), (0,))
            for bit in (1, 2):
                other = lax.select(lane_bit[bit], pltpu.roll(s, bit, 1), pltpu.roll(s, LANES - bit, 1))
                s = lax.add(s, other)
            if off < DILATION * w:
                row = row0 + off + lax.broadcasted_iota(jnp.int32, (SUB, LANES), 0)
                s = jnp.where(row >= DILATION * w, s, MASKED_LOGIT / scale)
            logits.append(s)
        top = functools.reduce(lax.max, logits)
        weights = [lax.exp2(_times(lax.sub(s, top), scale * np.log2(np.e))) for s in logits]
        inv = lax.div(np.float32(1), functools.reduce(lax.add, weights))
        out = functools.reduce(lax.add, [
            lax.mul(lax.broadcast(weights[w], (groups,)), load(2, w)) for w in range(WINDOW)])
        out = [lax.mul(v, _times(inv, DELTA[q] / DELTA[g // 2])) for g, v in enumerate(_unstack(out))]
        mbuf[1, q, :, :, pl.ds(lo % (2 * PACK), SUB), :] = lax.reshape(
            _stack(swap_group_and_lane_bits(out, 1)), (4, 2, SUB, LANES))

    _wait(*down_copies(0), *down_copies(1))

    @pl.loop(0, n_tiles)
    def _(step):
        row0 = pl.multiple_of(step * TILE, TILE)
        plan = []
        for lo in range(0, TILE, PACK):
            first, last = 43 * lo / TILE, 43 * (lo + PACK) / TILE
            plan += [
                (_jobs(attend, [(row0, q, lo + i) for q in range(4) for i in (0, SUB)]), first, last),
                (left_jobs(lambda q, g, lo: mbuf[1, q, g // 2, g % 2, pl.ds(lo % (2 * PACK), PACK), :],
                           row0, [lo]), last + 1, last + 5)]
        matmul = _Matmuls(*plan)
        row0 = pl.multiple_of(step // 2 * (2 * TILE), 2 * TILE)
        for i in range(7):
            half = (step + 2 * i) % 2
            right = _operands(STRASSEN_RIGHT, [i], lambda r, c: lax.concatenate(
                [_unpack(wbuf.bitcast(U32)[down_slot + n // 2, 4 * half + c,
                                           pl.ds((n % 2 * FCHUNK + r * LANES) // 2, LANES // 2), :])
                 for n in range(n_chunks)], 0))
            blocks = _strassen(lambda j: matmul(
                _load(ha, (i, j, slice(None)), row0, 2 * TILE), _bf16(_unstack(right(j))[0])))
            for j, block in enumerate(blocks):
                mbuf[0, i, j] = lax.reshape(block, (2, TILE, LANES))
        for j in range(4):
            blocks = _strassen(lambda i: lax.reshape(mbuf[0, i, j], (2 * TILE, LANES)))
            for i, block in enumerate(blocks):
                r, c = _position(i, j)
                gbuf[step % 2, c, r, pl.ds(row0, 2 * TILE), :] = _silu(block, _unscale(r, c))

    def output_jobs(t, quadrants=range(4)):
        def use(r, c, g, lo, attn):
            rows = pl.ds(t * TILE + lo, PACK)
            x = lax.convert_element_type(xbuf[r, rows, pl.ds(g * hd + c * LANES, LANES)], F32)
            group = 4 * g + c + (zero if lo == g == r % 2 == c % 2 == 0 else 0)
            wbuf[down_slot + r % 2, group, pl.ds(r // 2 * quarter + t * TILE + lo, PACK), :] = (
                _bf16(lax.add(x, lax.mul(attn, gbuf[g, c, r, rows, :]))))

        def send(token):
            _start(*[cp for h in range(2) if 3 * h in quadrants for cp in out_copies(t, h)])
            if quadrants == [0]:
                wbuf.bitcast(U32)[down_slot, zero, pl.ds((quarter + t * TILE) // 2, SUB), :] = token(SUB, U32)

        return finish_jobs(1 - t % 2, PACK, use, quadrants) + [send]

    matmul = _Matmuls(
        *refill_late(o_slot, heads=True),
        (output_jobs(0), *during(1)), (output_jobs(1), *during(2)),
        (output_jobs(2), 147, 176), (output_jobs(3, [1]), 176, 182), (output_jobs(3, [0]), 182, 188))
    for t in range(n_tiles):
        project(matmul, t, 1 - t % 2)
    for job in output_jobs(3, [2, 3]):
        job(None)
    _wait(*[cp for t in range(n_tiles) for h in range(2) for cp in out_copies(t, h)])


@jax.jit
def pallas_recurrent_scan__sliding_local_dilated__geglu_ffn__prompt_kernel(
    A_x: jax.Array,
    A_wqkv: jax.Array,
    A_wo: jax.Array,
    B_x: jax.Array,
    B_w_gate: jax.Array,
    B_w_up: jax.Array,
    B_w_down: jax.Array,
):
    del B_x
    b, s, d = A_x.shape
    f = B_w_gate.shape[1]
    assert (b, s, d, f) == (1, 16 * TILE, 8 * LANES, 7 * FCHUNK) and A_x.dtype == BF16
    quarter, groups = s // 4, d // LANES

    hbm = pl.BlockSpec(memory_space=pl.ANY)
    out = pl.pallas_call(
        _kernel,
        out_shape=jax.ShapeDtypeStruct((4, quarter, d), BF16),
        in_specs=[hbm] * 6,
        out_specs=hbm,
        scratch_shapes=[
            pltpu.VMEM((4, quarter, d), BF16),
            pltpu.VMEM((6, groups, d, LANES), BF16),
            pltpu.VMEM((7, 7, 2, quarter, LANES), BF16),
            pltpu.VMEM((7, 7, 2, d // 4, LANES), BF16),
            pltpu.VMEM((3, 7, 2, d // 4, LANES), BF16),
            pltpu.VMEM((7, 7, f // FCHUNK, quarter, LANES), BF16),
            pltpu.VMEM((2, 7, 4, 2, TILE, LANES), F32),
            pltpu.VMEM((3, groups, HALO + s, LANES), F32),
            pltpu.VMEM((2, 4, 4, quarter, LANES), F32),
            pltpu.SemaphoreType.DMA((4,)),
            pltpu.SemaphoreType.DMA((12,)),
            pltpu.SemaphoreType.DMA((8,)),
        ],
        compiler_params=pltpu.CompilerParams(
            vmem_limit_bytes=127 * 1024 * 1024, disable_bounds_checks=True),
        name="fused_local_attn_geglu",
    )(A_x.reshape(4, quarter, d), A_wqkv, A_wo, B_w_gate, B_w_up, B_w_down)
    return out.reshape(b, s, d)
```

```python
import functools

import jax
import jax.numpy as jnp
import numpy as np
from jax import lax
import jax.experimental.pallas as pl
import jax.experimental.pallas.tpu as pltpu

F32 = jnp.float32
BF16 = jnp.bfloat16
U32 = jnp.uint32

N_HEADS = 32
WINDOW = 8
DILATION = 2
LN_EPS = 1e-5
MASKED_LOGIT = -1e9

LANES = 128
SUB = 8
PACK = 16
HALO = 16
FCHUNK = 512
TILE = 128
PLAIN = 2


STRASSEN_LEFT = ("c+d", "d", "a+b", "a", "t", "c-a", "b-d")
STRASSEN_RIGHT = ("a", "c-a", "d", "b-d", "t", "a+b", "c+d")


def _strassen(m):
    m0, m1 = m(0), m(1)
    c = lax.add(m0, m1)
    m2, m3 = m(2), m(3)
    b = lax.add(m2, m3)
    m4 = m(4)
    d = lax.add(lax.add(m4, lax.sub(m3, m0)), m(5))
    a = lax.add(lax.add(m4, lax.sub(m1, m2)), m(6))
    return a, b, c, d


BALANCED_LEFT = ("a-b", "a+b", "t+t", "d-b", "d+b", "t-s", "t+s")
BALANCED_RIGHT = ("d-b", "d+b", "t", "t+s", "t-s", "a+b", "a-b")
LEFT_FAMILIES = ((0, 1), (2, 5, 6), (3, 4))
LEFT_ORDER = sum(LEFT_FAMILIES, ())
RIGHT_FAMILIES = ((0, 1), (2, 3, 4), (5, 6))
DELTA = (1.0, 3.0 ** 0.5, 3.0 ** 0.5, 3.0)


def _balanced(m):
    m0, m1 = m(0), m(1)
    b = lax.sub(m1, m0)
    diag = lax.sub(m(2), lax.add(m0, m1))
    m3, m4 = m(3), m(4)
    a = lax.sub(diag, lax.add(m3, m4))
    low = lax.add(b, lax.sub(m3, m4))
    m5, m6 = m(5), m(6)
    return a, b, lax.add(low, lax.sub(m6, m5)), lax.sub(diag, lax.add(m5, m6))


def _unscale(r, c):
    return DELTA[c] / DELTA[r] / 4


def _position(outer, inner):
    return outer // 2 * 2 + inner // 2, outer % 2 * 2 + inner % 2


def _combinations(quadrant):
    @functools.cache
    def term(name):
        if len(name) == 3:
            return (lax.add if name[1] == "+" else lax.sub)(term(name[0]), term(name[2]))
        if name in "ts":
            return term("a+d" if name == "t" else "b+c")
        return quadrant("abcd".index(name))

    return term


def _operands(side, family, block):
    outer = _combinations(lambda i: _stack([block(*_position(i, j)) for j in range(4)]))
    parts = _stack([outer(side[i]) for i in family])
    inner = _combinations(lambda j: lax.index_in_dim(parts, j, 1, keepdims=False))
    return lambda j: inner(side[j])


def _token(value, row, n, dtype):
    x = lax.slice(value, (row, 0), (row + SUB, LANES))
    return lax.concatenate([x if dtype == x.dtype else pltpu.bitcast(x, dtype)] * (n // SUB), 0)


class _Matmuls:
    def __init__(self, *plan):
        self.calls = 0
        self.jobs = sorted(
            ((first + (last - first) * (i + 0.618 * n % 1) / len(jobs), n, job)
             for n, (jobs, first, last) in enumerate(plan) for i, job in enumerate(jobs)),
            key=lambda t: t[:2], reverse=True)

    def __call__(self, lhs, rhs):
        value = lax.dot_general(lhs, rhs, (((1,), (0,)), ((), ())), preferred_element_type=F32)
        while self.jobs and self.jobs[-1][0] < self.calls + 1:
            when, _, job = self.jobs.pop()
            row = int((when - self.calls) * (value.shape[0] // SUB)) * SUB
            job(functools.cache(functools.partial(_token, value, row)))
        self.calls += 1
        return value


def _jobs(fn, args):
    return [functools.partial(fn, *a) for a in args]


def _times(x, c):
    return x if c == 1.0 else lax.mul(x, np.float32(c))


def _plus(x, c):
    return lax.add(x, np.float32(c))


def _aligned(i, n):
    return i if isinstance(i, int) else pl.multiple_of(i, n)


def _stack(xs):
    return lax.reshape(lax.concatenate(xs, 0), (len(xs), *xs[0].shape))


def _unstack(x):
    return [lax.index_in_dim(x, i, 0, keepdims=False) for i in range(x.shape[0])]


def _rows(x, lo, n):
    return lax.slice_in_dim(x, lo, lo + n, axis=0)


def _lane_groups(x):
    return [lax.slice_in_dim(x, j, j + LANES, axis=1) for j in range(0, x.shape[1], LANES)]


def _bf16(x):
    return lax.convert_element_type(x, BF16)


def _unpack(words):
    return lax.convert_element_type(pltpu.bitcast(words, BF16), F32)


def _geglu(g, u, scale):
    k0 = (2 / np.pi) ** 0.5
    t = lax.tanh(lax.mul(g, _plus(_times(lax.mul(g, g), k0 * 0.044715 * scale ** 3), k0 * scale)))
    return lax.mul(lax.mul(_times(g, 0.5 * scale ** 2), u), _plus(t, 1.0))


def _silu(x, scale):
    h = _times(x, 0.5)
    return lax.mul(_times(h, scale), _plus(lax.tanh(h), 1.0))


def _load(ref, index, lo, n):
    words = ref.bitcast(U32)[(*index, pl.ds(_aligned(lo // 2, SUB), n // 2))]
    return lax.concatenate(_unstack(pltpu.bitcast(words, BF16)), 1)


class _ColumnCopy:
    def __init__(self, src, col, dst, sem):
        self.src, self.col, self.dst, self.sem = src, col, dst, sem

    def start(self):
        for g in range(self.dst.shape[0]):
            cols = pl.ds(self.col + g * LANES, LANES)
            pltpu.make_async_copy(self.src.at[:, cols], self.dst.at[g], self.sem).start()

    def wait(self):
        pltpu.make_async_copy(self.dst, self.dst, self.sem).wait()


def _start(*copies):
    for cp in copies:
        cp.start()


def _wait(*copies):
    for cp in copies:
        cp.wait()


def _kernel(x_hbm, wqkv_hbm, wo_hbm, wg_hbm, wu_hbm, wd_hbm, out_hbm,
            xbuf,
            wbuf,
            xa,
            wa,
            wb,
            ha,
            mbuf,
            qkv,
            gbuf,
            x_sem, w_sem, out_sem):
    _, quarter, d = x_hbm.shape
    n_chunks, n_tiles = ha.shape[2], quarter // TILE
    hd, qd, groups = d // 2, d // 4, d // LANES

    def chunk_slot(c):
        return 1 + (c + 2) % 3

    q_slot, k_slot, v_slot, o_slot, down_slot = 0, 4, chunk_slot(1), chunk_slot(n_chunks), 2

    def x_copies(t):
        at = [(slice(None), pl.ds(t * TILE, TILE), pl.ds(col, hd)) for col in (0, hd)]
        return [pltpu.make_async_copy(x_hbm.at[i], xbuf.at[i], x_sem.at[t]) for i in at]

    def w_copy(slot, h, src=None, col=None):
        rows = pl.ds(0, d if src is None else src.shape[0])
        dst = wbuf.at[slot, pl.ds(h * (groups // 2), groups // 2), rows]
        return _ColumnCopy(src, col, dst, w_sem.at[2 * slot + h])

    def chunk_copies(c):
        return [w_copy(chunk_slot(c), h, w, _aligned(c * FCHUNK, FCHUNK)) for h, w in enumerate((wg_hbm, wu_hbm))]

    def down_copies(h):
        f = wd_hbm.shape[0]
        return [w_copy(down_slot + lo // d, h, wd_hbm.at[pl.ds(lo, min(d, f - lo))], _aligned(h * hd, hd))
                for lo in range(0, f, d)]

    def staged(q, g, lo, n):
        return down_slot + q % 2, g, pl.ds(q // 2 * quarter + lo, n)

    def out_copies(t, q):
        return [pltpu.make_async_copy(
            wbuf.at[staged(q, g, t * TILE, TILE)],
            out_hbm.at[q, pl.ds(t * TILE, TILE), pl.ds(g * LANES, LANES)],
            out_sem) for g in range(groups)]

    xs = [x_copies(t) for t in range(n_tiles)]
    wq = [w_copy(q_slot, h, wqkv_hbm, h * hd) for h in range(2)]
    wk = [w_copy(k_slot, h, wqkv_hbm, d + h * hd) for h in range(2)]
    wv = [w_copy(v_slot, h, wqkv_hbm, 2 * d + h * hd) for h in range(2)]

    _start(*xs[0], wk[0])
    zero = lax.fori_loop(0, 2, lambda i, z: lax.min(i, z), 0)
    _start(*xs[1], wk[1])
    _wait(*xs[0])
    _start(*wv)

    never = {n: lax.broadcasted_iota(jnp.int32, (n, LANES), 0) < zero for n in (SUB, PACK, 2 * PACK)}
    lane = lax.broadcasted_iota(jnp.int32, (SUB, LANES), 1)
    lane_bit = {bit: (lane & bit) != 0 for bit in (1, 2, 4, 8, 16)}

    def after(token, x):
        if token is None:
            return x
        return lax.select(never[x.shape[0]], token(x.shape[0], x.dtype), x)

    def swap_group_and_lane_bits(cols, bits=3):
        cols = list(cols)
        for gbit, lbit in ((1, 4), (2, 8), (4, 16))[:bits]:
            for i in range(len(cols)):
                if not i & gbit:
                    a, b = cols[i], cols[i | gbit]
                    cols[i] = lax.select(lane_bit[lbit], pltpu.roll(b, lbit, 1), a)
                    cols[i | gbit] = lax.select(lane_bit[lbit], b, pltpu.roll(a, LANES - lbit, 1))
        return cols

    def operand_jobs(side, family, load, dst, first, row0, positions):
        def job(g, lo, token):
            operand = _operands(side, family, lambda r, c: load(r, c, g, lo, token))
            for j in range(7):
                dst[pl.ds(first, len(family)), j, g, pl.ds(row0 + lo, PACK), :] = _bf16(operand(j))

        return _jobs(job, positions)

    def left_jobs(load, row0, rows):
        return [job for family in LEFT_FAMILIES for job in operand_jobs(
            BALANCED_LEFT, family, lambda r, c, g, lo, token: after(token, load(r, 2 * c + g, lo)),
            xa, LEFT_ORDER.index(family[0]), row0, [(g, lo) for lo in rows for g in range(2)])]

    def right_jobs(slot, family, dst=wa, heads=False):
        family = RIGHT_FAMILIES[family]

        def load(r, c, g, lo, token):
            def rows(at):
                return _unpack(after(token, wbuf.bitcast(U32)[slot, 4 * g + c, pl.ds(at // 2, SUB)]))

            if heads:
                at = lo // PACK % 2 * hd + lo // (2 * PACK) * (2 * PACK) + r // 2 * PACK
                x = lax.concatenate([_rows(rows(at + i * qd), r % 2 * SUB, SUB) for i in range(2)], 0)
            else:
                x = rows(r * qd + lo)
            return _times(x, DELTA[r] / DELTA[c])

        return operand_jobs(BALANCED_RIGHT, family, load, dst, family[0] if dst is wa else 0, 0,
                            [(g, lo) for lo in range(0, qd, PACK) for g in range(2)])

    def move(i, j, g, lo, token):
        rows = pl.ds(lo, 4 * SUB)
        wa.bitcast(U32)[2 + i, j, g, rows, :] = after(token, wb.bitcast(U32)[i, j, g, rows, :])

    moves = _jobs(move, [(i, j, g, lo) for i in range(3) for j in range(7) for g in range(2)
                         for lo in range(0, qd // 2, 4 * SUB)])

    def refill_early(slot, last, **kw):
        return [(right_jobs(slot, 1, wb, **kw), max(last - 90, 23), max(last - 3, 62)),
                (right_jobs(slot, 0, **kw), last + 15.5, last + 46),
                (moves[:len(moves) // 2], last + 24, last + 47)]

    def refill_late(slot, **kw):
        return [(moves[len(moves) // 2:], 0, 22), (right_jobs(slot, 2, **kw), 0, 32)]

    def partial(slot, i, j, g, lo, n):
        if slot < 2:
            return mbuf, (slot, i, j, pl.ds(*g), pl.ds(lo, n))
        return gbuf, (1, j, pl.ds(i // 4 * 2 + g[0], g[1]), pl.ds(i % 4 * TILE + lo, n))

    def project(matmul, t, slot):
        for i in range(7):
            blocks = _balanced(lambda j: matmul(
                _load(xa, (LEFT_ORDER.index(i), j, slice(None)), t * TILE, TILE),
                _load(wa, (i, j, slice(None)), 0, qd)))
            for j, block in enumerate(blocks):
                ref, index = partial(slot, i, j, (0, 2), 0, TILE)
                ref[index] = _stack(_lane_groups(block))

    def finish_jobs(slot, n, use, outer=range(4), inner=range(4)):
        def job(lo, j, g, token):
            def product(i):
                ref, index = partial(slot, i, j, g, lo, n)
                return after(None if i else token, lax.reshape(ref[index], (PACK, LANES)))

            out = _balanced(product)
            for i in outer:
                use(*_position(i, j), g[0], lo, out[i])

        return _jobs(job, [(lo, j, g) for lo in range(0, TILE, n) for j in inner
                           for g in (((0, 1), (1, 1)) if n == PACK else ((0, 2),))])

    def during(step):
        return 49 * step, 49 * step + 48

    def norm(q, lo, scaled, plain, token):
        def rows(lo):
            first, *rest = _lane_groups(lax.convert_element_type(xbuf[q, pl.ds(lo, SUB), :], F32))
            x = lax.concatenate([after(token, first)] + rest, 1)
            x = x - jnp.sum(x, axis=-1, keepdims=True) * (1.0 / d)
            inv = lax.rsqrt(jnp.sum(x * x, axis=-1, keepdims=True) * (1.0 / d) + LN_EPS)
            inv = lax.broadcast_in_dim(inv, (SUB, LANES), (0, 1))
            return [lax.mul(v, _times(inv, DELTA[q] / DELTA[g // 2] if scaled else 1.0))
                    for g, v in enumerate(_lane_groups(x))]

        if scaled:
            gbuf[:, :, q, pl.ds(lo, SUB), :] = lax.reshape(_stack(rows(lo)), (2, 4, SUB, LANES))
        if plain and lo % PACK:
            lo -= SUB
            cols = ([_times(gbuf[g // 4, g % 4, q, pl.ds(lo, PACK), :], DELTA[g // 2] / DELTA[q])
                     for g in range(groups)] if scaled else
                    [lax.concatenate(v, 0) for v in zip(rows(lo), rows(lo + SUB))])
            for g, v in enumerate(cols):
                ha[lo // TILE, g // 4, g % 4, pl.ds(q * TILE + lo % TILE, PACK), :] = _bf16(v)

    def norm_jobs(t, scaled=True, plain=False):
        return _jobs(norm, [(q, t * TILE + lo, scaled, plain)
                            for q in range(4) for lo in range(0, TILE, SUB)])

    def split_x_jobs(t):
        return left_jobs(lambda q, g, lo: gbuf[g // 4, g % 4, q, pl.ds(lo, PACK), :],
                         0, range(t * TILE, (t + 1) * TILE, PACK))

    def shuffle_weight_jobs(slot):
        words = wbuf.bitcast(U32)

        def job(lo, token):
            at = (slot, slice(None), pl.ds(lo // 2, SUB))
            words[at] = _stack(swap_group_and_lane_bits([after(token, v) for v in _unstack(words[at])]))

        return _jobs(job, [(lo + r * qd,) for lo in range(0, qd, PACK) for r in range(4)])

    def plain_k(t, gs, *plan):
        matmul = _Matmuls(*plan)
        for g in gs:
            k = lax.add(*[matmul(_load(ha, (t, h, pl.ds(0, 4)), 0, 4 * TILE),
                                 _load(wbuf, (k_slot, pl.ds(g, 1)), h * hd, hd)) for h in range(2)])
            k = pltpu.bitcast(_bf16(k), F32)
            for lo in range(0, 4 * TILE, PACK):
                row = HALO + lo // TILE * quarter + t * TILE + lo % TILE
                qkv[1, g, pl.ds(row, SUB), :] = _rows(k, lo // 2, SUB)

    def shuffle_k(row, token):
        cols = [after(token, v) for v in _unstack(pltpu.bitcast(qkv[1, :, pl.ds(row, SUB), :], U32))]
        qkv[1, :, pl.ds(row, PACK), :] = _unpack(_stack(swap_group_and_lane_bits(cols)))

    def finish_qkv(p, t, slot):
        def use(r, c, _, lo, x):
            x = _times(x, _unscale(r, c))
            for g in range(2):
                qkv[p, 4 * g + c, pl.ds(HALO + r * quarter + t * TILE + lo, SUB), :] = _rows(x, g * SUB, SUB)

        return finish_jobs(slot, SUB, use)

    for job in norm_jobs(0, plain=True):
        job(None)
    wk[0].wait()
    _start(*xs[2], *xs[3])
    plain_k(0, range(4), (split_x_jobs(0), 0, 7))
    _wait(*xs[1], wk[1])
    _start(*wq, *chunk_copies(0))
    plain_k(0, range(4, 8), (norm_jobs(1, plain=True), 0, 6.5))
    _wait(*wv)
    plain_k(1, range(8), (shuffle_weight_jobs(v_slot), 0, 13.5),
            *[(right_jobs(v_slot, f), 1.5, 15.5) for f in range(3)])
    _start(*chunk_copies(1))
    _wait(*xs[2], *xs[3])
    matmul = _Matmuls((norm_jobs(2) + norm_jobs(3), 0, 42), (split_x_jobs(1)[:28], 0, 48))
    project(matmul, 0, 0)
    _wait(*wq)
    matmul = _Matmuls(
        (split_x_jobs(1)[28:], 0, 19), (split_x_jobs(2), 0, 49), (split_x_jobs(3), 49, 97.5),
        *[(finish_qkv(2, t, t % 2), *during(t)) for t in range(3)],
        (shuffle_weight_jobs(k_slot), 0, 96),
        (right_jobs(k_slot, 1, wb), 98, 119), (right_jobs(k_slot, 0), 119, 146),
        (moves[:len(moves) // 2], 121, 146))
    project(matmul, 1, 1)
    project(matmul, 2, 0)

    @pl.loop(0, 2)
    def _(h):
        w_copy(chunk_slot(0), h).wait()

    project(matmul, 3, 1)
    matmul = _Matmuls(
        *refill_late(k_slot), *refill_early(chunk_slot(0), 49),
        (shuffle_weight_jobs(q_slot), 0, 92),
        (finish_qkv(2, 3, 1), *during(0)), (finish_qkv(1, 2, 0), *during(1)))
    project(matmul, 2, 0)
    project(matmul, 3, 2)

    def geglu_jobs(t):
        def use(r, c, _, lo, x):
            gbuf[0, c, r, pl.ds(t * TILE + lo, SUB), :] = _geglu(
                _rows(x, 0, SUB), _rows(x, SUB, SUB), _unscale(r, c))

        return finish_jobs(t % 2, SUB, use)

    def split_hidden_jobs(chunk, t):
        return [job for lo in range(t * TILE, (t + 1) * TILE, PACK)
                for family in ((0, 1), (2, 3), (4,), (5,), (6,)) for job in operand_jobs(
                    STRASSEN_LEFT, family,
                    lambda r, c, g, lo, token: after(token, gbuf[0, c, r, pl.ds(lo, PACK), :]),
                    ha, family[0], 0, [(chunk, lo)])]

    @pl.loop(0, n_chunks)
    def _(c):
        pl.when(c + 1 < n_chunks)(lambda: _wait(*chunk_copies(c + 1)))
        pl.when(c + 2 < n_chunks)(lambda: _start(*chunk_copies(c + 2)))
        pl.when(c + 2 == n_chunks)(
            lambda: _start(*[w_copy(o_slot, h, wo_hbm, h * hd) for h in range(2)]))
        previous = jnp.maximum(c - 1, 0)
        following = jnp.where(c + 1 < n_chunks, chunk_slot(c + 1), q_slot)
        matmul = _Matmuls(
            *refill_late(chunk_slot(c)), *refill_early(following, 147),
            *[(geglu_jobs((t - 1) % n_tiles), *during(t)) for t in range(n_tiles)],
            (split_hidden_jobs(previous, 2), 30, 60), (split_hidden_jobs(previous, 3), 60, 98),
            (split_hidden_jobs(c, 0), 98, 145), (split_hidden_jobs(c, 1), 145, 160))
        for t in range(n_tiles):
            project(matmul, t, t % 2)

    @pl.loop(0, 2)
    def _(h):
        w_copy(o_slot, h).wait()
        _start(*down_copies(h))

    matmul = _Matmuls(
        *refill_late(q_slot), *refill_early(o_slot, 147, heads=True),
        (split_hidden_jobs(n_chunks - 1, 2), 30, 60), (split_hidden_jobs(n_chunks - 1, 3), 60, 98),
        (finish_qkv(1, 3, 2), 49, 147),
        (_jobs(shuffle_k, [(HALO + q * quarter + lo,) for lo in range(0, PLAIN * TILE, PACK)
                           for q in range(4)]), 35, 165),
        (geglu_jobs(n_tiles - 1), *during(0)),
        *[(finish_qkv(0, t, t % 2), *during(t + 1)) for t in range(n_tiles - 1)])
    for t in range(n_tiles):
        project(matmul, t, t % 2)
    for job in finish_qkv(0, n_tiles - 1, 1):
        job(None)

    for p in (1, 2):
        for g in range(groups):
            qkv[p, g, pl.ds(0, HALO), :] = jnp.broadcast_to(qkv[p, g, pl.ds(HALO, 1), :], (HALO, LANES))

    scale = float(d // N_HEADS) ** -0.5

    def attend(row0, q, lo, token):
        off = q * quarter + lo

        def load(p, w):
            return qkv[p, :, pl.ds(row0 + (HALO + off - DILATION * w), SUB), :]

        first, *rest = _unstack(load(0, 0))
        query = _stack([after(token, first)] + rest)
        logits = []
        for w in range(WINDOW):
            s = lax.reduce_sum(lax.mul(query, load(1, w)), (0,))
            for bit in (1, 2):
                other = lax.select(lane_bit[bit], pltpu.roll(s, bit, 1), pltpu.roll(s, LANES - bit, 1))
                s = lax.add(s, other)
            if off < DILATION * w:
                row = row0 + off + lax.broadcasted_iota(jnp.int32, (SUB, LANES), 0)
                s = jnp.where(row >= DILATION * w, s, MASKED_LOGIT / scale)
            logits.append(s)
        top = functools.reduce(lax.max, logits)
        weights = [lax.exp2(_times(lax.sub(s, top), scale * np.log2(np.e))) for s in logits]
        inv = lax.div(np.float32(1), functools.reduce(lax.add, weights))
        out = functools.reduce(lax.add, [
            lax.mul(lax.broadcast(weights[w], (groups,)), load(2, w)) for w in range(WINDOW)])
        out = [lax.mul(v, _times(inv, DELTA[q] / DELTA[g // 2])) for g, v in enumerate(_unstack(out))]
        mbuf[1, q, :, :, pl.ds(lo % (2 * PACK), SUB), :] = lax.reshape(
            _stack(swap_group_and_lane_bits(out, 1)), (4, 2, SUB, LANES))

    _wait(*down_copies(0), *down_copies(1))

    @pl.loop(0, n_tiles)
    def _(step):
        row0 = pl.multiple_of(step * TILE, TILE)
        plan = []
        for lo in range(0, TILE, PACK):
            first, last = 43 * lo / TILE, 43 * (lo + PACK) / TILE
            plan += [
                (_jobs(attend, [(row0, q, lo + i) for q in range(4) for i in (0, SUB)]), first, last),
                (left_jobs(lambda q, g, lo: mbuf[1, q, g // 2, g % 2, pl.ds(lo % (2 * PACK), PACK), :],
                           row0, [lo]), last + 1, last + 5)]
        matmul = _Matmuls(*plan)
        row0 = pl.multiple_of(step // 2 * (2 * TILE), 2 * TILE)
        for i in range(7):
            half = (step + 2 * i) % 2
            right = _operands(STRASSEN_RIGHT, [i], lambda r, c: lax.concatenate(
                [_unpack(wbuf.bitcast(U32)[down_slot + n // 2, 4 * half + c,
                                           pl.ds((n % 2 * FCHUNK + r * LANES) // 2, LANES // 2), :])
                 for n in range(n_chunks)], 0))
            blocks = _strassen(lambda j: matmul(
                _load(ha, (i, j, slice(None)), row0, 2 * TILE), _bf16(_unstack(right(j))[0])))
            for j, block in enumerate(blocks):
                mbuf[0, i, j] = lax.reshape(block, (2, TILE, LANES))
        for j in range(4):
            blocks = _strassen(lambda i: lax.reshape(mbuf[0, i, j], (2 * TILE, LANES)))
            for i, block in enumerate(blocks):
                r, c = _position(i, j)
                gbuf[step % 2, c, r, pl.ds(row0, 2 * TILE), :] = _silu(block, _unscale(r, c))

    def output_jobs(t, complete=range(4), outer=range(4), inner=range(4)):
        def use(r, c, g, lo, attn):
            rows = pl.ds(t * TILE + lo, PACK)
            x = lax.convert_element_type(xbuf[r, rows, pl.ds(g * hd + c * LANES, LANES)], F32)
            group = 4 * g + c + (zero if lo == g == 0 and (r, c) == _position(outer[0], inner[0]) else 0)
            wbuf[staged(r, group, t * TILE + lo, PACK)] = _bf16(
                lax.add(x, lax.mul(attn, gbuf[g, c, r, rows, :])))

        return finish_jobs(1 - t % 2, PACK, use, outer, inner) + [
            lambda _: _start(*[cp for q in complete for cp in out_copies(t, q)])]

    matmul = _Matmuls(
        *refill_late(o_slot, heads=True),
        (output_jobs(0), *during(1)), (output_jobs(1), *during(2)),
        (output_jobs(2), 147, 176), (output_jobs(3, [], [1]), 176, 182), (output_jobs(3, [0, 1], [0]), 182, 188))
    for t in range(n_tiles):
        project(matmul, t, 1 - t % 2)
    for job in output_jobs(3, [2], [2, 3], [1, 0]) + output_jobs(3, [3], [2, 3], [2, 3]):
        job(None)
    pltpu.make_async_copy(out_hbm, out_hbm, out_sem).wait()


@jax.jit
def pallas_recurrent_scan__sliding_local_dilated__geglu_ffn__prompt_kernel(
    A_x: jax.Array,
    A_wqkv: jax.Array,
    A_wo: jax.Array,
    B_x: jax.Array,
    B_w_gate: jax.Array,
    B_w_up: jax.Array,
    B_w_down: jax.Array,
):
    del B_x
    b, s, d = A_x.shape
    f = B_w_gate.shape[1]
    assert (b, s, d, f) == (1, 16 * TILE, 8 * LANES, 7 * FCHUNK) and A_x.dtype == BF16
    quarter, groups = s // 4, d // LANES

    hbm = pl.BlockSpec(memory_space=pl.ANY)
    out = pl.pallas_call(
        _kernel,
        out_shape=jax.ShapeDtypeStruct((4, quarter, d), BF16),
        in_specs=[hbm] * 6,
        out_specs=hbm,
        scratch_shapes=[
            pltpu.VMEM((4, quarter, d), BF16),
            pltpu.VMEM((6, groups, d, LANES), BF16),
            pltpu.VMEM((7, 7, 2, quarter, LANES), BF16),
            pltpu.VMEM((7, 7, 2, d // 4, LANES), BF16),
            pltpu.VMEM((3, 7, 2, d // 4, LANES), BF16),
            pltpu.VMEM((7, 7, f // FCHUNK, quarter, LANES), BF16),
            pltpu.VMEM((2, 7, 4, 2, TILE, LANES), F32),
            pltpu.VMEM((3, groups, HALO + s, LANES), F32),
            pltpu.VMEM((2, 4, 4, quarter, LANES), F32),
            pltpu.SemaphoreType.DMA((4,)),
            pltpu.SemaphoreType.DMA((12,)),
            pltpu.SemaphoreType.DMA(()),
        ],
        compiler_params=pltpu.CompilerParams(
            vmem_limit_bytes=127 * 1024 * 1024, disable_bounds_checks=True),
        name="fused_local_attn_geglu",
    )(A_x.reshape(4, quarter, d), A_wqkv, A_wo, B_w_gate, B_w_up, B_w_down)
    return out.reshape(b, s, d)
```

```python
import functools

import jax
import jax.numpy as jnp
import numpy as np
from jax import lax
import jax.experimental.pallas as pl
import jax.experimental.pallas.tpu as pltpu

F32 = jnp.float32
BF16 = jnp.bfloat16
U32 = jnp.uint32

N_HEADS = 32
WINDOW = 8
DILATION = 2
LN_EPS = 1e-5
MASKED_LOGIT = -1e9

LANES = 128
SUB = 8
PACK = 16
HALO = 16
FCHUNK = 512
TILE = 128
PLAIN = 2


STRASSEN_LEFT = ("c+d", "d", "a+b", "a", "t", "c-a", "b-d")
STRASSEN_RIGHT = ("a", "c-a", "d", "b-d", "t", "a+b", "c+d")


def _strassen(m):
    m0, m1 = m(0), m(1)
    c = lax.add(m0, m1)
    m2, m3 = m(2), m(3)
    b = lax.add(m2, m3)
    m4 = m(4)
    d = lax.add(lax.add(m4, lax.sub(m3, m0)), m(5))
    a = lax.add(lax.add(m4, lax.sub(m1, m2)), m(6))
    return a, b, c, d


BALANCED_LEFT = ("a-b", "a+b", "t+t", "d-b", "d+b", "t-s", "t+s")
BALANCED_RIGHT = ("d-b", "d+b", "t", "t+s", "t-s", "a+b", "a-b")
LEFT_FAMILIES = ((0, 1), (2, 5, 6), (3, 4))
LEFT_ORDER = sum(LEFT_FAMILIES, ())
RIGHT_FAMILIES = ((0, 1), (2, 3, 4), (5, 6))
DELTA = (1.0, 3.0 ** 0.5, 3.0 ** 0.5, 3.0)


def _balanced(m):
    m0, m1 = m(0), m(1)
    b = lax.sub(m1, m0)
    diag = lax.sub(m(2), lax.add(m0, m1))
    m3, m4 = m(3), m(4)
    a = lax.sub(diag, lax.add(m3, m4))
    low = lax.add(b, lax.sub(m3, m4))
    m5, m6 = m(5), m(6)
    return a, b, lax.add(low, lax.sub(m6, m5)), lax.sub(diag, lax.add(m5, m6))


def _unscale(r, c):
    return DELTA[c] / DELTA[r] / 4


def _position(outer, inner):
    return outer // 2 * 2 + inner // 2, outer % 2 * 2 + inner % 2


def _combinations(quadrant):
    @functools.cache
    def term(name):
        if len(name) == 3:
            return (lax.add if name[1] == "+" else lax.sub)(term(name[0]), term(name[2]))
        if name in "ts":
            return term("a+d" if name == "t" else "b+c")
        return quadrant("abcd".index(name))

    return term


def _operands(side, family, block):
    outer = _combinations(lambda i: _stack([block(*_position(i, j)) for j in range(4)]))
    parts = _stack([outer(side[i]) for i in family])
    inner = _combinations(lambda j: lax.index_in_dim(parts, j, 1, keepdims=False))
    return lambda j: inner(side[j])


def _token(value, row, n, dtype):
    x = lax.slice(value, (row, 0), (row + SUB, LANES))
    return lax.concatenate([x if dtype == x.dtype else pltpu.bitcast(x, dtype)] * (n // SUB), 0)


class _Matmuls:
    def __init__(self, *plan):
        self.calls = 0
        self.jobs = sorted(
            ((first + (last - first) * (i + 0.618 * n % 1) / len(jobs), n, job)
             for n, (jobs, first, last) in enumerate(plan) for i, job in enumerate(jobs)),
            key=lambda t: t[:2], reverse=True)

    def __call__(self, lhs, rhs):
        value = lax.dot_general(lhs, rhs, (((1,), (0,)), ((), ())), preferred_element_type=F32)
        while self.jobs and self.jobs[-1][0] < self.calls + 1:
            when, _, job = self.jobs.pop()
            row = int((when - self.calls) * (value.shape[0] // SUB)) * SUB
            job(functools.cache(functools.partial(_token, value, row)))
        self.calls += 1
        return value


def _jobs(fn, args):
    return [functools.partial(fn, *a) for a in args]


def _times(x, c):
    return x if c == 1.0 else lax.mul(x, np.float32(c))


def _plus(x, c):
    return lax.add(x, np.float32(c))


def _aligned(i, n):
    return i if isinstance(i, int) else pl.multiple_of(i, n)


def _stack(xs):
    return lax.reshape(lax.concatenate(xs, 0), (len(xs), *xs[0].shape))


def _unstack(x):
    return [lax.index_in_dim(x, i, 0, keepdims=False) for i in range(x.shape[0])]


def _rows(x, lo, n):
    return lax.slice_in_dim(x, lo, lo + n, axis=0)


def _lane_groups(x):
    return [lax.slice_in_dim(x, j, j + LANES, axis=1) for j in range(0, x.shape[1], LANES)]


def _bf16(x):
    return lax.convert_element_type(x, BF16)


def _unpack(words):
    return lax.convert_element_type(pltpu.bitcast(words, BF16), F32)


def _geglu(g, u, scale):
    k0 = (2 / np.pi) ** 0.5
    t = lax.tanh(lax.mul(g, _plus(_times(lax.mul(g, g), k0 * 0.044715 * scale ** 3), k0 * scale)))
    return lax.mul(lax.mul(_times(g, 0.5 * scale ** 2), u), _plus(t, 1.0))


def _silu(x, scale):
    h = _times(x, 0.5)
    return lax.mul(_times(h, scale), _plus(lax.tanh(h), 1.0))


def _load(ref, index, lo, n):
    words = ref.bitcast(U32)[(*index, pl.ds(_aligned(lo // 2, SUB), n // 2))]
    return lax.concatenate(_unstack(pltpu.bitcast(words, BF16)), 1)


class _ColumnCopy:
    def __init__(self, src, col, dst, sem):
        self.src, self.col, self.dst, self.sem = src, col, dst, sem

    def start(self):
        for g in range(self.dst.shape[0]):
            cols = pl.ds(self.col + g * LANES, LANES)
            pltpu.make_async_copy(self.src.at[:, cols], self.dst.at[g], self.sem).start()

    def wait(self):
        pltpu.make_async_copy(self.dst, self.dst, self.sem).wait()


def _start(*copies):
    for cp in copies:
        cp.start()


def _wait(*copies):
    for cp in copies:
        cp.wait()


def _kernel(x_hbm, wqkv_hbm, wo_hbm, wg_hbm, wu_hbm, wd_hbm, out_hbm,
            xbuf,
            wbuf,
            xa,
            wa,
            wb,
            ha,
            mbuf,
            qkv,
            gbuf,
            x_sem, w_sem, out_sem):
    _, quarter, d = x_hbm.shape
    n_chunks, n_tiles = ha.shape[2], quarter // TILE
    hd, qd, groups = d // 2, d // 4, d // LANES

    def chunk_slot(c):
        return 1 + (c + 2) % 3

    q_slot, k_slot, v_slot, o_slot, down_slot = 0, 4, chunk_slot(1), chunk_slot(n_chunks), 2

    def x_copies(t):
        at = [(slice(None), pl.ds(t * TILE, TILE), pl.ds(col, hd)) for col in (0, hd)]
        return [pltpu.make_async_copy(x_hbm.at[i], xbuf.at[i], x_sem.at[t]) for i in at]

    def w_copy(slot, h, src=None, col=None):
        rows = pl.ds(0, d if src is None else src.shape[0])
        dst = wbuf.at[slot, pl.ds(h * (groups // 2), groups // 2), rows]
        return _ColumnCopy(src, col, dst, w_sem.at[2 * slot + h])

    def chunk_copies(c):
        return [w_copy(chunk_slot(c), h, w, _aligned(c * FCHUNK, FCHUNK)) for h, w in enumerate((wg_hbm, wu_hbm))]

    def down_copies(h):
        f = wd_hbm.shape[0]
        return [w_copy(down_slot + lo // d, h, wd_hbm.at[pl.ds(lo, min(d, f - lo))], _aligned(h * hd, hd))
                for lo in range(0, f, d)]

    def staged(q, g, lo, n):
        return down_slot + q % 2, g, pl.ds(q // 2 * quarter + lo, n)

    def out_copies(t, q):
        return [pltpu.make_async_copy(
            wbuf.at[staged(q, g, t * TILE, TILE)],
            out_hbm.at[q, pl.ds(t * TILE, TILE), pl.ds(g * LANES, LANES)],
            out_sem) for g in range(groups)]

    xs = [x_copies(t) for t in range(n_tiles)]
    wq = [w_copy(q_slot, h, wqkv_hbm, h * hd) for h in range(2)]
    wk = [w_copy(k_slot, h, wqkv_hbm, d + h * hd) for h in range(2)]
    wv = [w_copy(v_slot, h, wqkv_hbm, 2 * d + h * hd) for h in range(2)]

    _start(*xs[0], wk[0])
    zero = lax.fori_loop(0, 2, lambda i, z: lax.min(i, z), 0)
    _start(*xs[1], wk[1])
    _wait(*xs[0])
    _start(*wv)

    never = {n: lax.broadcasted_iota(jnp.int32, (n, LANES), 0) < zero for n in (SUB, PACK, 2 * PACK)}
    lane = lax.broadcasted_iota(jnp.int32, (SUB, LANES), 1)
    lane_bit = {bit: (lane & bit) != 0 for bit in (1, 2, 4, 8, 16)}

    def after(token, x):
        if token is None:
            return x
        return lax.select(never[x.shape[0]], token(x.shape[0], x.dtype), x)

    def swap_group_and_lane_bits(cols, bits=3):
        cols = list(cols)
        for gbit, lbit in ((1, 4), (2, 8), (4, 16))[:bits]:
            for i in range(len(cols)):
                if not i & gbit:
                    a, b = cols[i], cols[i | gbit]
                    cols[i] = lax.select(lane_bit[lbit], pltpu.roll(b, lbit, 1), a)
                    cols[i | gbit] = lax.select(lane_bit[lbit], b, pltpu.roll(a, LANES - lbit, 1))
        return cols

    def operand_jobs(side, family, load, dst, first, row0, positions):
        def job(g, lo, token):
            operand = _operands(side, family, lambda r, c: load(r, c, g, lo, token))
            for j in range(7):
                dst[pl.ds(first, len(family)), j, g, pl.ds(row0 + lo, PACK), :] = _bf16(operand(j))

        return _jobs(job, positions)

    def left_jobs(load, row0, rows):
        return [job for family in LEFT_FAMILIES for job in operand_jobs(
            BALANCED_LEFT, family, lambda r, c, g, lo, token: after(token, load(r, 2 * c + g, lo)),
            xa, LEFT_ORDER.index(family[0]), row0, [(g, lo) for lo in rows for g in range(2)])]

    def right_jobs(slot, family, dst=wa, heads=False):
        family = RIGHT_FAMILIES[family]

        def load(r, c, g, lo, token):
            def rows(at):
                return _unpack(after(token, wbuf.bitcast(U32)[slot, 4 * g + c, pl.ds(at // 2, SUB)]))

            if heads:
                at = lo // PACK % 2 * hd + lo // (2 * PACK) * (2 * PACK) + r // 2 * PACK
                x = lax.concatenate([_rows(rows(at + i * qd), r % 2 * SUB, SUB) for i in range(2)], 0)
            else:
                x = rows(r * qd + lo)
            return _times(x, DELTA[r] / DELTA[c])

        return operand_jobs(BALANCED_RIGHT, family, load, dst, family[0] if dst is wa else 0, 0,
                            [(g, lo) for lo in range(0, qd, PACK) for g in range(2)])

    def move(i, j, g, lo, token):
        rows = pl.ds(lo, 4 * SUB)
        wa.bitcast(U32)[2 + i, j, g, rows, :] = after(token, wb.bitcast(U32)[i, j, g, rows, :])

    moves = _jobs(move, [(i, j, g, lo) for i in range(3) for j in range(7) for g in range(2)
                         for lo in range(0, qd // 2, 4 * SUB)])

    def refill_early(slot, last, **kw):
        return [(right_jobs(slot, 1, wb, **kw), max(last - 90, 23), max(last - 3, 62)),
                (right_jobs(slot, 0, **kw), last + 15.5, last + 46),
                (moves[:len(moves) // 2], last + 24, last + 47)]

    def refill_late(slot, **kw):
        return [(moves[len(moves) // 2:], 0, 22), (right_jobs(slot, 2, **kw), 0, 32)]

    def partial(slot, i, j, g, lo, n):
        if slot < 2:
            return mbuf, (slot, i, j, pl.ds(*g), pl.ds(lo, n))
        return gbuf, (1, j, pl.ds(i // 4 * 2 + g[0], g[1]), pl.ds(i % 4 * TILE + lo, n))

    def project(matmul, t, slot):
        for i in range(7):
            blocks = _balanced(lambda j: matmul(
                _load(xa, (LEFT_ORDER.index(i), j, slice(None)), t * TILE, TILE),
                _load(wa, (i, j, slice(None)), 0, qd)))
            for j, block in enumerate(blocks):
                ref, index = partial(slot, i, j, (0, 2), 0, TILE)
                ref[index] = _stack(_lane_groups(block))

    def finish_jobs(slot, n, use, outer=range(4), inner=range(4)):
        def job(lo, j, g, token):
            def product(i):
                ref, index = partial(slot, i, j, g, lo, n)
                return after(None if i else token, lax.reshape(ref[index], (PACK, LANES)))

            out = _balanced(product)
            for i in outer:
                use(*_position(i, j), g[0], lo, out[i])

        return _jobs(job, [(lo, j, g) for lo in range(0, TILE, n) for j in inner
                           for g in (((0, 1), (1, 1)) if n == PACK else ((0, 2),))])

    def during(step):
        return 49 * step, 49 * step + 48

    def norm(q, lo, token):
        first, *rest = _lane_groups(lax.convert_element_type(xbuf[q, pl.ds(lo, SUB), :], F32))
        x = lax.concatenate([after(token, first)] + rest, 1)
        x = x - jnp.sum(x, axis=-1, keepdims=True) * (1.0 / d)
        inv = lax.rsqrt(jnp.sum(x * x, axis=-1, keepdims=True) * (1.0 / d) + LN_EPS)
        inv = lax.broadcast_in_dim(inv, (SUB, LANES), (0, 1))
        x = [lax.mul(v, _times(inv, DELTA[q] / DELTA[g // 2])) for g, v in enumerate(_lane_groups(x))]
        gbuf[:, :, q, pl.ds(lo, SUB), :] = lax.reshape(_stack(x), (2, 4, SUB, LANES))
        if lo < PLAIN * TILE and lo % PACK:
            lo -= SUB
            x = [_times(gbuf[g // 4, g % 4, q, pl.ds(lo, PACK), :], DELTA[g // 2] / DELTA[q])
                 for g in range(groups)]
            for g, v in enumerate(x):
                ha[lo // TILE, g // 4, g % 4, pl.ds(q * TILE + lo % TILE, PACK), :] = _bf16(v)

    def norm_jobs(t):
        return _jobs(norm, [(q, t * TILE + lo) for q in range(4) for lo in range(0, TILE, SUB)])

    def split_x_jobs(t):
        return left_jobs(lambda q, g, lo: gbuf[g // 4, g % 4, q, pl.ds(lo, PACK), :],
                         0, range(t * TILE, (t + 1) * TILE, PACK))

    def shuffle_weight_jobs(slot):
        words = wbuf.bitcast(U32)

        def job(lo, token):
            at = (slot, slice(None), pl.ds(lo // 2, SUB))
            words[at] = _stack(swap_group_and_lane_bits([after(token, v) for v in _unstack(words[at])]))

        return _jobs(job, [(lo + r * qd,) for lo in range(0, qd, PACK) for r in range(4)])

    def plain_k(t, gs, *plan):
        matmul = _Matmuls(*plan)
        for g in gs:
            k = lax.add(*[matmul(_load(ha, (t, h, pl.ds(0, 4)), 0, 4 * TILE),
                                 _load(wbuf, (k_slot, pl.ds(g, 1)), h * hd, hd)) for h in range(2)])
            k = pltpu.bitcast(_bf16(k), F32)
            for lo in range(0, 4 * TILE, PACK):
                row = HALO + lo // TILE * quarter + t * TILE + lo % TILE
                qkv[1, g, pl.ds(row, SUB), :] = _rows(k, lo // 2, SUB)

    def shuffle_k(row, token):
        cols = [after(token, v) for v in _unstack(pltpu.bitcast(qkv[1, :, pl.ds(row, SUB), :], U32))]
        qkv[1, :, pl.ds(row, PACK), :] = _unpack(_stack(swap_group_and_lane_bits(cols)))

    def finish_qkv(p, t, slot):
        def use(r, c, _, lo, x):
            x = _times(x, _unscale(r, c))
            for g in range(2):
                qkv[p, 4 * g + c, pl.ds(HALO + r * quarter + t * TILE + lo, SUB), :] = _rows(x, g * SUB, SUB)

        return finish_jobs(slot, SUB, use)

    for job in norm_jobs(0):
        job(None)
    wk[0].wait()
    _start(*xs[2], *xs[3])
    plain_k(0, range(4), (split_x_jobs(0), 0, 7))
    _wait(*xs[1], wk[1])
    _start(*wq, *chunk_copies(0))
    plain_k(0, range(4, 8), (norm_jobs(1), 0, 6.5))
    _wait(*wv)
    plain_k(1, range(8), (shuffle_weight_jobs(v_slot), 0, 13.5),
            *[(right_jobs(v_slot, f), 1.5, 15.5) for f in range(3)])
    _start(*chunk_copies(1))
    _wait(*xs[2], *xs[3])
    matmul = _Matmuls((norm_jobs(2) + norm_jobs(3), 0, 42), (split_x_jobs(1)[:28], 0, 48))
    project(matmul, 0, 0)
    _wait(*wq)
    matmul = _Matmuls(
        (split_x_jobs(1)[28:], 0, 19), (split_x_jobs(2), 0, 49), (split_x_jobs(3), 49, 97.5),
        *[(finish_qkv(2, t, t % 2), *during(t)) for t in range(3)],
        (shuffle_weight_jobs(k_slot), 0, 96),
        (right_jobs(k_slot, 1, wb), 98, 119), (right_jobs(k_slot, 0), 119, 146),
        (moves[:len(moves) // 2], 121, 146))
    project(matmul, 1, 1)
    project(matmul, 2, 0)

    @pl.loop(0, 2)
    def _(h):
        w_copy(chunk_slot(0), h).wait()

    project(matmul, 3, 1)
    matmul = _Matmuls(
        *refill_late(k_slot), *refill_early(chunk_slot(0), 49),
        (shuffle_weight_jobs(q_slot), 0, 92),
        (finish_qkv(2, 3, 1), *during(0)), (finish_qkv(1, 2, 0), *during(1)))
    project(matmul, 2, 0)
    project(matmul, 3, 2)

    def geglu_jobs(t):
        def use(r, c, _, lo, x):
            gbuf[0, c, r, pl.ds(t * TILE + lo, SUB), :] = _geglu(
                _rows(x, 0, SUB), _rows(x, SUB, SUB), _unscale(r, c))

        return finish_jobs(t % 2, SUB, use)

    def split_hidden_jobs(chunk, t):
        return [job for lo in range(t * TILE, (t + 1) * TILE, PACK)
                for family in ((0, 1), (2, 3), (4,), (5,), (6,)) for job in operand_jobs(
                    STRASSEN_LEFT, family,
                    lambda r, c, g, lo, token: after(token, gbuf[0, c, r, pl.ds(lo, PACK), :]),
                    ha, family[0], 0, [(chunk, lo)])]

    @pl.loop(0, n_chunks)
    def _(c):
        pl.when(c + 1 < n_chunks)(lambda: _wait(*chunk_copies(c + 1)))
        pl.when(c + 2 < n_chunks)(lambda: _start(*chunk_copies(c + 2)))
        pl.when(c + 2 == n_chunks)(
            lambda: _start(*[w_copy(o_slot, h, wo_hbm, h * hd) for h in range(2)]))
        previous = jnp.maximum(c - 1, 0)
        following = jnp.where(c + 1 < n_chunks, chunk_slot(c + 1), q_slot)
        matmul = _Matmuls(
            *refill_late(chunk_slot(c)), *refill_early(following, 147),
            *[(geglu_jobs((t - 1) % n_tiles), *during(t)) for t in range(n_tiles)],
            (split_hidden_jobs(previous, 2), 30, 60), (split_hidden_jobs(previous, 3), 60, 98),
            (split_hidden_jobs(c, 0), 98, 145), (split_hidden_jobs(c, 1), 145, 160))
        for t in range(n_tiles):
            project(matmul, t, t % 2)

    @pl.loop(0, 2)
    def _(h):
        w_copy(o_slot, h).wait()
        _start(*down_copies(h))

    matmul = _Matmuls(
        *refill_late(q_slot), *refill_early(o_slot, 147, heads=True),
        (split_hidden_jobs(n_chunks - 1, 2), 30, 60), (split_hidden_jobs(n_chunks - 1, 3), 60, 98),
        (finish_qkv(1, 3, 2), 49, 147),
        (_jobs(shuffle_k, [(HALO + q * quarter + lo,) for lo in range(0, PLAIN * TILE, PACK)
                           for q in range(4)]), 35, 165),
        (geglu_jobs(n_tiles - 1), *during(0)),
        *[(finish_qkv(0, t, t % 2), *during(t + 1)) for t in range(n_tiles - 1)])
    for t in range(n_tiles):
        project(matmul, t, t % 2)
    for job in finish_qkv(0, n_tiles - 1, 1):
        job(None)

    for p in (1, 2):
        for g in range(groups):
            qkv[p, g, pl.ds(0, HALO), :] = jnp.broadcast_to(qkv[p, g, pl.ds(HALO, 1), :], (HALO, LANES))

    scale = float(d // N_HEADS) ** -0.5

    def attend(row0, q, lo, token):
        off = q * quarter + lo

        def load(p, w):
            return qkv[p, :, pl.ds(row0 + (HALO + off - DILATION * w), SUB), :]

        first, *rest = _unstack(load(0, 0))
        query = _stack([after(token, first)] + rest)
        logits = []
        for w in range(WINDOW):
            s = lax.reduce_sum(lax.mul(query, load(1, w)), (0,))
            for bit in (1, 2):
                other = lax.select(lane_bit[bit], pltpu.roll(s, bit, 1), pltpu.roll(s, LANES - bit, 1))
                s = lax.add(s, other)
            if off < DILATION * w:
                row = row0 + off + lax.broadcasted_iota(jnp.int32, (SUB, LANES), 0)
                s = jnp.where(row >= DILATION * w, s, MASKED_LOGIT / scale)
            logits.append(s)
        top = functools.reduce(lax.max, logits)
        weights = [lax.exp2(_times(lax.sub(s, top), scale * np.log2(np.e))) for s in logits]
        inv = lax.div(np.float32(1), functools.reduce(lax.add, weights))
        out = functools.reduce(lax.add, [
            lax.mul(lax.broadcast(weights[w], (groups,)), load(2, w)) for w in range(WINDOW)])
        out = [lax.mul(v, _times(inv, DELTA[q] / DELTA[g // 2])) for g, v in enumerate(_unstack(out))]
        mbuf[1, q, :, :, pl.ds(lo % (2 * PACK), SUB), :] = lax.reshape(
            _stack(swap_group_and_lane_bits(out, 1)), (4, 2, SUB, LANES))

    _wait(*down_copies(0), *down_copies(1))

    @pl.loop(0, n_tiles)
    def _(step):
        row0 = pl.multiple_of(step * TILE, TILE)
        plan = []
        for lo in range(0, TILE, PACK):
            first, last = 43 * lo / TILE, 43 * (lo + PACK) / TILE
            plan += [
                (_jobs(attend, [(row0, q, lo + i) for q in range(4) for i in (0, SUB)]), first, last),
                (left_jobs(lambda q, g, lo: mbuf[1, q, g // 2, g % 2, pl.ds(lo % (2 * PACK), PACK), :],
                           row0, [lo]), last + 1, last + 5)]
        matmul = _Matmuls(*plan)
        row0 = pl.multiple_of(step // 2 * (2 * TILE), 2 * TILE)
        for i in range(7):
            half = (step + 2 * i) % 2
            right = _operands(STRASSEN_RIGHT, [i], lambda r, c: lax.concatenate(
                [_unpack(wbuf.bitcast(U32)[down_slot + n // 2, 4 * half + c,
                                           pl.ds((n % 2 * FCHUNK + r * LANES) // 2, LANES // 2), :])
                 for n in range(n_chunks)], 0))
            blocks = _strassen(lambda j: matmul(
                _load(ha, (i, j, slice(None)), row0, 2 * TILE), _bf16(_unstack(right(j))[0])))
            for j, block in enumerate(blocks):
                mbuf[0, i, j] = lax.reshape(block, (2, TILE, LANES))
        for j in range(4):
            blocks = _strassen(lambda i: lax.reshape(mbuf[0, i, j], (2 * TILE, LANES)))
            for i, block in enumerate(blocks):
                r, c = _position(i, j)
                gbuf[step % 2, c, r, pl.ds(row0, 2 * TILE), :] = _silu(block, _unscale(r, c))

    def output_jobs(t, complete=range(4), outer=range(4), inner=range(4)):
        def use(r, c, g, lo, attn):
            rows = pl.ds(t * TILE + lo, PACK)
            x = lax.convert_element_type(xbuf[r, rows, pl.ds(g * hd + c * LANES, LANES)], F32)
            group = 4 * g + c + (zero if lo == g == 0 and (r, c) == _position(outer[0], inner[0]) else 0)
            wbuf[staged(r, group, t * TILE + lo, PACK)] = _bf16(
                lax.add(x, lax.mul(attn, gbuf[g, c, r, rows, :])))

        return finish_jobs(1 - t % 2, PACK, use, outer, inner) + [
            lambda _: _start(*[cp for q in complete for cp in out_copies(t, q)])]

    matmul = _Matmuls(
        *refill_late(o_slot, heads=True),
        (output_jobs(0), *during(1)), (output_jobs(1), *during(2)),
        (output_jobs(2), 147, 176), (output_jobs(3, [], [1]), 176, 182), (output_jobs(3, [0, 1], [0]), 182, 188))
    for t in range(n_tiles):
        project(matmul, t, 1 - t % 2)
    for job in output_jobs(3, [2], [2, 3], [1, 0]) + output_jobs(3, [3], [2, 3], [2, 3]):
        job(None)
    pltpu.make_async_copy(out_hbm, out_hbm, out_sem).wait()


@jax.jit
def pallas_recurrent_scan__sliding_local_dilated__geglu_ffn__prompt_kernel(
    A_x: jax.Array,
    A_wqkv: jax.Array,
    A_wo: jax.Array,
    B_x: jax.Array,
    B_w_gate: jax.Array,
    B_w_up: jax.Array,
    B_w_down: jax.Array,
):
    del B_x
    b, s, d = A_x.shape
    f = B_w_gate.shape[1]
    assert (b, s, d, f) == (1, 16 * TILE, 8 * LANES, 7 * FCHUNK) and A_x.dtype == BF16
    quarter, groups = s // 4, d // LANES

    hbm = pl.BlockSpec(memory_space=pl.ANY)
    out = pl.pallas_call(
        _kernel,
        out_shape=jax.ShapeDtypeStruct((4, quarter, d), BF16),
        in_specs=[hbm] * 6,
        out_specs=hbm,
        scratch_shapes=[
            pltpu.VMEM((4, quarter, d), BF16),
            pltpu.VMEM((6, groups, d, LANES), BF16),
            pltpu.VMEM((7, 7, 2, quarter, LANES), BF16),
            pltpu.VMEM((7, 7, 2, d // 4, LANES), BF16),
            pltpu.VMEM((3, 7, 2, d // 4, LANES), BF16),
            pltpu.VMEM((7, 7, f // FCHUNK, quarter, LANES), BF16),
            pltpu.VMEM((2, 7, 4, 2, TILE, LANES), F32),
            pltpu.VMEM((3, groups, HALO + s, LANES), F32),
            pltpu.VMEM((2, 4, 4, quarter, LANES), F32),
            pltpu.SemaphoreType.DMA((4,)),
            pltpu.SemaphoreType.DMA((12,)),
            pltpu.SemaphoreType.DMA(()),
        ],
        compiler_params=pltpu.CompilerParams(
            vmem_limit_bytes=127 * 1024 * 1024, disable_bounds_checks=True),
        name="fused_local_attn_geglu",
    )(A_x.reshape(4, quarter, d), A_wqkv, A_wo, B_w_gate, B_w_up, B_w_down)
    return out.reshape(b, s, d)
```
